```python
import jax
import jax.numpy as jnp

def _softmax(x, axis=-1):
    return jax.nn.softmax(x, axis=axis)
def _gelu(x):
    return jax.nn.gelu(x, approximate=True)
def _silu(x):
    return jax.nn.silu(x)
def _sigmoid(x):
    return jax.nn.sigmoid(x)
def _layernorm(x, axis=-1, eps=1e-5):
    m = jnp.mean(x, axis=axis, keepdims=True)
    v = jnp.var(x, axis=axis, keepdims=True)
    return (x - m) / jnp.sqrt(v + eps)
def _scatter_add(tgt, idx, src, axis=0):
    return tgt.at[idx].add(src)
def _segment_sum(src, seg, n):
    return jax.ops.segment_sum(src, seg, n)
class _Rng:
    def __init__(self, key):
        self._k = key
    def _next(self):
        self._k, sub = jax.random.split(self._k)
        return sub
    def normal(self, shape):
        return jax.random.normal(self._next(), shape, dtype=jnp.bfloat16)
    def randint(self, lo, hi, shape):
        return jax.random.randint(self._next(), shape, lo, hi, dtype=jnp.int32)
    def uniform(self, shape, lo=0.0, hi=1.0):
        return jax.random.uniform(self._next(), shape, jnp.bfloat16, lo, hi)
    def permutation(self, n):
        return jax.random.permutation(self._next(), n)


kernel_name = 'interleave_layers__sliding_local_dilated__softmax_full_mha__prompt'

def setup_inputs():
    _rng = _Rng(jax.random.key(int.from_bytes(__import__("os").urandom(4), "little")))
    _w = (lambda a: (lambda t: t.astype(jnp.bfloat16) if jnp.issubdtype(t.dtype, jnp.floating) else t)(jnp.asarray(a)))
    def _A_setup():
        B, S, D = 1, 2048, 1024
        return {
            "x": _w((lambda *s: _rng.normal(s) * 0.05)(B, S, D)),
            "wqkv": _w((lambda *s: _rng.normal(s) * 0.05)(D, 3 * D)),
            "wo": _w((lambda *s: _rng.normal(s) * 0.05)(D, D)),
        }
    _A_in = _A_setup()

    def _B_setup():
        B, S, D = 1, 2048, 1024
        return {
            "x": _w((lambda *s: _rng.normal(s) * 0.05)(B, S, D)),
            "wqkv": _w((lambda *s: _rng.normal(s) * 0.05)(D, 3 * D)),
            "wo": _w((lambda *s: _rng.normal(s) * 0.05)(D, D)),
        }
    _B_in = _B_setup()

    return {
        "A_x": _A_in["x"],
        "A_wqkv": _A_in["wqkv"],
        "A_wo": _A_in["wo"],
        "B_x": _B_in["x"],
        "B_wqkv": _B_in["wqkv"],
        "B_wo": _B_in["wo"],
    }

def reference(A_x, A_wqkv, A_wo, B_x, B_wqkv, B_wo):
    def _A_ref(x, wqkv, wo):
        B, S, D = x.shape
        H = 32; Dh = D // H
        W, dil = 8, 2
        qkv = (lambda x, *d: x.transpose(*d))((x @ wqkv).reshape(B, S, 3, H, Dh), 2, 0, 3, 1, 4)
        q, k, v = qkv[0], qkv[1], qkv[2]
        scale = Dh ** -0.5
        pos = jnp.arange(S)
        off = jnp.arange(W) * dil
        idx = pos[:, None] - off[None, :]
        mask = idx >= 0
        idx_c = jnp.where(mask, idx, 0).reshape(-1)
        kg = k[:, :, idx_c, :].reshape(B, H, S, W, Dh)
        vg = v[:, :, idx_c, :].reshape(B, H, S, W, Dh)
        logits = jnp.einsum("bhsd,bhswd->bhsw", q, kg) * scale
        logits = jnp.where(mask[None, None, :, :], logits, -1e9)
        attn = _softmax(logits, axis=-1)
        o = jnp.einsum("bhsw,bhswd->bhsd", attn, vg)
        return (lambda x, *d: x.transpose(*d))(o, 0, 2, 1, 3).reshape(B, S, D) @ wo

    def _B_ref(x, wqkv, wo):
        B, S, D = x.shape
        H = 32; Dh = D // H
        qkv = (lambda x, *d: x.transpose(*d))((x @ wqkv).reshape(B, S, 3, H, Dh), 2, 0, 3, 1, 4)
        q, k, v = qkv[0], qkv[1], qkv[2]
        scale = Dh ** -0.5
        scores = jnp.einsum("bhqd,bhkd->bhqk", q, k) * scale
        p = _softmax(scores, axis=-1)
        o = jnp.einsum("bhqk,bhkd->bhqd", p, v)
        return (lambda x, *d: x.transpose(*d))(o, 0, 2, 1, 3).reshape(B, S, D) @ wo

    x = A_x
    x = x + _A_ref(_layernorm(x, axis=-1), A_wqkv, A_wo)
    x = x + _B_ref(_layernorm(x, axis=-1), B_wqkv, B_wo)
    x = x + _A_ref(_layernorm(x, axis=-1), A_wqkv, A_wo)
    x = x + _B_ref(_layernorm(x, axis=-1), B_wqkv, B_wo)
    return x
```

```python
import math

import jax
import jax.numpy as jnp
from jax import lax
import jax.experimental.pallas as pl
import jax.experimental.pallas.tpu as pltpu

SEQ, D, HEADS, DH = 2048, 1024, 32, 32
WIN = 8
NT = SEQ // 128
NG = D // 128
EPS = 1e-5
LOG2E = math.log2(math.e)
QSCALE = DH ** -0.5 * LOG2E
MASKED = -1e9 * LOG2E
ATT_UNROLL = 16

bf16, f32, u32 = jnp.bfloat16, jnp.float32, jnp.uint32


def _words(x):
    return pltpu.bitcast(x.astype(bf16), u32)


def _halves(x):
    return pltpu.bitcast(x, bf16)


def _dot(a, b):
    return jnp.dot(a, b, preferred_element_type=f32)


def _fold(x, op, acc=None):
    for i in range(x.shape[0] // 8):
        slab = x[8 * i:8 * i + 8]
        acc = slab if acc is None else op(acc, slab)
    return acc


def _rows(i, n=128):
    return slice(i * n, (i + 1) * n)


def _interleave(main, side):
    done = 0
    for i, step in enumerate(main):
        step()
        upto = (i + 1) * len(side) // len(main)
        for s in side[done:upto]:
            s()
        done = upto
    for s in side[done:]:
        s()


def _merge(*lists):
    keyed = [((i + 0.5) / len(l), k, s) for k, l in enumerate(lists) for i, s in enumerate(l)]
    return [s for _, _, s in sorted(keyed, key=lambda e: e[:2])]


def _layernorm_steps(load, store):
    st = {}

    def mean():
        acc = None
        for c in range(NG):
            acc = _fold(load(c), jnp.add, acc)
        st["mean"] = jnp.sum(acc, axis=0, keepdims=True) * (1.0 / D)

    def var():
        acc = None
        for c in range(NG):
            d = load(c) - st["mean"]
            acc = _fold(d * d, jnp.add, acc)
        st["rstd"] = lax.rsqrt(jnp.sum(acc, axis=0, keepdims=True) * (1.0 / D) + EPS)

    def norm(c0, c1):
        def step():
            for c in range(c0, c1):
                store(c, (load(c) - st["mean"]) * st["rstd"])
        return step

    return [mean, var, norm(0, NG // 2), norm(NG // 2, NG)]


def _kernel(x_hbm, wqa_hbm, woa_hbm, wqb_hbm, wob_hbm, out_hbm,
            xio, wqa, woa, wqb, wob, wj0, wj1, wot, wqt,
            xa, xb, ht, ot, q0, q1, k0, k1, v0, v1, y0, y1,
            qt, kk, vt, s0, s1, x_sem, w_sem, o_sem):
    wj, qbuf, kbuf, vbuf, ybuf, sbuf = (wj0, wj1), (q0, q1), (k0, k1), (v0, v1), (y0, y1), (s0, s1)

    def x_copy(c):
        return pltpu.make_async_copy(x_hbm.at[:, _rows(c)], xio.at[c], x_sem.at[c])

    def out_copy(c, col):
        return pltpu.make_async_copy(xio.at[c], out_hbm.at[:, col], o_sem.at[c])

    def wqa_copies(g):
        return [pltpu.make_async_copy(wqa_hbm.at[:, _rows(i * NG + g)], wqa.at[3 * g + i],
                                      w_sem.at[g]) for i in range(3)]

    def late_copies():
        cps = [pltpu.make_async_copy(woa_hbm.at[:, _rows(c)], woa.at[c], w_sem.at[NG])
               for c in range(NG)]
        cps += [pltpu.make_async_copy(wqb_hbm.at[:, _rows(i * NG + g)], wqb.at[3 * g + i],
                                      w_sem.at[NG]) for g in range(NG) for i in range(3)]
        cps += [pltpu.make_async_copy(wob_hbm.at[:, _rows(c)], wob.at[c], w_sem.at[NG])
                for c in range(NG)]
        return cps

    def transpose_steps(src, i, dst, j):
        def step(k):
            def run():
                for kt in (2 * k, 2 * k + 1):
                    dst[j, :, _rows(kt)] = pltpu.bitcast(src[i, _rows(kt), :].T, u32)
            return run
        return [step(k) for k in range(NG // 2)]

    def local_qkv_steps(unit, slot):
        par = unit // NG

        def step(r, i):
            def run():
                y = _dot(_halves(wj[slot][i]), _halves(ht[2 * r + par]))
                if i == 0:
                    qbuf[slot][r] = y * QSCALE
                    return
                buf = kbuf[slot] if i == 1 else vbuf[slot]
                buf[r + WIN - 1] = y
                if r > 0:
                    buf[r - 1] = pltpu.roll(y, 1, 1)
            return run
        return [step(r, i) for r in range(WIN) for i in (1, 2, 0)]

    def local_att_steps(unit, slot):
        g, par = unit % NG, unit // NG

        def step(r, h):
            def run():
                rows = _rows(h, DH)
                q = qbuf[slot][r, rows, :]
                first = lax.broadcasted_iota(jnp.int32, (1, 128), 1) == 0
                logits = []
                for w in range(WIN):
                    l = jnp.sum(q * kbuf[slot][r - w + WIN - 1, rows, :], axis=0, keepdims=True)
                    logits.append(jnp.where(first, MASKED, l) if w > r else l)
                m = logits[0]
                for l in logits[1:]:
                    m = jnp.maximum(m, l)
                den = acc = None
                for w in range(WIN):
                    p = jnp.exp2(logits[w] - m)
                    pv = p * vbuf[slot][r - w + WIN - 1, rows, :]
                    den = p if den is None else den + p
                    acc = pv if acc is None else acc + pv
                o = acc * pl.reciprocal(den)
                ot[2 * r + par, g, _rows(h, DH // 2), :] = _words(o)
            return run
        return [step(r, h) for h in range(4) for r in range(WIN)]

    def local_w_steps(unit, slot):
        g = unit % NG
        return [s for i in range(3) for s in transpose_steps(wqa, 3 * g + i, wj[slot], i)]

    def tile_ln_steps(t):
        def store(c, h):
            ht[t, _rows(c, 64), :] = _words(h)
        return _layernorm_steps(lambda c: xa[t, c], store)

    def proj_steps(t, slot):
        def step(c):
            def run():
                ybuf[slot][c] = xa[t, c] + _dot(_halves(wot[c]), _halves(ot[t].reshape(D // 2, 128)))
            return run
        return [step(c) for c in range(NG)]

    def proj_ln_steps(t, slot):
        def store(c, h):
            xb[t, c] = ybuf[slot][c]
            ht[t, _rows(c, 64), :] = _words(h)
        return _layernorm_steps(lambda c: ybuf[slot][c], store)

    def local_layer(rep):
        def wait_w(g):
            @pl.when(rep == 0)
            def _():
                pltpu.make_async_copy(wqa.at[pl.ds(0, 3)], wqa.at[pl.ds(0, 3)], w_sem.at[g]).wait()

        wait_w(1)
        ln = [tile_ln_steps(t) for t in list(range(0, NT, 2)) + list(range(1, NT, 2))]
        for s in ln[0]:
            s()
        mm = local_qkv_steps(0, 0)
        wsteps = local_w_steps(1, 1)
        for r in range(WIN):
            side = (ln[r + 1] if r + 1 < WIN else []) + ln[WIN + r]
            _interleave(mm[3 * r:3 * r + 3], _merge(side, wsteps[len(wsteps) * r // WIN:
                                                                  len(wsteps) * (r + 1) // WIN]))

        def unit_pair(j, _):
            @pl.when(j < NG // 2 - 1)
            def _():
                wait_w(2 * j + 2)
                wait_w(2 * j + 3)

            for u, slot in ((2 * j + 1, 1), (2 * j + 2, 0)):
                _interleave(local_qkv_steps(u, slot),
                            _merge(local_att_steps(u - 1, 1 - slot), local_w_steps(u + 1, 1 - slot)))

        lax.fori_loop(0, NG - 1, unit_pair, None)

        @pl.when(rep == 0)
        def _():
            for cp in late_copies():
                cp.wait()

        last = 2 * NG - 1
        _interleave(local_qkv_steps(last, 1),
                    _merge(local_att_steps(last - 1, 0),
                           [s for c in range(NG) for s in transpose_steps(woa, c, wot, c)]))

        _interleave(proj_steps(0, 0) + proj_steps(2, 1), local_att_steps(last, 1))

        def tile(i):
            return 2 * (i % WIN) + i // WIN

        for s in proj_ln_steps(0, 0):
            s()

        def tile_pair(j, _):
            for i, slot in ((2 * j + 2, 0), (2 * j + 3, 1)):
                cols = [jnp.minimum(2 * i - 4 + e, 3 * NG - 1) for e in range(2)]
                _interleave(proj_steps(tile(i), slot),
                            _merge(proj_ln_steps(tile(i - 1), 1 - slot),
                                   [s for c in cols for s in transpose_steps(wqb, c, wqt, c)]))

        lax.fori_loop(0, NT // 2 - 1, tile_pair, None)
        for s in proj_ln_steps(NT - 1, 1):
            s()

    def full_qkv(g, _):
        def step(t, i):
            def run():
                y = _dot(_halves(wqt[3 * g + i]), _halves(ht[t]))
                if i == 0:
                    qt[g * NT + t] = _words(y * QSCALE)
                elif i == 1:
                    kk[g, _rows(t, 64), :] = pltpu.bitcast(y.astype(bf16).T, u32)
                else:
                    vt[g, :, _rows(t)] = _words(y)
            return run
        _interleave([step(t, i) for i in (1, 0, 2) for t in range(NT)],
                    transpose_steps(wob, g, wot, g))

    chunk = 512
    nchunk = SEQ // chunk

    def full_att(base, count, state, first=False, last=False):
        m, m_next, den, acc = state
        for u in range(count + (2 if last else 0)):
            scores = u < count
            if scores:
                blk = base + u // 4
                h = u % 4
                parts = [jnp.zeros((DH // 2, 128), u32)] * 4
                parts[h] = qt[blk, _rows(h, DH // 2), :]
                q = _halves(jnp.concatenate(parts, axis=0))
                top = None
            for c in range(nchunk):
                if scores:
                    for kt in range(4 * c, 4 * c + 4):
                        s = _dot(_halves(kk[blk // NT, _rows(kt, 64), :]), q)
                        sbuf[u % 2][_rows(kt), :] = s
                        top = _fold(s, jnp.maximum, top)
                up, cp = divmod((u - 1) * nchunk + c - 1, nchunk)
                if (first and up < 0) or up >= count:
                    continue
                if cp == 0:
                    m, den, acc = m_next, None, None
                blkp = base + up // 4
                gp, hp = blkp // NT, up % 4
                ps = []
                for kt in range(4 * cp, 4 * cp + 4):
                    p = jnp.exp2(sbuf[up % 2][_rows(kt), :] - m)
                    den = _fold(p, jnp.add, den)
                    ps.append(p.astype(bf16))
                for kt, p in zip(range(4 * cp, 4 * cp + 4), ps):
                    o = _dot(_halves(vt[gp, _rows(hp, DH // 2), _rows(kt)]), p)
                    acc = o if acc is None else acc + o
                if cp == nchunk - 1:
                    inv = pl.reciprocal(jnp.sum(den, axis=0, keepdims=True))
                    ot[blkp % NT, gp, _rows(hp, DH // 2), :] = _words(acc * inv)
            if scores:
                m_next = jnp.max(top, axis=0, keepdims=True)
        return m, m_next, den, acc

    def full_layer(rep):
        lax.fori_loop(0, NG, full_qkv, None)

        items = HEADS * NT
        head = ATT_UNROLL // 2
        state = full_att(0, head, (None,) * 4, first=True)
        state = lax.fori_loop(
            0, items // ATT_UNROLL - 1,
            lambda j, st: full_att(head // 4 + j * (ATT_UNROLL // 4), ATT_UNROLL, st), state)
        full_att((items - ATT_UNROLL + head) // 4, ATT_UNROLL - head, state, last=True)

        def proj(c, _):
            stage = xio.at[c].bitcast(u32)
            for tp in range(NT // 2):
                bits = []
                for t in (2 * tp, 2 * tp + 1):
                    y = xb[t, c] + _dot(_halves(wot[c]), _halves(ot[t].reshape(D // 2, 128)))
                    xa[t, c] = y
                    bits.append(lax.bitcast_convert_type(y.astype(bf16).astype(f32), u32))
                stage[pl.ds(tp, 128, stride=NT // 2), :] = ((bits[0] >> 16) | bits[1]).T
                if tp == 0:
                    i = jnp.minimum(c, 2)
                    for s in transpose_steps(wqa, i, wj0, i):
                        s()

            @pl.when(rep == 1)
            def _():
                out_copy(c, pl.ds(pl.multiple_of(c * 128, 128), 128)).start()

        lax.fori_loop(0, NG, proj, None)

    for c in range(NG):
        x_copy(c).start()
    for cp in wqa_copies(0):
        cp.start()
    for c in range(NG):
        x_copy(c).wait()
        if c == NG - 1:
            for g in range(1, NG):
                for cp in wqa_copies(g):
                    cp.start()
            for cp in late_copies():
                cp.start()
        stage = xio.at[c].bitcast(u32)
        for tp in range(NT // 2):
            pair = stage[pl.ds(tp, 128, stride=NT // 2), :].T
            xa[2 * tp, c] = lax.bitcast_convert_type(pair << 16, f32)
            xa[2 * tp + 1, c] = lax.bitcast_convert_type((pair >> 16) << 16, f32)
    for cp in wqa_copies(0):
        cp.wait()
    for s in local_w_steps(0, 0):
        s()

    def two_layers(rep, _):
        local_layer(rep)
        full_layer(rep)

    lax.fori_loop(0, 2, two_layers, None)
    for c in range(NG):
        out_copy(c, _rows(c)).wait()


@jax.jit
def pallas_interleave_layers__sliding_local_dilated__softmax_full_mha__prompt_kernel(
    A_x: jax.Array,
    A_wqkv: jax.Array,
    A_wo: jax.Array,
    B_x: jax.Array,
    B_wqkv: jax.Array,
    B_wo: jax.Array,
):
    del B_x
    assert A_x.shape == (1, SEQ, D) and A_x.dtype == bf16
    vmem = pltpu.VMEM
    tile = (128, 128)
    scratch = [
        vmem((NG, SEQ, 128), bf16),
        vmem((3 * NG, D, 128), bf16), vmem((NG, D, 128), bf16),
        vmem((3 * NG, D, 128), bf16), vmem((NG, D, 128), bf16),
        vmem((3, 64, D), u32), vmem((3, 64, D), u32),
        vmem((NG, 64, D), u32), vmem((3 * NG, 64, D), u32),
        vmem((NT, NG) + tile, f32), vmem((NT, NG) + tile, f32),
        vmem((NT, D // 2, 128), u32), vmem((NT, NG, 64, 128), u32),
        vmem((WIN,) + tile, f32), vmem((WIN,) + tile, f32),
        *[vmem((2 * WIN - 1,) + tile, f32) for _ in range(4)],
        vmem((NG,) + tile, f32), vmem((NG,) + tile, f32),
        vmem((NG * NT, 64, 128), u32), vmem((NG, SEQ // 2, 128), u32),
        vmem((NG, 64, SEQ), u32),
        vmem((SEQ, 128), f32), vmem((SEQ, 128), f32),
        pltpu.SemaphoreType.DMA((NG,)), pltpu.SemaphoreType.DMA((NG + 1,)),
        pltpu.SemaphoreType.DMA((NG,)),
    ]
    hbm = pl.BlockSpec(memory_space=pl.ANY)
    out = pl.pallas_call(
        _kernel,
        out_shape=jax.ShapeDtypeStruct((SEQ, D), bf16),
        in_specs=[hbm] * 5,
        out_specs=hbm,
        scratch_shapes=scratch,
        compiler_params=pltpu.CompilerParams(
            vmem_limit_bytes=110 * 1024 * 1024,
            flags={"XLA_TPU_FORCE_LP_LLO_SCHEDULER": True},
        ),
        name="interleaved_layers",
    )(A_x.reshape(SEQ, D), A_wqkv, A_wo, B_wqkv, B_wo)
    return out.reshape(1, SEQ, D)
```

```python
import math

import jax
import jax.numpy as jnp
from jax import lax
import jax.experimental.pallas as pl
import jax.experimental.pallas.tpu as pltpu

SEQ, D, HEADS, DH = 2048, 1024, 32, 32
WIN = 8
NT = SEQ // 128
NG = D // 128
EPS = 1e-5
LOG2E = math.log2(math.e)
QSCALE = DH ** -0.5 * LOG2E
MASKED = -1e9 * LOG2E
ATT_UNROLL = 16

bf16, f32, u32 = jnp.bfloat16, jnp.float32, jnp.uint32


def _words(x):
    return pltpu.bitcast(x.astype(bf16), u32)


def _halves(x):
    return pltpu.bitcast(x, bf16)


def _dot(a, b):
    return jnp.dot(a, b, preferred_element_type=f32)


def _fold(x, op, acc=None):
    for i in range(x.shape[0] // 8):
        slab = x[8 * i:8 * i + 8]
        acc = slab if acc is None else op(acc, slab)
    return acc


def _rows(i, n=128):
    return slice(i * n, (i + 1) * n)


def _after(x, dep):
    return x if dep is None else jnp.maximum(x, jnp.minimum(x, dep))


def _interleave(main, *sides):
    done = [0] * len(sides)
    prev = None
    for i, step in enumerate(main):
        y = step()
        for k, side in enumerate(sides):
            upto = (i + 1) * len(side) // len(main)
            for e, s in enumerate(side[done[k]:upto]):
                slab = e * 16 // (upto - done[k])
                s(None if prev is None else prev[8 * slab:8 * slab + 8])
            done[k] = upto
        prev = y


def _layernorm_steps(load, store):
    st = {}

    def mean(dep):
        acc = _after(jnp.zeros((8, 128), f32), dep)
        for c in range(NG):
            x = load(c, 0)
            acc = _fold(x[:64] + x[64:], jnp.add, acc)
        st["mean"] = jnp.broadcast_to(jnp.sum(acc, axis=0, keepdims=True) * (1.0 / D), (8, 128))

    def var(dep):
        mu = jnp.tile(st["mean"], (16, 1))
        acc = _after(jnp.zeros((8, 128), f32), dep)
        for c in range(NG):
            d = load(c, 1) - mu
            acc = _fold(d * d, jnp.add, acc)
        st["rstd"] = lax.rsqrt(jnp.sum(acc, axis=0, keepdims=True) * (1.0 / D) + EPS)

    def norm(dep):
        dep = _after(jnp.broadcast_to(st["rstd"], (8, 128)), dep)
        for c in range(NG):
            x = load(c, 2)
            hs = []
            for i in range(2):
                mu = jnp.tile(_after(st["mean"], dep), (8, 1))
                hs.append((x[_rows(i, 64)] - mu) * st["rstd"])
                dep = hs[-1][-8:]
            store(c, x, jnp.concatenate(hs, axis=0))

    return [mean, var, norm]


def _kernel(x_hbm, wqa_hbm, woa_hbm, wqb_hbm, wob_hbm, out_hbm,
            xio, wqa, woa, wqb, wob, wj0, wj1, wot, wqt,
            xa, xb, ht, ot, q0, q1, k0, k1, v0, v1, y0, y1,
            qt, kk, vt, s0, s1, zeros, x_sem, w_sem, o_sem):
    wj, qbuf, kbuf, vbuf, ybuf, sbuf = (wj0, wj1), (q0, q1), (k0, k1), (v0, v1), (y0, y1), (s0, s1)

    for i in range(WIN):
        zeros[i] = 0

    def x_copy(c):
        return pltpu.make_async_copy(x_hbm.at[:, _rows(c)], xio.at[c], x_sem.at[c])

    def out_copy(c, col):
        return pltpu.make_async_copy(xio.at[c], out_hbm.at[:, col], o_sem.at[c])

    def wqa_copies(g):
        return [pltpu.make_async_copy(wqa_hbm.at[:, _rows(i * NG + g)], wqa.at[3 * g + i],
                                      w_sem.at[g]) for i in range(3)]

    def late_copies():
        cps = [pltpu.make_async_copy(woa_hbm.at[:, _rows(c)], woa.at[c], w_sem.at[NG])
               for c in range(NG)]
        cps += [pltpu.make_async_copy(wqb_hbm.at[:, _rows(i * NG + g)], wqb.at[3 * g + i],
                                      w_sem.at[NG]) for g in range(NG) for i in range(3)]
        cps += [pltpu.make_async_copy(wob_hbm.at[:, _rows(c)], wob.at[c], w_sem.at[NG])
                for c in range(NG)]
        return cps

    def transpose_steps(src, i, dst, j):
        def step(k):
            def run(dep=None):
                for kt in (2 * k, 2 * k + 1):
                    dst[j, :, _rows(kt)] = pltpu.bitcast(src[i, _rows(kt), :].T, u32)
            return run
        return [step(k) for k in range(NG // 2)]

    def local_qkv_steps(unit, slot):
        par = unit // NG

        def step(r, i):
            def run():
                y = _dot(_halves(wj[slot][i]), _halves(ht[2 * r + par]))
                if i == 0:
                    qbuf[slot][r] = y * QSCALE
                    return y
                buf = kbuf[slot] if i == 1 else vbuf[slot]
                buf[r + WIN - 1] = y
                if r > 0:
                    buf[r - 1] = pltpu.roll(y, 1, 1)
                return y
            return run
        return [step(r, i) for r in range(WIN) for i in (1, 2, 0)]

    def local_att_steps(unit, slot):
        g, par = unit % NG, unit // NG

        def step(r, h):
            def run(dep):
                rows = _rows(h, DH)
                z = zeros[r]
                q = qbuf[slot][r + z, rows, :]
                q = jnp.concatenate([_after(q[:8], dep), q[8:]], axis=0)
                first = lax.broadcasted_iota(jnp.int32, (1, 128), 1) == 0
                logits = []
                for w in range(WIN):
                    l = _fold(q * kbuf[slot][r - w + WIN - 1 + z, rows, :], jnp.add)
                    l = jnp.sum(l, axis=0, keepdims=True)
                    logits.append(jnp.where(first, MASKED, l) if w > r else l)
                m = logits[0]
                for l in logits[1:]:
                    m = jnp.maximum(m, l)
                den = acc = None
                for w in range(WIN):
                    p = jnp.exp2(logits[w] - m)
                    pv = p * vbuf[slot][r - w + WIN - 1 + z, rows, :]
                    den = p if den is None else den + p
                    acc = pv if acc is None else acc + pv
                o = acc * pl.reciprocal(den)
                ot[2 * r + par, g, _rows(h, DH // 2), :] = _words(o)
            return run
        return [step(r, h) for h in range(4) for r in range(WIN)]

    def local_w_steps(unit, slot):
        g = unit % NG
        return [s for i in range(3) for s in transpose_steps(wqa, 3 * g + i, wj[slot], i)]

    def tile_ln_steps(t):
        def store(c, x, h):
            ht[t, _rows(c, 64), :] = _words(h)
        return _layernorm_steps(lambda c, i: xa[t + zeros[i], c], store)

    def proj_steps(t, slot):
        def step(c):
            def run():
                y = xa[t, c] + _dot(_halves(wot[c]), _halves(ot[t].reshape(D // 2, 128)))
                ybuf[slot][c] = y
                return y
            return run
        return [step(c) for c in range(NG)]

    def proj_ln_steps(t, slot):
        def store(c, x, h):
            xb[t, c] = x
            ht[t, _rows(c, 64), :] = _words(h)
        return _layernorm_steps(lambda c, i: ybuf[slot][c + zeros[i]], store)

    def local_layer(rep):
        def wait_w(g):
            @pl.when(rep == 0)
            def _():
                pltpu.make_async_copy(wqa.at[pl.ds(0, 3)], wqa.at[pl.ds(0, 3)], w_sem.at[g]).wait()

        wait_w(1)
        ln = [tile_ln_steps(t) for t in list(range(0, NT, 2)) + list(range(1, NT, 2))]
        for s in ln[0] + ln[1]:
            s(None)
        _interleave(local_qkv_steps(0, 0),
                    [s for r in range(WIN - 1) for e in (r + 2, WIN + 1 + r) for s in ln[e]]
                    + [lambda dep: None] * 6,
                    local_w_steps(1, 1))

        def unit_pair(j, _):
            @pl.when(j < NG // 2 - 1)
            def _():
                wait_w(2 * j + 2)
                wait_w(2 * j + 3)

            for u, slot in ((2 * j + 1, 1), (2 * j + 2, 0)):
                _interleave(local_qkv_steps(u, slot),
                            local_att_steps(u - 1, 1 - slot), local_w_steps(u + 1, 1 - slot))

        lax.fori_loop(0, NG - 1, unit_pair, None)

        @pl.when(rep == 0)
        def _():
            for cp in late_copies():
                cp.wait()

        last = 2 * NG - 1
        _interleave(local_qkv_steps(last, 1),
                    local_att_steps(last - 1, 0),
                    [s for c in range(NG) for s in transpose_steps(woa, c, wot, c)])

        _interleave(proj_steps(0, 0) + proj_steps(2, 1), local_att_steps(last, 1))

        def tile(i):
            return 2 * (i % WIN) + i // WIN

        for s in proj_ln_steps(0, 0):
            s(None)

        def tile_pair(j, _):
            for i, slot in ((2 * j + 2, 0), (2 * j + 3, 1)):
                cols = [jnp.minimum(2 * i - 4 + e, 3 * NG - 1) for e in range(2)]
                _interleave(proj_steps(tile(i), slot),
                            proj_ln_steps(tile(i - 1), 1 - slot) + [lambda dep: None],
                            [s for c in cols for s in transpose_steps(wqb, c, wqt, c)])

        lax.fori_loop(0, NT // 2 - 1, tile_pair, None)
        for s in proj_ln_steps(NT - 1, 1):
            s(None)

    def full_qkv(g, _):
        def step(t, i):
            def run():
                y = _dot(_halves(wqt[3 * g + i]), _halves(ht[t]))
                if i == 0:
                    qt[g * NT + t] = _words(y * QSCALE)
                elif i == 1:
                    kk[g, _rows(t, 64), :] = pltpu.bitcast(y.astype(bf16).T, u32)
                else:
                    vt[g, :, _rows(t)] = _words(y)
                return y
            return run
        _interleave([step(t, i) for i in (1, 0, 2) for t in range(NT)],
                    transpose_steps(wob, g, wot, g))

    chunk = 512
    nchunk = SEQ // chunk

    def full_att(base, count, state, first=False, last=False):
        m, m_next, den, acc = state
        for u in range(count + (2 if last else 0)):
            scores = u < count
            if scores:
                blk = base + u // 4
                h = u % 4
                parts = [jnp.zeros((DH // 2, 128), u32)] * 4
                parts[h] = qt[blk, _rows(h, DH // 2), :]
                q = _halves(jnp.concatenate(parts, axis=0))
                top = None
            for c in range(nchunk):
                if scores:
                    for kt in range(4 * c, 4 * c + 4):
                        s = _dot(_halves(kk[blk // NT, _rows(kt, 64), :]), q)
                        sbuf[u % 2][_rows(kt), :] = s
                        top = _fold(s, jnp.maximum, top)
                up, cp = divmod((u - 1) * nchunk + c - 1, nchunk)
                if (first and up < 0) or up >= count:
                    continue
                if cp == 0:
                    m, den, acc = m_next, None, None
                blkp = base + up // 4
                gp, hp = blkp // NT, up % 4
                ps = []
                for kt in range(4 * cp, 4 * cp + 4):
                    p = jnp.exp2(sbuf[up % 2][_rows(kt), :] - m)
                    den = _fold(p, jnp.add, den)
                    ps.append(p.astype(bf16))
                for kt, p in zip(range(4 * cp, 4 * cp + 4), ps):
                    o = _dot(_halves(vt[gp, _rows(hp, DH // 2), _rows(kt)]), p)
                    acc = o if acc is None else acc + o
                if cp == nchunk - 1:
                    inv = pl.reciprocal(jnp.sum(den, axis=0, keepdims=True))
                    ot[blkp % NT, gp, _rows(hp, DH // 2), :] = _words(acc * inv)
            if scores:
                m_next = jnp.max(top, axis=0, keepdims=True)
        return m, m_next, den, acc

    def full_layer(rep):
        lax.fori_loop(0, NG, full_qkv, None)

        items = HEADS * NT
        head = ATT_UNROLL // 2
        state = full_att(0, head, (None,) * 4, first=True)
        state = lax.fori_loop(
            0, items // ATT_UNROLL - 1,
            lambda j, st: full_att(head // 4 + j * (ATT_UNROLL // 4), ATT_UNROLL, st), state)
        full_att((items - ATT_UNROLL + head) // 4, ATT_UNROLL - head, state, last=True)

        def proj(c, _):
            stage = xio.at[c].bitcast(u32)
            for tp in range(NT // 2):
                bits = []
                for t in (2 * tp, 2 * tp + 1):
                    y = xb[t, c] + _dot(_halves(wot[c]), _halves(ot[t].reshape(D // 2, 128)))
                    xa[t, c] = y
                    bits.append(lax.bitcast_convert_type(y.astype(bf16).astype(f32), u32))
                stage[pl.ds(tp, 128, stride=NT // 2), :] = ((bits[0] >> 16) | bits[1]).T
                if tp == 0:
                    i = jnp.minimum(c, 2)
                    for s in transpose_steps(wqa, i, wj0, i):
                        s()

            @pl.when(rep == 1)
            def _():
                out_copy(c, pl.ds(pl.multiple_of(c * 128, 128), 128)).start()

        lax.fori_loop(0, NG, proj, None)

    for c in range(NG):
        x_copy(c).start()
    for cp in wqa_copies(0):
        cp.start()
    for c in range(NG):
        x_copy(c).wait()
        if c == NG - 1:
            for g in range(1, NG):
                for cp in wqa_copies(g):
                    cp.start()
            for cp in late_copies():
                cp.start()
        stage = xio.at[c].bitcast(u32)
        for tp in range(NT // 2):
            pair = stage[pl.ds(tp, 128, stride=NT // 2), :].T
            xa[2 * tp, c] = lax.bitcast_convert_type(pair << 16, f32)
            xa[2 * tp + 1, c] = lax.bitcast_convert_type((pair >> 16) << 16, f32)
    for cp in wqa_copies(0):
        cp.wait()
    for s in local_w_steps(0, 0):
        s()

    def two_layers(rep, _):
        local_layer(rep)
        full_layer(rep)

    lax.fori_loop(0, 2, two_layers, None)
    for c in range(NG):
        out_copy(c, _rows(c)).wait()


@jax.jit
def pallas_interleave_layers__sliding_local_dilated__softmax_full_mha__prompt_kernel(
    A_x: jax.Array,
    A_wqkv: jax.Array,
    A_wo: jax.Array,
    B_x: jax.Array,
    B_wqkv: jax.Array,
    B_wo: jax.Array,
):
    del B_x
    assert A_x.shape == (1, SEQ, D) and A_x.dtype == bf16
    vmem = pltpu.VMEM
    tile = (128, 128)
    scratch = [
        vmem((NG, SEQ, 128), bf16),
        vmem((3 * NG, D, 128), bf16), vmem((NG, D, 128), bf16),
        vmem((3 * NG, D, 128), bf16), vmem((NG, D, 128), bf16),
        vmem((3, 64, D), u32), vmem((3, 64, D), u32),
        vmem((NG, 64, D), u32), vmem((3 * NG, 64, D), u32),
        vmem((NT, NG) + tile, f32), vmem((NT, NG) + tile, f32),
        vmem((NT, D // 2, 128), u32), vmem((NT, NG, 64, 128), u32),
        vmem((WIN,) + tile, f32), vmem((WIN,) + tile, f32),
        *[vmem((2 * WIN - 1,) + tile, f32) for _ in range(4)],
        vmem((NG,) + tile, f32), vmem((NG,) + tile, f32),
        vmem((NG * NT, 64, 128), u32), vmem((NG, SEQ // 2, 128), u32),
        vmem((NG, 64, SEQ), u32),
        vmem((SEQ, 128), f32), vmem((SEQ, 128), f32),
        pltpu.SMEM((WIN,), jnp.int32),
        pltpu.SemaphoreType.DMA((NG,)), pltpu.SemaphoreType.DMA((NG + 1,)),
        pltpu.SemaphoreType.DMA((NG,)),
    ]
    hbm = pl.BlockSpec(memory_space=pl.ANY)
    out = pl.pallas_call(
        _kernel,
        out_shape=jax.ShapeDtypeStruct((SEQ, D), bf16),
        in_specs=[hbm] * 5,
        out_specs=hbm,
        scratch_shapes=scratch,
        compiler_params=pltpu.CompilerParams(
            vmem_limit_bytes=110 * 1024 * 1024,
            flags={"XLA_TPU_FORCE_LP_LLO_SCHEDULER": True},
        ),
        name="interleaved_layers",
    )(A_x.reshape(SEQ, D), A_wqkv, A_wo, B_wqkv, B_wo)
    return out.reshape(1, SEQ, D)
```

```python
import math

import jax
import jax.numpy as jnp
from jax import lax
import jax.experimental.pallas as pl
import jax.experimental.pallas.tpu as pltpu

SEQ, D, HEADS, DH = 2048, 1024, 32, 32
WIN = 8
NT = SEQ // 128
NP = NT // 2
NG = D // 128
EPS = 1e-5
LOG2E = math.log2(math.e)
QSCALE = DH ** -0.5 * LOG2E
MASKED = -1e9 * LOG2E
ATT_UNROLL = 16
DELAY = 2
PHASES = 'abcd'
GROUPW = 2
GROUPV = 2

bf16, f32, u32, i32 = jnp.bfloat16, jnp.float32, jnp.uint32, jnp.int32


def _words(ref, *idx, block=0, rows=None):
    rows = rows or ref.shape[-2]
    return ref.bitcast(i32)[(*idx, _rows(block, rows // 2), slice(None))]


def _load(ref, *idx, **block):
    return pltpu.bitcast(_words(ref, *idx, **block), bf16)


def _dot(a, b):
    return jnp.dot(a, b, preferred_element_type=f32)


def _fold(x, op, acc=None):
    for i in range(x.shape[0] // 8):
        slab = x[8 * i:8 * i + 8]
        acc = slab if acc is None else op(acc, slab)
    return acc


def _rows(i, n=128):
    return slice(i * n, (i + 1) * n)


def _after(x, dep):
    return x if dep is None else jnp.maximum(x, jnp.minimum(x, dep))


def _left_operands(a11, a12, a21, a22):
    f11, f12, f21, f22 = (a.astype(f32) for a in (a11, a12, a21, a22))
    return [f21 + f22, a22, f11 + f22, f12 - f22, f21 - f11, f11 + f12, a11]


def _right_operands(b11, b12, b21, b22):
    return [b11, b21 - b11, b11 - b22, b21 - b22, b11 - b12, b22, b12 - b22]


def _project(w, i, h, j):
    ms = [_dot(jnp.concatenate([_load(w, i, e, block=k, rows=64) for k in range(4)], axis=1),
               _load(h, j, e)) for e in range(7)]
    m2, m4, m1, m7, m6, m5, m3 = ms
    y1 = jnp.concatenate([m4 + m1 + m7 + m5, m2 + m4], axis=0)
    y2 = jnp.concatenate([m5 + m3, m2 - m1 - m6 + m3], axis=0)
    return (y1, y2), [m[:8] for m in ms]


def _interleave(main, *sides):
    done = [0] * len(sides)
    marks = [None] * DELAY
    for i, step in enumerate(main):
        marks += step()
        total = (len(marks) - DELAY) * len(main) // (i + 1)
        for k, side in enumerate(sides):
            upto = (i + 1) * len(side) // len(main)
            for e in range(done[k], upto):
                side[e](marks[e * total // len(side)])
            done[k] = upto


def _layernorm_steps(load, store):
    mean, rstd = [None] * 2, [None] * 2

    def mean_step(n):
        def run(dep):
            acc = _after(jnp.zeros((8, 128), f32), dep) if n == 0 else _after(
                jnp.zeros((8, 128), f32), _after(mean[0], dep))
            for c in range(NG):
                x = load(n, c, 0)
                acc = _fold(x[:64] + x[64:], jnp.add, acc)
            mean[n] = jnp.broadcast_to(jnp.sum(acc, axis=0, keepdims=True) * (1.0 / D), (8, 128))
        return run

    def var_step(n):
        def run(dep):
            mu = jnp.tile(mean[n], (16, 1))
            acc = _after(jnp.zeros((8, 128), f32), _after(mean[1] if n == 0 else rstd[0], dep))
            for c in range(NG):
                d = load(n, c, 1) - mu
                acc = _fold(d * d, jnp.add, acc)
            r = lax.rsqrt(jnp.sum(acc, axis=0, keepdims=True) * (1.0 / D) + EPS)
            rstd[n] = jnp.broadcast_to(r, (8, 128))
        return run

    last = [None]

    def norm_step(c0, c1):
        def run(dep):
            dep = _after(rstd[1] if c0 == 0 else last[0], dep)
            for c in range(c0, c1):
                x = [load(n, c, 2) for n in range(2)]
                ops = []
                for i in range(4):
                    mu = [jnp.tile(_after(mean[n], dep), (2, 1)) for n in range(2)]
                    b = [(x[n][_rows(4 * e + i, 16)] - mu[n]) * jnp.tile(rstd[n], (2, 1))
                         for e in range(2) for n in range(2)]
                    ops.append(_right_operands(*b))
                    dep = ops[-1][-1][:8]
                store(c, x, [jnp.concatenate(o, axis=0) for o in zip(*ops)])
            last[0] = dep
        return run

    return [mean_step(0), mean_step(1), var_step(0), var_step(1),
            norm_step(0, NG // 2), norm_step(NG // 2, NG)]


def _kernel(x_hbm, wqa_hbm, woa_hbm, wqb_hbm, wob_hbm, out_hbm,
            xio, wa, wb, wj, wot, wqt,
            xa, xb, ht, ot, q0, q1, k0, k1, v0, v1, y0, y1,
            qt, kk, vt, s0, s1, oq, zeros, x_sem, w_sem, o_sem):
    qbuf, kbuf, vbuf, ybuf, sbuf = (q0, q1), (k0, k1), (v0, v1), (y0, y1), (s0, s1)

    for i in range(WIN):
        zeros[i] = 0

    def x_copy(c):
        return pltpu.make_async_copy(x_hbm.at[:, _rows(c)], xio.at[c], x_sem.at[c])

    def out_copy(c, col):
        return pltpu.make_async_copy(xio.at[c], out_hbm.at[:, col], o_sem.at[c])

    def w_copies(qkv_hbm, o_hbm, dst, g, sem):
        srcs = [qkv_hbm.at[:, _rows(i * NG + g)] for i in range(3)] + [o_hbm.at[:, _rows(g)]]
        return [pltpu.make_async_copy(src, dst.at[4 * g + i], sem) for i, src in enumerate(srcs)]

    def local_copies(g):
        return w_copies(wqa_hbm, woa_hbm, wa, g, w_sem.at[g])

    def full_copies():
        return [cp for g in range(NG) for cp in w_copies(wqb_hbm, wob_hbm, wb, g, w_sem.at[NG])]

    def weight_steps(src, i, dst, j):
        def step(k):
            def run(dep=None):
                w = [_words(src, i, block=4 * k + e, rows=64) for e in range(4)]
                if dep is not None:
                    dep = lax.bitcast_convert_type(dep, i32)
                    w[0] = jnp.concatenate([_after(w[0][:8], dep), w[0][8:]], axis=0)
                t1, t2 = (pltpu.bitcast(jnp.concatenate(w[e::2], axis=0), bf16).T for e in range(2))
                for e, a in enumerate(_left_operands(t1[:64], t2[:64], t1[64:], t2[64:])):
                    if a.dtype == bf16:
                        dst.bitcast(i32)[j, e, _rows(k, 32), :] = pltpu.bitcast(a, i32)
                    else:
                        dst[j, e, _rows(k, 64), :] = a.astype(bf16)
            return run
        return [step(k) for k in range(NG // 2)]

    def store_head(j, g, n, h, o):
        i = n + h // 2 * 2
        if i < 3:
            oq[i] = o
            return
        rows = pl.ds(pl.multiple_of((2 * g + h % 2) * DH, DH), DH)
        for e, b in enumerate(_right_operands(*[oq[i + zeros[0]] for i in range(3)], o)):
            ot[j, e, rows, :] = b.astype(bf16)

    def local_tile(j, n):
        return 4 * (j % (NP // 2)) + 2 * n + j // (NP // 2)

    def local_qkv_steps(par):
        def step(j, i):
            def run():
                ys, marks = _project(wj, i, ht, par * (NP // 2) + j)
                for r, y in zip((2 * j, 2 * j + 1), ys):
                    if i == 0:
                        qbuf[par][r] = y * QSCALE
                        continue
                    buf = kbuf[par] if i == 1 else vbuf[par]
                    buf[r + WIN - 1] = y
                    if r > 0:
                        buf[r - 1] = pltpu.roll(y, 1, 1)
                return marks
            return run
        return [step(j, i) for i in (1, 2, 0) for j in range(NP // 2)]

    def local_att_steps(g, par):
        def step(r, h):
            def run(dep):
                rows = _rows(h, DH)
                z = zeros[r]
                q = qbuf[par][r + z, rows, :]
                first = lax.broadcasted_iota(jnp.int32, (1, 128), 1) == 0
                logits = []
                for w in range(WIN):
                    if w % GROUPW == 0:
                        qw = jnp.concatenate([_after(q[:8], dep), q[8:]], axis=0)
                    dep = _fold(qw * kbuf[par][r - w + WIN - 1 + z, rows, :], jnp.add)
                    l = jnp.sum(dep, axis=0, keepdims=True)
                    logits.append(jnp.where(first, MASKED, l) if w > r else l)
                m = logits[0]
                for l in logits[1:]:
                    m = jnp.maximum(m, l)
                den = acc = None
                for w in range(WIN):
                    p = jnp.exp2(logits[w] - m)
                    if w and w % GROUPV == 0:
                        p = _after(p, acc[:1])
                    pv = p * vbuf[par][r - w + WIN - 1 + z, rows, :]
                    den = p if den is None else den + p
                    acc = pv if acc is None else acc + pv
                store_head(par * (NP // 2) + r // 2, g, r % 2, h, acc * pl.reciprocal(den))
            return run
        return [step(2 * j + n, h + 2 * e)
                for j in range(NP // 2) for h in range(2) for e in range(2) for n in range(2)]

    def store_normed(j, c, ops):
        for e, b in enumerate(ops):
            ht[j, e, _rows(c, 64), :] = b.astype(bf16)

    def input_ln_steps(j):
        return _layernorm_steps(lambda n, c, i: xa[local_tile(j, n) + zeros[i], c],
                                lambda c, x, ops: store_normed(j, c, ops))

    def proj_steps(j, slot):
        def step(c):
            def run():
                ys, marks = _project(wot, c, ot, j)
                for n in range(2):
                    ybuf[slot][n, c] = xa[local_tile(j, n), c] + ys[n]
                return marks
            return run
        return [step(c) for c in range(NG)]

    def proj_ln_steps(j, slot):
        def store(c, x, ops):
            for n in range(2):
                xb[local_tile(j, n), c] = x[n]
            store_normed(j, c, ops)
        return _layernorm_steps(lambda n, c, i: ybuf[slot][n + zeros[i], c], store)

    def local_layer(rep):
        idle = lambda dep: None

        def wait_weights(g):
            @pl.when(jnp.logical_and(rep == 0, g < NG))
            def _():
                pltpu.make_async_copy(wa.at[pl.ds(0, 4)], wa.at[pl.ds(0, 4)], w_sem.at[g]).wait()

        def w_steps(g):
            nxt = 4 * ((g + 1) % NG)
            return (weight_steps(wa, 4 * g, wj, 0) + [idle] * 4 + weight_steps(wa, 4 * g + 3, wot, g)
                    + [idle] * 4 + weight_steps(wa, nxt + 1, wj, 1) + weight_steps(wa, nxt + 2, wj, 2))

        if 'a' in PHASES:
            wait_weights(1)
            ln = [input_ln_steps(j) for j in range(NP)]
            for s in ln[0]:
                s(None)
            for s in w_steps(0)[:4]:
                s(None)
            even = local_qkv_steps(0)
            _interleave([even[4 * i + j] for j in range(NP // 2) for i in range(3)],
                        [s for j in range(1, NP) for s in ln[j]] + [idle] * 2)
            _interleave(local_qkv_steps(1), local_att_steps(0, 0), w_steps(0)[8:12] + w_steps(0)[16:])

        def group(g, _):
            wait_weights(g + 1)
            _interleave(local_qkv_steps(0) + local_qkv_steps(1),
                        local_att_steps(g - 1, 1) + local_att_steps(g, 0), w_steps(g))

        if 'b' in PHASES:
            lax.fori_loop(1, NG, group, None)

        @pl.when(rep == 0)
        def _():
            for cp in full_copies():
                cp.wait()

        def full_w_steps(g):
            return [s for i in range(3) for s in weight_steps(wb, 4 * g + i, wqt, 3 * g + i)]

        if 'c' not in PHASES:
            proj_steps(0, 0)[0]()
            xb[0] = y0[0]
            return
        _interleave(proj_steps(0, 0), local_att_steps(NG - 1, 1))
        _interleave(proj_steps(1, 1), proj_ln_steps(0, 0) + [idle], full_w_steps(0) + full_w_steps(1))

        def two_pairs(i, _):
            j = 2 * i + 2
            _interleave(proj_steps(j, 0) + proj_steps(j + 1, 1),
                        proj_ln_steps(j - 1, 1) + [idle] * 2 + proj_ln_steps(j, 0) + [idle],
                        full_w_steps(j) + full_w_steps(j + 1) + [idle])

        lax.fori_loop(0, NP // 2 - 1, two_pairs, None)
        for s in proj_ln_steps(NP - 1, 1):
            s(None)

    def full_qkv(g, _):
        def step(j, i):
            def run():
                ys, marks = _project(wqt, 3 * g + i, ht, j)
                for n, y in enumerate(ys):
                    t = local_tile(j, n)
                    if i == 0:
                        qt[g * NT + t] = (y * QSCALE).astype(bf16)
                    elif i == 1:
                        kk.bitcast(i32)[g, t] = pltpu.bitcast(y.astype(bf16).T, i32)
                    else:
                        vt[g, t] = y.astype(bf16)
                return marks
            return run
        _interleave([step(j, i) for i in (1, 0, 2) for j in range(NP)],
                    weight_steps(wb, 4 * g + 3, wot, g))

    chunk = 512
    nchunk = SEQ // chunk

    def full_att(base, count, state, first=False, last=False):
        def item(u):
            return base + u // 8, u % 2, u % 8 // 4 + 2 * (u % 4 // 2)

        m, m_next, den, acc = state
        for u in range(count + (2 if last else 0)):
            scores = u < count
            if scores:
                blk, n, h = item(u)
                parts = [jnp.zeros((DH // 2, 128), i32)] * 4
                parts[h] = _words(qt, 2 * blk + n, block=h, rows=DH)
                q = pltpu.bitcast(jnp.concatenate(parts, axis=0), bf16)
                top = None
            for c in range(nchunk):
                if scores:
                    for kt in range(4 * c, 4 * c + 4):
                        s = _dot(_load(kk, blk // NP, kt), q)
                        sbuf[u % 2][_rows(kt), :] = s
                        top = _fold(s, jnp.maximum, top)
                up, cp = divmod((u - 1) * nchunk + c - 1, nchunk)
                if (first and up < 0) or up >= count:
                    continue
                if cp == 0:
                    m, den, acc = m_next, None, None
                blkp, np_, hp = item(up)
                ps = []
                for kt in range(4 * cp, 4 * cp + 4):
                    p = jnp.exp2(sbuf[up % 2][_rows(kt), :] - m)
                    den = _fold(p, jnp.add, den)
                    ps.append(p.astype(bf16))
                for kt, p in zip(range(4 * cp, 4 * cp + 4), ps):
                    o = _dot(_load(vt, blkp // NP, kt, block=hp, rows=DH), p)
                    acc = o if acc is None else acc + o
                if cp == nchunk - 1:
                    o = acc * pl.reciprocal(jnp.sum(den, axis=0, keepdims=True))
                    store_head(blkp % NP, blkp // NP, np_, hp, o)
            if scores:
                m_next = jnp.max(top, axis=0, keepdims=True)
        return m, m_next, den, acc

    def full_layer(rep):
        if 'c' in PHASES:
            lax.fori_loop(0, NG, full_qkv, None)

        items = HEADS * NT
        head = ATT_UNROLL // 2
        if 'd' in PHASES:
            state = full_att(0, head, (None,) * 4, first=True)
            state = lax.fori_loop(
                0, items // ATT_UNROLL - 1,
                lambda j, st: full_att(head // 8 + j * (ATT_UNROLL // 8), ATT_UNROLL, st), state)
            full_att((items - ATT_UNROLL + head) // 8, ATT_UNROLL - head, state, last=True)
        elif 'c' in PHASES:
            full_att(0, 4, (None,) * 4, first=True, last=True)

        def proj(c, _):
            stage = xio.at[c].bitcast(u32)
            for j in range(NP):
                ys, marks = _project(wot, c, ot, j)
                bits = []
                for n in range(2):
                    y = xb[2 * j + n, c] + ys[n]
                    xa[2 * j + n, c] = y
                    bits.append(lax.bitcast_convert_type(y.astype(bf16).astype(f32), u32))
                stage[pl.ds(j, 128, stride=NP), :] = ((bits[0] >> 16) | bits[1]).T

            @pl.when(rep == 1)
            def _():
                out_copy(c, pl.ds(pl.multiple_of(c * 128, 128), 128)).start()

        lax.fori_loop(0, NG, proj, None)

    for c in range(NG):
        x_copy(c).start()
    for cp in local_copies(0):
        cp.start()
    for c in range(NG):
        x_copy(c).wait()
        if c == NG - 1:
            for g in range(1, NG):
                for cp in local_copies(g):
                    cp.start()
            for cp in full_copies():
                cp.start()
        stage = xio.at[c].bitcast(u32)
        for j in range(NP):
            pair = stage[pl.ds(j, 128, stride=NP), :].T
            xa[2 * j, c] = lax.bitcast_convert_type(pair << 16, f32)
            xa[2 * j + 1, c] = lax.bitcast_convert_type((pair >> 16) << 16, f32)
    for cp in local_copies(0):
        cp.wait()
    for s in weight_steps(wa, 1, wj, 1) + weight_steps(wa, 2, wj, 2):
        s()

    def two_layers(rep, _):
        local_layer(rep)
        full_layer(rep)

    lax.fori_loop(0, 2, two_layers, None)
    for c in range(NG):
        out_copy(c, _rows(c)).wait()


@jax.jit
def pallas_interleave_layers__sliding_local_dilated__softmax_full_mha__prompt_kernel(
    A_x: jax.Array,
    A_wqkv: jax.Array,
    A_wo: jax.Array,
    B_x: jax.Array,
    B_wqkv: jax.Array,
    B_wo: jax.Array,
):
    del B_x
    assert A_x.shape == (1, SEQ, D) and A_x.dtype == bf16
    vmem = pltpu.VMEM
    tile = (128, 128)
    left, right = (7, D // 4, 128), (7, D // 2, 128)
    scratch = [
        vmem((NG, SEQ, 128), bf16),
        vmem((4 * NG, D, 128), bf16), vmem((4 * NG, D, 128), bf16),
        vmem((3,) + left, bf16),
        vmem((NG,) + left, bf16), vmem((3 * NG,) + left, bf16),
        vmem((NT, NG) + tile, f32), vmem((NT, NG) + tile, f32),
        vmem((NP,) + right, bf16), vmem((NP,) + right, bf16),
        vmem((WIN,) + tile, f32), vmem((WIN,) + tile, f32),
        *[vmem((2 * WIN - 1,) + tile, f32) for _ in range(4)],
        vmem((2, NG) + tile, f32), vmem((2, NG) + tile, f32),
        vmem((NG * NT,) + tile, bf16), vmem((NG, NT) + tile, bf16),
        vmem((NG, NT) + tile, bf16),
        vmem((SEQ, 128), f32), vmem((SEQ, 128), f32),
        vmem((3, DH, 128), f32),
        pltpu.SMEM((WIN,), jnp.int32),
        pltpu.SemaphoreType.DMA((NG,)), pltpu.SemaphoreType.DMA((NG + 1,)),
        pltpu.SemaphoreType.DMA((NG,)),
    ]
    hbm = pl.BlockSpec(memory_space=pl.ANY)
    out = pl.pallas_call(
        _kernel,
        out_shape=jax.ShapeDtypeStruct((SEQ, D), bf16),
        in_specs=[hbm] * 5,
        out_specs=hbm,
        scratch_shapes=scratch,
        compiler_params=pltpu.CompilerParams(
            vmem_limit_bytes=110 * 1024 * 1024,
            flags={"XLA_TPU_FORCE_LP_LLO_SCHEDULER": True},
        ),
        name="interleaved_layers",
    )(A_x.reshape(SEQ, D), A_wqkv, A_wo, B_wqkv, B_wo)
    return out.reshape(1, SEQ, D)
```

```python
import math

import jax
import jax.numpy as jnp
from jax import lax
import jax.experimental.pallas as pl
import jax.experimental.pallas.tpu as pltpu

SEQ, D, HEADS, DH = 2048, 1024, 32, 32
WIN = 8
NT = SEQ // 128
NP = NT // 2
NG = D // 128
EPS = 1e-5
LOG2E = math.log2(math.e)
QSCALE = DH ** -0.5 * LOG2E
MASKED = -1e9 * LOG2E
ATT_UNROLL = 32
DELAY = 16
OUT_UNROLL = 2
PHASES = 'abcd'
SCOPES = False
import contextlib
def scope(n):
    return jax.named_scope(n) if SCOPES else contextlib.nullcontext()
GROUPW = 2
GROUPV = 2

bf16, f32, u32, i32 = jnp.bfloat16, jnp.float32, jnp.uint32, jnp.int32


def _words(ref, *idx, block=0, rows=None):
    rows = rows or ref.shape[-2]
    return ref.bitcast(i32)[(*idx, _rows(block, rows // 2), slice(None))]


def _load(ref, *idx, **block):
    return pltpu.bitcast(_words(ref, *idx, **block), bf16)


def _dot(a, b):
    return jnp.dot(a, b, preferred_element_type=f32)


def _fold(x, op, acc=None):
    for i in range(x.shape[0] // 8):
        slab = x[8 * i:8 * i + 8]
        acc = slab if acc is None else op(acc, slab)
    return acc


def _rows(i, n=128):
    return slice(i * n, (i + 1) * n)


def _after(x, dep):
    return x if dep is None else jnp.maximum(x, jnp.minimum(x, dep))


def _left_operands(a11, a12, a21, a22):
    f11, f12, f21, f22 = (a.astype(f32) for a in (a11, a12, a21, a22))
    return [f21 + f22, a22, f11 + f22, f12 - f22, f21 - f11, f11 + f12, a11]


def _right_operands(b11, b12, b21, b22):
    return [b11, b21 - b11, b11 - b22, b21 - b22, b11 - b12, b22, b12 - b22]


def _project(w, i, h, j):
    ms = [_dot(jnp.concatenate([_load(w, i, e, block=k, rows=64) for k in range(4)], axis=1),
               _load(h, j, e)) for e in range(7)]
    m2, m4, m1, m7, m6, m5, m3 = ms
    y1 = jnp.concatenate([m4 + m1 + m7 + m5, m2 + m4], axis=0)
    y2 = jnp.concatenate([m5 + m3, m2 - m1 - m6 + m3], axis=0)
    return (y1, y2), [(m, i) for m in ms for i in range(8)]


def _interleave(main, *sides, marks=None):
    done = [0] * len(sides)
    marks = marks or [None] * DELAY
    for i, step in enumerate(main):
        marks += step()
        total = (len(marks) - DELAY) * len(main) // (i + 1)
        for k, side in enumerate(sides):
            upto = (i + 1) * len(side) // len(main)
            for e in range(done[k], upto):
                if side[e] is not None:
                    mark = marks[e * total // len(side)]
                    side[e](mark and mark[0][_rows(mark[1], 8)])
            done[k] = upto
    return marks[-DELAY:]


def _moments(x):
    mean = _fold(x, jnp.add) * (1.0 / 16)
    d = x - jnp.tile(mean, (16, 1))
    return jnp.concatenate([mean, _fold(d * d, jnp.add)], axis=0)


def _layernorm_steps(moments, load, store):
    mean, rstd, last = [], [], []

    def stats(n):
        def run(dep):
            part = moments(n)
            means = [part[i, :8] for i in range(NG)]
            mu = _after(means[0], dep)
            for m in means[1:]:
                mu = mu + m
            mu = jnp.sum(mu, axis=0, keepdims=True) * (16.0 / D)
            dev = sq = None
            for i, m in enumerate(means):
                d = m - mu
                dev = d * d if dev is None else dev + d * d
                sq = part[i, 8:] if sq is None else sq + part[i, 8:]
            var = jnp.sum(sq + 16.0 * dev, axis=0, keepdims=True) * (1.0 / D)
            mean.append(jnp.broadcast_to(mu, (8, 128)))
            rstd.append(jnp.broadcast_to(lax.rsqrt(var + EPS), (16, 128)))
            last[:] = [rstd[-1][:8]]
        return run

    def step(c, i):
        def run(dep):
            dep = last[0] if dep is None else jnp.minimum(dep, last[0])
            mu = [jnp.tile(_after(mean[n], dep), (2, 1)) for n in range(2)]
            ops = _right_operands(*[(load(n, c, _rows(4 * e + i, 16)) - mu[n]) * rstd[n]
                                    for e in range(2) for n in range(2)])
            store(_rows(4 * c + i, 16), ops)
            last[:] = [ops[2][:8]]
        return run

    return [stats(0), stats(1), None] + [step(c, i) for c in range(NG) for i in range(4)]


def _kernel(x_hbm, wqa_hbm, woa_hbm, wqb_hbm, wob_hbm, out_hbm,
            xio, wa, wb, wj, wot, wqt,
            xa, xb, ht, ot, q0, q1, k0, k1, v0, v1, y0, y1, ma, m0, m1,
            qt, kk, vt, s0, s1, oq, zeros, x_sem, w_sem, o_sem):
    qbuf, kbuf, vbuf, ybuf, sbuf = (q0, q1), (k0, k1), (v0, v1), (y0, y1), (s0, s1)
    mbuf = (m0, m1)

    for i in range(WIN):
        zeros[i] = 0

    def x_copy(c):
        return pltpu.make_async_copy(x_hbm.at[:, _rows(c)], xio.at[c], x_sem.at[c])

    def out_copy(c, col):
        return pltpu.make_async_copy(xio.at[c], out_hbm.at[:, col], o_sem.at[c])

    def w_copies(qkv_hbm, o_hbm, dst, g, sem):
        def cols(i):
            return pl.ds(pl.multiple_of((i * NG + g) * 128, 128), 128)
        srcs = [qkv_hbm.at[:, cols(i)] for i in range(3)] + [o_hbm.at[:, cols(0)]]
        return [pltpu.make_async_copy(src, dst.at[4 * g + i], sem) for i, src in enumerate(srcs)]

    def local_copies(g):
        return w_copies(wqa_hbm, woa_hbm, wa, g, w_sem.at[g])

    def full_copies(g):
        return w_copies(wqb_hbm, wob_hbm, wb, g, w_sem.at[NG])

    def weight_steps(src, i, dst, j):
        def step(k):
            def run(dep=None):
                w = [_words(src, i, block=4 * k + e, rows=64) for e in range(4)]
                if dep is not None:
                    dep = lax.bitcast_convert_type(dep, i32)
                    w[0] = jnp.concatenate([_after(w[0][:8], dep), w[0][8:]], axis=0)
                t1, t2 = (pltpu.bitcast(jnp.concatenate(w[e::2], axis=0), bf16).T for e in range(2))
                for e, a in enumerate(_left_operands(t1[:64], t2[:64], t1[64:], t2[64:])):
                    if a.dtype == bf16:
                        dst.bitcast(i32)[j, e, _rows(k, 32), :] = pltpu.bitcast(a, i32)
                    else:
                        dst[j, e, _rows(k, 64), :] = a.astype(bf16)
            return run
        return [step(k) for k in range(NG // 2)]

    def store_head(j, g, n, h, o):
        i = n + h // 2 * 2
        if i < 3:
            oq[i] = o
            return
        rows = pl.ds(pl.multiple_of((2 * g + h % 2) * DH, DH), DH)
        for e, b in enumerate(_right_operands(*[oq[i + zeros[0]] for i in range(3)], o)):
            ot[j, e, rows, :] = b.astype(bf16)

    def local_tile(j, n):
        return 4 * (j % (NP // 2)) + 2 * n + j // (NP // 2)

    def local_qkv_steps(par):
        def step(j, i):
            def run():
                ys, marks = _project(wj, i, ht, par * (NP // 2) + j)
                for r, y in zip((2 * j, 2 * j + 1), ys):
                    if i == 0:
                        qbuf[par][r] = y * QSCALE
                        continue
                    buf = kbuf[par] if i == 1 else vbuf[par]
                    buf[r + WIN - 1] = y
                    if r > 0:
                        buf[r - 1] = pltpu.roll(y, 1, 1)
                return marks
            return run
        return [step(j, i) for i in (1, 2, 0) for j in range(NP // 2)]

    def local_att_steps(g, par):
        def step(r, h):
            def run(dep):
                rows = _rows(h, DH)
                z = zeros[r]
                q = qbuf[par][r + z, rows, :]
                first = lax.broadcasted_iota(jnp.int32, (1, 128), 1) == 0
                logits = []
                for w in range(WIN):
                    if w % GROUPW == 0:
                        qw = jnp.concatenate([_after(q[:8], dep), q[8:]], axis=0)
                    dep = _fold(qw * kbuf[par][r - w + WIN - 1 + z, rows, :], jnp.add)
                    l = jnp.sum(dep, axis=0, keepdims=True)
                    logits.append(jnp.where(first, MASKED, l) if w > r else l)
                m = logits[0]
                for l in logits[1:]:
                    m = jnp.maximum(m, l)
                den = acc = None
                for w in range(WIN):
                    p = jnp.exp2(logits[w] - m)
                    if w and w % GROUPV == 0:
                        p = _after(p, acc[:1])
                    pv = p * vbuf[par][r - w + WIN - 1 + z, rows, :]
                    den = p if den is None else den + p
                    acc = pv if acc is None else acc + pv
                store_head(par * (NP // 2) + r // 2, g, r % 2, h, acc * pl.reciprocal(den))
            return run
        return [step(2 * j + n, h + 2 * e)
                for j in range(NP // 2) for h in range(2) for e in range(2) for n in range(2)]

    def store_normed(j):
        def run(rows, ops):
            for e, b in enumerate(ops):
                ht[j, e, rows, :] = b.astype(bf16)
        return run

    def input_ln_steps(j):
        return _layernorm_steps(lambda n: ma[local_tile(j, n)],
                                lambda n, c, rows: xa[local_tile(j, n), c, rows, :],
                                store_normed(j))

    def proj_steps(j, slot):
        def step(c):
            def run():
                ys, marks = _project(wot, c, ot, j)
                for n in range(2):
                    y = xa[local_tile(j, n), c] + ys[n]
                    xb[local_tile(j, n), c] = y
                    ybuf[slot][n, c] = y
                    mbuf[slot][n, c] = _moments(y)
                return marks
            return run
        return [step(c) for c in range(NG)]

    def proj_ln_steps(j, slot):
        z = zeros[0]
        return _layernorm_steps(lambda n: mbuf[slot][n + z],
                                lambda n, c, rows: ybuf[slot][n + z, c, rows, :],
                                store_normed(j))

    def local_layer(rep):
        idle = None

        def fetch_weights(g):
            @pl.when(rep == 0)
            def _():
                @pl.when(g + 1 < NG)
                def _():
                    for cp in local_copies(g + 1):
                        cp.wait()

                @pl.when(g + 2 < NG)
                def _():
                    for cp in local_copies(g + 2):
                        cp.start()

                for cp in full_copies(g):
                    cp.start()

        def w_steps(g):
            nxt = 4 * ((g + 1) % NG)
            return (weight_steps(wa, 4 * g, wj, 0) + [idle] * 4 + weight_steps(wa, 4 * g + 3, wot, g)
                    + [idle] * 4 + weight_steps(wa, nxt + 1, wj, 1) + weight_steps(wa, nxt + 2, wj, 2))

        if 'a' in PHASES:
          with scope('A0'):
            ln = [input_ln_steps(j) for j in range(NP)]
            for s in ln[0]:
                s and s(None)
            even, odd = local_qkv_steps(0), local_qkv_steps(1)
            marks = _interleave(even[0:8:4], [idle] * 6 + ln[1] + [idle] * 10, w_steps(0)[:2])
            marks = _interleave(even[1:8:4], ln[2] + [idle] * 10, w_steps(0)[2:4], marks=marks)
            marks = _interleave(even[2:8:4] + even[8:9], ln[3] + ln[4], marks=marks)
            _interleave(even[3:8:4] + even[9:], ln[5] + ln[6] + ln[7], marks=marks)
            fetch_weights(0)
            _interleave(odd, local_att_steps(0, 0), w_steps(0)[8:12] + w_steps(0)[16:])

        def group(g, _):
            fetch_weights(g)
            _interleave(local_qkv_steps(0) + local_qkv_steps(1),
                        local_att_steps(g - 1, 1) + local_att_steps(g, 0), w_steps(g))

        if 'b' in PHASES:
          with scope('A1'):
            lax.fori_loop(1, NG, group, None)

        @pl.when(rep == 0)
        def _():
            pltpu.make_async_copy(wb, wb, w_sem.at[NG]).wait()

        def full_w_steps(g):
            return [s for i in range(3) for s in weight_steps(wb, 4 * g + i, wqt, 3 * g + i)]

        if 'c' not in PHASES:
            proj_steps(0, 0)[0]()
            return
        _interleave(proj_steps(0, 0) + proj_steps(1, 1),
                    local_att_steps(NG - 1, 1) + [idle] * 8,
                    [idle] * 41 + proj_ln_steps(0, 0),
                    full_w_steps(0) + full_w_steps(1) + [idle])

        def two_pairs(i, _):
            j = 2 * i + 2
            _interleave(proj_steps(j, 0) + proj_steps(j + 1, 1),
                        proj_ln_steps(j - 1, 1) + [idle] * 6 + proj_ln_steps(j, 0),
                        full_w_steps(j) + full_w_steps(j + 1) + [idle])

        with scope('A2'):
            lax.fori_loop(0, NP // 2 - 1, two_pairs, None)
        for s in proj_ln_steps(NP - 1, 1):
            s and s(None)

    def full_qkv(g, _):
        def step(j, i):
            def run():
                ys, marks = _project(wqt, 3 * g + i, ht, j)
                for n, y in enumerate(ys):
                    t = local_tile(j, n)
                    if i == 0:
                        qt[g * NT + t] = (y * QSCALE).astype(bf16)
                    elif i == 1:
                        kk.bitcast(i32)[g, t] = pltpu.bitcast(y.astype(bf16).T, i32)
                    else:
                        vt[g, t] = y.astype(bf16)
                return marks
            return run
        _interleave([step(j, i) for i in (1, 0, 2) for j in range(NP)],
                    weight_steps(wb, 4 * g + 3, wot, g))

    chunk = 512
    nchunk = SEQ // chunk

    def full_att(base, count, state, first=False, last=False):
        def item(u):
            return base + u // 8, u % 2, u % 8 // 4 + 2 * (u % 4 // 2)

        m, m_next, den, acc = state
        for u in range(count + (2 if last else 0)):
            scores = u < count
            if scores:
                blk, n, h = item(u)
                parts = [jnp.zeros((DH // 2, 128), i32)] * 4
                parts[h] = _words(qt, 2 * blk + n, block=h, rows=DH)
                q = pltpu.bitcast(jnp.concatenate(parts, axis=0), bf16)
                top = None
            for c in range(nchunk):
                if scores:
                    for kt in range(4 * c, 4 * c + 4):
                        s = _dot(_load(kk, blk // NP, kt), q)
                        sbuf[u % 2][_rows(kt), :] = s
                        top = _fold(s, jnp.maximum, top)
                up, cp = divmod((u - 1) * nchunk + c - 1, nchunk)
                if (first and up < 0) or up >= count:
                    continue
                if cp == 0:
                    m, den, acc = m_next, None, None
                blkp, np_, hp = item(up)
                ps = []
                for kt in range(4 * cp, 4 * cp + 4):
                    p = jnp.exp2(sbuf[up % 2][_rows(kt), :] - m)
                    den = _fold(p, jnp.add, den)
                    ps.append(p.astype(bf16))
                for kt, p in zip(range(4 * cp, 4 * cp + 4), ps):
                    o = _dot(_load(vt, blkp // NP, kt, block=hp, rows=DH), p)
                    acc = o if acc is None else acc + o
                if cp == nchunk - 1:
                    o = acc * pl.reciprocal(jnp.sum(den, axis=0, keepdims=True))
                    store_head(blkp % NP, blkp // NP, np_, hp, o)
            if scores:
                m_next = jnp.max(top, axis=0, keepdims=True)
        return m, m_next, den, acc

    def full_layer(rep):
        if 'c' in PHASES:
          with scope('B1'):
            lax.fori_loop(0, NG, full_qkv, None)

        items = HEADS * NT
        head = ATT_UNROLL // 2
        if 'd' in PHASES:
          with scope('B2'):
            state = full_att(0, head, (None,) * 4, first=True)
            state = lax.fori_loop(
                0, items // ATT_UNROLL - 1,
                lambda j, st: full_att(head // 8 + j * (ATT_UNROLL // 8), ATT_UNROLL, st), state)
            full_att((items - ATT_UNROLL + head) // 8, ATT_UNROLL - head, state, last=True)
        elif 'c' in PHASES:
            full_att(0, 4, (None,) * 4, first=True, last=True)

        def proj(i, _):
            cols = [OUT_UNROLL * i + e for e in range(OUT_UNROLL)]
            for c in cols:
                stage = xio.at[c].bitcast(u32)
                for j in range(NP):
                    ys, _ = _project(wot, c, ot, j)
                    bits = []
                    for n in range(2):
                        y = xb[2 * j + n, c] + ys[n]
                        xa[2 * j + n, c] = y
                        ma[2 * j + n, c] = _moments(y)
                        bits.append(lax.bitcast_convert_type(y.astype(bf16).astype(f32), u32))
                    stage[pl.ds(j, 128, stride=NP), :] = ((bits[0] >> 16) | bits[1]).T

            @pl.when(rep == 1)
            def _():
                for c in cols:
                    out_copy(c, pl.ds(pl.multiple_of(c * 128, 128), 128)).start()

        with scope('B3'):
            lax.fori_loop(0, NG // OUT_UNROLL, proj, None)

    for c in range(NG):
        x_copy(c).start()
    for cp in local_copies(0):
        cp.start()
    for c in range(NG):
        with scope(f'xw{c}'):
            x_copy(c).wait()
        if c == NG - 1:
            for cp in local_copies(1):
                cp.start()
        stage = xio.at[c].bitcast(u32)
        for j in range(NP):
            pair = stage[pl.ds(j, 128, stride=NP), :].T
            for n, bits in enumerate((pair << 16, (pair >> 16) << 16)):
                y = lax.bitcast_convert_type(bits, f32)
                xa[2 * j + n, c] = y
                ma[2 * j + n, c] = _moments(y)
    for cp in local_copies(0):
        cp.wait()
    for s in weight_steps(wa, 1, wj, 1) + weight_steps(wa, 2, wj, 2):
        s()

    def two_layers(rep, _):
        local_layer(rep)
        full_layer(rep)

    with scope('main'):
        lax.fori_loop(0, 2, two_layers, None)
    with scope('tail'):
      for c in range(NG):
        out_copy(c, _rows(c)).wait()


@jax.jit
def pallas_interleave_layers__sliding_local_dilated__softmax_full_mha__prompt_kernel(
    A_x: jax.Array,
    A_wqkv: jax.Array,
    A_wo: jax.Array,
    B_x: jax.Array,
    B_wqkv: jax.Array,
    B_wo: jax.Array,
):
    del B_x
    assert A_x.shape == (1, SEQ, D) and A_x.dtype == bf16
    vmem = pltpu.VMEM
    tile = (128, 128)
    left, right = (7, D // 4, 128), (7, D // 2, 128)
    scratch = [
        vmem((NG, SEQ, 128), bf16),
        vmem((4 * NG, D, 128), bf16), vmem((4 * NG, D, 128), bf16),
        vmem((3,) + left, bf16),
        vmem((NG,) + left, bf16), vmem((3 * NG,) + left, bf16),
        vmem((NT, NG) + tile, f32), vmem((NT, NG) + tile, f32),
        vmem((NP,) + right, bf16), vmem((NP,) + right, bf16),
        vmem((WIN,) + tile, f32), vmem((WIN,) + tile, f32),
        *[vmem((2 * WIN - 1,) + tile, f32) for _ in range(4)],
        vmem((2, NG) + tile, f32), vmem((2, NG) + tile, f32),
        vmem((NT, NG, 16, 128), f32),
        vmem((2, NG, 16, 128), f32), vmem((2, NG, 16, 128), f32),
        vmem((NG * NT,) + tile, bf16), vmem((NG, NT) + tile, bf16),
        vmem((NG, NT) + tile, bf16),
        vmem((SEQ, 128), f32), vmem((SEQ, 128), f32),
        vmem((3, DH, 128), f32),
        pltpu.SMEM((WIN,), jnp.int32),
        pltpu.SemaphoreType.DMA((NG,)), pltpu.SemaphoreType.DMA((NG + 1,)),
        pltpu.SemaphoreType.DMA((NG,)),
    ]
    hbm = pl.BlockSpec(memory_space=pl.ANY)
    out = pl.pallas_call(
        _kernel,
        out_shape=jax.ShapeDtypeStruct((SEQ, D), bf16),
        in_specs=[hbm] * 5,
        out_specs=hbm,
        scratch_shapes=scratch,
        compiler_params=pltpu.CompilerParams(
            vmem_limit_bytes=110 * 1024 * 1024,
            disable_bounds_checks=True,
            flags={"XLA_TPU_FORCE_LP_LLO_SCHEDULER": True},
        ),
        name="interleaved_layers",
    )(A_x.reshape(SEQ, D), A_wqkv, A_wo, B_wqkv, B_wo)
    return out.reshape(1, SEQ, D)
```

```python
import math

import jax
import jax.numpy as jnp
from jax import lax
import jax.experimental.pallas as pl
import jax.experimental.pallas.tpu as pltpu

SEQ, D, HEADS, DH = 2048, 1024, 32, 32
WIN = 8
NT = SEQ // 128
NP = NT // 2
NG = D // 128
EPS = 1e-5
LOG2E = math.log2(math.e)
QSCALE = DH ** -0.5 * LOG2E
MASKED = -1e9 * LOG2E
ATT_UNROLL = 32
VPU_TILES = 4
DELAY = 16
PHASES = 'abcd'
SCOPES = False
import contextlib
def scope(n):
    return jax.named_scope(n) if SCOPES else contextlib.nullcontext()

bf16, f32, i32 = jnp.bfloat16, jnp.float32, jnp.int32


def _rows(i, n=128):
    return slice(i * n, (i + 1) * n)


def _words(x):
    return pltpu.bitcast(x.astype(bf16), i32)


def _halves(x):
    return pltpu.bitcast(x, bf16)


def _put(ref, idx, block, x):
    x = x.astype(bf16) if ref.dtype == bf16 else _words(x)
    n = x.shape[0]
    ref[(*idx, pl.ds(pl.multiple_of(block * n, n), n), slice(None))] = x


def _get(ref, *idx):
    return ref[idx] if ref.dtype == bf16 else _halves(ref[idx])


def _dot(a, b):
    return jnp.dot(a, b, preferred_element_type=f32)


def _slab_sum(x, acc=None):
    x = x if acc is None else jnp.concatenate([acc, x], axis=0)
    return jnp.sum(x.reshape(-1, 8, x.shape[1]), axis=0)


def _slab_max(x, acc=None):
    x = x if acc is None else jnp.concatenate([acc, x], axis=0)
    return jnp.max(x.reshape(-1, 8, x.shape[1]), axis=0)


def _inverse(x):
    r = pl.reciprocal(x, approx=True)
    return r * (2.0 - x * r)


def _after(x, *deps):
    low = x
    for dep in deps:
        if dep is not None:
            low = jnp.minimum(low, lax.bitcast_convert_type(dep, x.dtype))
    return x if low is x else jnp.maximum(x, low)


def _head_after(x, n, *deps):
    return jnp.concatenate([_after(x[:n], *deps), x[n:]], axis=0)


def _slab(mark):
    return mark and mark[0][_rows(mark[1], 8)]


def _left_operands(a11, a12, a21, a22):
    f11, f12, f21, f22 = (a.astype(f32) for a in (a11, a12, a21, a22))
    return [f21 + f22, a22, f11 + f22, f12 - f22, f21 - f11, f11 + f12, a11]


def _right_operands(b11, b12, b21, b22):
    return [b11, b21 - b11, b11 - b22, b21 - b22, b11 - b12, b22, b12 - b22]


def _project(w, i, h, j):
    ms = [_dot(jnp.concatenate(jnp.split(_get(w, i, e), 4), axis=1), _get(h, j, e))
          for e in range(7)]
    m2, m4, m1, m7, m6, m5, m3 = ms
    y1 = jnp.concatenate([m4 + m1 + m7 + m5, m2 + m4], axis=0)
    y2 = jnp.concatenate([m5 + m3, m2 - m1 - m6 + m3], axis=0)
    return (y1, y2), [(m, s) for m in ms for s in range(8)]


def _interleave(main, *sides, marks=None):
    done = [0] * len(sides)
    marks = marks or [None] * DELAY
    for i, step in enumerate(main):
        marks += step()
        total = (len(marks) - DELAY) * len(main) // (i + 1)
        for k, side in enumerate(sides):
            upto = (i + 1) * len(side) // len(main)
            for e in range(done[k], upto):
                if side[e] is not None:
                    side[e](_slab(marks[e * total // len(side)]))
            done[k] = upto
    return marks[-DELAY:]


def _run(steps):
    for step in steps:
        if step is not None:
            step(None)


def _moments(x):
    mean = _slab_sum(x) * (1.0 / 16)
    d = x - jnp.tile(mean, (16, 1))
    return jnp.concatenate([mean, _slab_sum(d * d)], axis=0)


def _layernorm_steps(moments, load, store):
    mean, rstd, last = [], [], []

    def stats(n):
        def run(dep):
            part = moments(n)
            mu = jnp.sum(_head_after(part[:, :8], 1, dep), axis=0)
            mu = jnp.sum(mu, axis=0, keepdims=True) * (16.0 / D)
            d = part[:, :8] - mu
            var = jnp.sum(part[:, 8:], axis=0) + 16.0 * jnp.sum(d * d, axis=0)
            var = jnp.sum(var, axis=0, keepdims=True) * (1.0 / D)
            mean.append(jnp.broadcast_to(mu, (8, 128)))
            rstd.append(jnp.broadcast_to(lax.rsqrt(var + EPS), (16, 128)))
            last[:] = [rstd[-1][:8]]
        return run

    def step(c, i):
        def run(dep):
            dep = last[0] if dep is None else jnp.minimum(dep, last[0])
            mu = [jnp.tile(_after(mean[n], dep), (2, 1)) for n in range(2)]
            ops = _right_operands(*[(load(n, c, _rows(4 * e + i, 16)) - mu[n]) * rstd[n]
                                    for e in range(2) for n in range(2)])
            store(4 * c + i, ops)
            last[:] = [ops[2][:8]]
        return run

    return [stats(0), stats(1), None] + [step(c, i) for c in range(NG) for i in range(4)]


def _kernel(x_hbm, wqa_hbm, woa_hbm, wqb_hbm, wob_hbm, out_hbm,
            xio, xw0, xw1, wa, wb, wj, wot, wqt, xa, xb, ht, ot,
            q0, q1, k0, k1, v0, v1, ol, y0, y1, ma, m0, m1,
            qt, kk, vt, kb, qb0, qb1, s0, s1, oq, x_sem, a_sem, b_sem, o_sem):
    xw, qbuf, kbuf, vbuf = (xw0, xw1), (q0, q1), (k0, k1), (v0, v1)
    ybuf, mbuf, qb, sbuf = (y0, y1), (m0, m1), (qb0, qb1), (s0, s1)

    zeros = []

    def cols(c):
        return pl.ds(pl.multiple_of(c * 128, 128), 128)

    def x_copy(c):
        return pltpu.make_async_copy(x_hbm.at[:, cols(c)], xio.at[c], x_sem.at[c])

    def out_copy(c):
        return pltpu.make_async_copy(xio.at[c], out_hbm.at[:, cols(c)], o_sem.at[c])

    def w_copies(qkv_hbm, o_hbm, dst, g, sem):
        srcs = [qkv_hbm.at[:, cols(i * NG + g)] for i in range(3)] + [o_hbm.at[:, cols(g)]]
        return [pltpu.make_async_copy(src, dst.at[4 * g + i], sem(i)) for i, src in enumerate(srcs)]

    def local_copies(g):
        return w_copies(wqa_hbm, woa_hbm, wa, g, lambda i: a_sem.at[4 * g + i])

    def full_copies(g):
        return w_copies(wqb_hbm, wob_hbm, wb, g, lambda i: b_sem)

    def unstage_steps(stage, c):
        def step(t):
            def run(dep):
                x = _after(stage[_rows(t, 32), :], None if dep is None else jnp.tile(dep, (4, 1)))
                xio[c, _rows(t, 64), :] = _halves(x)
            return run
        return [step(t) for t in range(2 * NT)]

    def weight_steps(src, i, dst, j):
        def step(k):
            def run(dep):
                w = [src[i, _rows(4 * k + e, 64), :] for e in range(4)]
                w[0] = _halves(_head_after(_words(w[0]), 8, dep))
                t1, t2 = (jnp.concatenate(w[e::2], axis=0).T for e in range(2))
                for e, a in enumerate(_left_operands(t1[:64], t2[:64], t1[64:], t2[64:])):
                    _put(dst, (j, e), k, a)
            return run
        return [step(k) for k in range(NG // 2)]

    def operand_store(dst, j):
        def run(block, ops):
            for e, b in enumerate(ops):
                _put(dst, (j, e), block, b)
        return run

    def local_tile(j, n):
        return 4 * (j & 3) + 2 * n + (j >> 2)

    def local_qkv_steps(par):
        def put(buf, i, y):
            for h in range(4):
                buf[i, pl.ds(h, DH, stride=4), :] = y[_rows(h, DH)]

        def step(j, i):
            def run():
                ys, marks = _project(wj, i, ht, par * (NP // 2) + j)
                for r, y in zip((2 * j, 2 * j + 1), ys):
                    if i == 0:
                        put(qbuf[par], r, y)
                        continue
                    buf = kbuf[par] if i == 1 else vbuf[par]
                    put(buf, r + WIN - 1, y)
                    if r > 0:
                        put(buf, r - 1, pltpu.roll(y, 1, 1))
                return marks
            return run
        return [step(j, i) for i in (1, 2, 0) for j in range(NP // 2)]

    def local_att_steps(g, par):
        def tile_steps(r):
            logits, probs = [], []

            def score(i):
                def run(dep):
                    q = _head_after(qbuf[par][r + zeros[i]], 8, dep, *logits[-1:])
                    for w in (i, i + 1):
                        s = _slab_sum(q * kbuf[par][r + w + zeros[r]])
                        logits.append(s + pltpu.roll(s, 4, 0))
                return run

            def softmax(dep):
                s = jnp.concatenate(logits, axis=0) * QSCALE
                if r < WIN - 1:
                    wrapped = 8 * (WIN - 1 - r)
                    first = lax.broadcasted_iota(i32, (wrapped, 128), 1) == 0
                    s = jnp.concatenate([jnp.where(first, MASKED, s[:wrapped]), s[wrapped:]], axis=0)
                s = s.reshape(WIN, 8, 128)
                p = jnp.exp2(s - jnp.max(s, axis=0))
                probs.append(p * _inverse(jnp.sum(p, axis=0)))

            def mix(i):
                def run(dep):
                    p = _head_after(probs[0], 1, dep)
                    v = vbuf[par][pl.ds(r + zeros[r], WIN), _rows(i, 16), :]
                    ol[r % 2, _rows(i, 16), :] = jnp.sum(jnp.concatenate([p, p], axis=1) * v, axis=0)
                return run

            return ([s for i in range(0, WIN, 2) for s in (score(i), None)] + [softmax, None]
                    + [mix(i) for i in range(8)])

        def operands(j, i):
            def run(dep):
                b = [ol[n + zeros[0], pl.ds(64 * (i % 2) + i // 2 + 2 * e, 16, stride=4), :]
                     for e in range(2) for n in range(2)]
                for e in (0, 3):
                    b[e] = _head_after(b[e], 8, dep)
                operand_store(ot, par * (NP // 2) + j)(4 * g + i, _right_operands(*b))
            return run

        return [s for j in range(NP // 2) for s in tile_steps(2 * j) + tile_steps(2 * j + 1)
                + [operands(j, i) for i in range(4)]]

    def input_ln_steps(j):
        return _layernorm_steps(lambda n: ma[local_tile(j, n)],
                                lambda n, c, rows: xa[local_tile(j, n), c, rows, :],
                                operand_store(ht, j))

    def proj_steps(j, slot):
        def step(c):
            def run():
                ys, marks = _project(wot, c, ot, j)
                for n in range(2):
                    y = xa[local_tile(j, n), c] + ys[n]
                    xb[local_tile(j, n), c] = y
                    ybuf[slot][n, c] = y
                    mbuf[slot][n, c] = _moments(y)
                return marks
            return run
        return [step(c) for c in range(NG)]

    def proj_ln_steps(j, slot):
        return _layernorm_steps(lambda n: mbuf[slot][n + zeros[0]],
                                lambda n, c, rows: ybuf[slot][n + zeros[0], c, rows, :],
                                operand_store(ht, j))

    def local_layer(rep):
        def fetch_weights(g):
            @pl.when(rep == 0)
            def _():
                @pl.when(g + 1 < NG)
                def _():
                    for cp in local_copies(g + 1):
                        cp.wait()

                @pl.when(g + 2 < NG)
                def _():
                    for cp in local_copies(g + 2):
                        cp.start()

                for cp in full_copies(g):
                    cp.start()

        def w_steps(g):
            nxt = 4 * ((g + 1) & (NG - 1))
            return (weight_steps(wa, 4 * g, wj, 0) + [None] * 4
                    + weight_steps(wa, 4 * g + 3, wot, g) + [None] * 4
                    + weight_steps(wa, nxt + 1, wj, 1) + weight_steps(wa, nxt + 2, wj, 2))

        if 'a' in PHASES:
          with scope('A0'):
            ln = [input_ln_steps(j) for j in range(NP)]
            even, odd, first = local_qkv_steps(0), local_qkv_steps(1), w_steps(0)
            _run(ln[0])
            marks = _interleave(even[0:8:4], [None] * 6 + ln[1] + [None] * 10, first[:2])
            marks = _interleave(even[1:8:4], ln[2] + [None] * 10, first[2:4], marks=marks)
            marks = _interleave(even[2:8:4] + even[8:9], ln[3] + ln[4], marks=marks)
            _interleave(even[3:8:4] + even[9:], ln[5] + ln[6] + ln[7], marks=marks)
            fetch_weights(0)
            _interleave(odd, local_att_steps(0, 0), first[8:12] + first[16:])

        def group(g, _):
            fetch_weights(g)
            _interleave(local_qkv_steps(0) + local_qkv_steps(1),
                        local_att_steps(g - 1, 1) + local_att_steps(g, 0), w_steps(g))

        if 'b' in PHASES:
          with scope('A1'):
            lax.fori_loop(1, NG, group, None)

        @pl.when(rep == 0)
        def _():
            pltpu.make_async_copy(wb, wb, b_sem).wait()

        def full_w_steps(g):
            return [s for i in range(3) for s in weight_steps(wb, 4 * g + i, wqt, 3 * g + i)]

        if 'c' not in PHASES:
            proj_steps(0, 0)[0]()
            return
        _interleave(proj_steps(0, 0) + proj_steps(1, 1),
                    local_att_steps(NG - 1, 1) + [None] * 40,
                    [None] * 41 + proj_ln_steps(0, 0),
                    full_w_steps(0) + full_w_steps(1) + [None])

        def two_pairs(i, _):
            j = 2 * i + 2
            _interleave(proj_steps(j, 0) + proj_steps(j + 1, 1),
                        proj_ln_steps(j - 1, 1) + [None] * 6 + proj_ln_steps(j, 0),
                        full_w_steps(j) + full_w_steps(j + 1) + [None])

        with scope('A2'):
            lax.fori_loop(0, NP // 2 - 1, two_pairs, None)
        _run(proj_ln_steps(NP - 1, 1))

    def full_qkv(g, _):
        tails = {}

        def step(j, i):
            def run():
                ys, marks = _project(wqt, 3 * g + i, ht, j)
                for n, y in enumerate(ys):
                    t = local_tile(j, n)
                    if i == 0:
                        qt[g * NT + t] = _words(y * QSCALE)
                        xa[t, g] = y * QSCALE
                    elif i == 1:
                        k = y.astype(bf16).T
                        kk[g, 2 * j + n] = _words(k)
                        tails[2 * j + n] = k
                    else:
                        vt[g, 2 * j + n] = _words(y)
                return marks
            return run

        def spread(kt, e):
            def run(dep):
                k = _head_after(tails[kt][112:].astype(f32), 8, dep)
                for d in range(8 * e, 8 * e + 8):
                    kb[g, d, _rows(kt, 16), :] = jnp.broadcast_to(k[:, d:d + 1], (16, 128))
            return run

        _interleave([step(j, i) for i in (1, 0, 2) for j in range(NP)],
                    weight_steps(wb, 4 * g + 3, wot, g),
                    [None] * 8 + [spread(kt, e) for kt in range(VPU_TILES) for e in range(16)]
                    + [None] * 2)

    def full_att(base, count, state, first=False, last=False):
        def item(u):
            return base + u // 8, u % 2, u % 8 // 4 + 2 * (u % 4 // 2)

        m, m_next, den, acc = state
        marks = None
        for u in range(count + (2 if last else 0)):
            scores = u < count
            if scores:
                blk, n, h = item(u)
                parts = [jnp.zeros((DH // 2, 128), i32)] * 4
                parts[h] = qt[2 * blk + n, _rows(h, DH // 2), :]
                q = _halves(jnp.concatenate(parts, axis=0))
                for i in range(4):
                    rows = _after(xa[2 * (blk & 7) + n, blk >> 3, _rows(4 * h + i, 8), :],
                                  marks and _slab(marks[42 + 3 * i]))
                    for d in range(8):
                        qb[u % 2][8 * i + d] = jnp.broadcast_to(rows[d:d + 1], (8, 128))
                top, marks = None, []
            for c in range(4):
                if scores:
                    for kt in range(4 * c, 4 * c + 4):
                        keys = 112 if kt < VPU_TILES else 128
                        s = _dot(_halves(kk[blk >> 3, kt, :keys // 2, :]), q)
                        sbuf[u % 2][128 * kt:128 * kt + keys, :] = s
                        top = _slab_max(s, top)
                    marks += [(s, i) for i in range(14)]
                up, cp = divmod(4 * (u - 1) + c - 2, 4)
                if (first and up < 0) or up >= count:
                    continue
                if cp == 0:
                    m, den, acc = m_next, None, None
                blkp, _, hp = item(up)
                for kt in range(4 * cp, 4 * cp + 4):
                    p = jnp.exp2(sbuf[up % 2][_rows(kt), :] - m)
                    den = _slab_sum(p, den)
                    o = _dot(_halves(vt[blkp >> 3, kt, _rows(hp, DH // 2), :]), p)
                    acc = o if acc is None else acc + o
                if cp == 3:
                    o = acc * _inverse(jnp.sum(den, axis=0, keepdims=True))
                    if up % 4 < 3:
                        oq[up % 4] = o
                    else:
                        operand_store(ot, blkp & 7)(
                            2 * (blkp >> 3) + hp % 2,
                            _right_operands(*[oq[i + zeros[0]] for i in range(3)], o))
            if scores:
                s = None
                for e in range(2 * VPU_TILES):
                    qd = _head_after(qb[u % 2][pl.ds(zeros[e], DH)], 1, _slab(marks[7 * e]), s)
                    s = jnp.sum(kb[(blk >> 3) + zeros[u % 8], _rows(h, DH), _rows(e, 8), :] * qd,
                                axis=0)
                    sbuf[u % 2][pl.ds(128 * (e // 2) + 112 + 8 * (e % 2), 8), :] = s
                    top = jnp.maximum(top, s)
                m_next = jnp.max(top, axis=0, keepdims=True)
        return m, m_next, den, acc

    def full_layer(rep):
        if 'c' in PHASES or 'd' in PHASES:
          with scope('B1'):
            lax.fori_loop(0, NG, full_qkv, None)

        items = HEADS * NT
        head = ATT_UNROLL // 2
        if 'd' in PHASES:
          with scope('B2'):
            state = full_att(0, head, (None,) * 4, first=True)
            state = lax.fori_loop(
                0, items // ATT_UNROLL - 1,
                lambda j, st: full_att(head // 8 + j * (ATT_UNROLL // 8), ATT_UNROLL, st), state)
            full_att((items - ATT_UNROLL + head) // 8, ATT_UNROLL - head, state, last=True)
        elif 'c' in PHASES:
            full_att(0, 4, (None,) * 4, first=True, last=True)

        def proj(i, _):
            def step(c, j, stage):
                def run():
                    ys, marks = _project(wot, c, ot, j)
                    bits = []
                    for n in range(2):
                        y = xb[2 * j + n, c] + ys[n]
                        xa[2 * j + n, c] = y
                        ma[2 * j + n, c] = _moments(y)
                        bits.append(lax.bitcast_convert_type(y.astype(bf16).astype(f32), i32))
                    pair = lax.shift_right_logical(bits[0], 16) | bits[1]
                    stage[pl.ds(j, 128, stride=NP), :] = pair.T
                    return marks
                return run

            _interleave([step(2 * i + e, j, xw[e]) for e in range(2) for j in range(NP)],
                        [None] * 4 + unstage_steps(xw[1], jnp.maximum(2 * i - 1, 0)) + [None] * 44
                        + unstage_steps(xw[0], 2 * i) + [None] * 16)

            @pl.when(rep == 1)
            def _():
                @pl.when(i > 0)
                def _():
                    out_copy(2 * i - 1).start()

                out_copy(2 * i).start()

        with scope('B3'):
            lax.fori_loop(0, NG // 2, proj, None)

    first_w = local_copies(0)
    for cp in first_w[1:3] + [x_copy(0)]:
        cp.start()
    for i in (1, 2):
        with scope(f'ww{i}'):
            first_w[i].wait()
        x_copy(i).start()
        _run(weight_steps(wa, i, wj, i))

    def quarters(copy):
        lax.fori_loop(0, 4, lambda i, _: copy(pl.ds(pl.multiple_of(i * 512, 512), 512),
                                              pl.ds(pl.multiple_of(i * 256, 256), 256)), None)

    def stage_in(c, _):
        with scope('xw'):
            x_copy(c).wait()

        @pl.when(c + 3 < NG)
        def _():
            x_copy(c + 3).start()

        @pl.when(c + 2 == NG)
        def _():
            for cp in local_copies(0)[::3]:
                cp.start()

        @quarters
        def _(rows, words):
            xw[1][words, :] = _words(xio[c, rows, :])

        for j in range(NP):
            pair = xw[1][pl.ds(j, 128, stride=NP), :].T
            for n, bits in enumerate((pair << 16, pair & -65536)):
                y = lax.bitcast_convert_type(bits, f32)
                xa[2 * j + n, c] = y
                ma[2 * j + n, c] = _moments(y)

    with scope('stage'):
        lax.fori_loop(0, NG, stage_in, None)
    for cp in local_copies(1):
        cp.start()
    with scope('ww03'):
      for cp in first_w[::3]:
        cp.wait()

    def two_layers(rep, _):
        zeros[:] = [(rep + i) >> 4 for i in range(8)]
        local_layer(rep)
        full_layer(rep)

    with scope('main'):
        lax.fori_loop(0, 2, two_layers, None)

    @quarters
    def _(rows, words):
        xio[NG - 1, rows, :] = _halves(xw[1][words, :])

    out_copy(NG - 1).start()
    with scope('tail'):
      for c in range(NG):
        out_copy(c).wait()


@jax.jit
def pallas_interleave_layers__sliding_local_dilated__softmax_full_mha__prompt_kernel(
    A_x: jax.Array,
    A_wqkv: jax.Array,
    A_wo: jax.Array,
    B_x: jax.Array,
    B_wqkv: jax.Array,
    B_wo: jax.Array,
):
    del B_x
    assert A_x.shape == (1, SEQ, D) and A_x.dtype == bf16
    vmem, dma = pltpu.VMEM, pltpu.SemaphoreType.DMA
    tile, words = (128, 128), (64, 128)
    scratch = [
        vmem((NG, SEQ, 128), bf16),
        *[vmem((SEQ // 2, 128), i32)] * 2,
        *[vmem((4 * NG, D, 128), bf16)] * 2,
        vmem((3, 7, D // 8, 128), i32),
        vmem((NG, 7, D // 8, 128), i32),
        vmem((3 * NG, 7, D // 4, 128), bf16),
        *[vmem((NT, NG) + tile, f32)] * 2,
        *[vmem((NP, 7, D // 2, 128), bf16)] * 2,
        *[vmem((WIN,) + tile, f32)] * 2,
        *[vmem((2 * WIN - 1,) + tile, f32)] * 4,
        vmem((2,) + tile, f32),
        *[vmem((2, NG) + tile, f32)] * 2,
        vmem((NT, NG, 16, 128), f32),
        *[vmem((2, NG, 16, 128), f32)] * 2,
        vmem((NG * NT,) + words, i32),
        *[vmem((NG, NT) + words, i32)] * 2,
        vmem((NG, 128, 16 * VPU_TILES, 128), f32),
        *[vmem((DH, 8, 128), f32)] * 2,
        *[vmem((SEQ, 128), f32)] * 2,
        vmem((3, DH, 128), f32),
        dma((NG,)), dma((4 * NG,)), dma(()), dma((NG,)),
    ]
    hbm = pl.BlockSpec(memory_space=pl.ANY)
    out = pl.pallas_call(
        _kernel,
        out_shape=jax.ShapeDtypeStruct((SEQ, D), bf16),
        in_specs=[hbm] * 5,
        out_specs=hbm,
        scratch_shapes=scratch,
        compiler_params=pltpu.CompilerParams(
            vmem_limit_bytes=126 * 1024 * 1024,
            disable_bounds_checks=True,
            flags={"XLA_TPU_FORCE_LP_LLO_SCHEDULER": True},
        ),
        name="interleaved_layers",
    )(A_x.reshape(SEQ, D), A_wqkv, A_wo, B_wqkv, B_wo)
    return out.reshape(1, SEQ, D)
```

```python
import math

import jax
import jax.numpy as jnp
from jax import lax
import jax.experimental.pallas as pl
import jax.experimental.pallas.tpu as pltpu

SEQ, D, HEADS, DH = 2048, 1024, 32, 32
WIN = 8
NT = SEQ // 128
NP = NT // 2
NQ = NT // 4
NG = D // 128
EPS = 1e-5
LOG2E = math.log2(math.e)
QSCALE = DH ** -0.5 * LOG2E
MASKED = -1e9 * LOG2E
ATT_UNROLL = 32
VPU_TILES = 4
DELAY = 16
PHASES = 'abcdef'
SCOPES = False
import contextlib
def scope(n):
    return jax.named_scope(n) if SCOPES else contextlib.nullcontext()

bf16, f32, i32 = jnp.bfloat16, jnp.float32, jnp.int32


def _rows(i, n=128):
    return slice(i * n, (i + 1) * n)


def _words(x):
    return pltpu.bitcast(x.astype(bf16), i32)


def _halves(x):
    return pltpu.bitcast(x, bf16)


def _put(ref, idx, block, x):
    x = x.astype(bf16) if ref.dtype == bf16 else pltpu.bitcast(x.astype(bf16), ref.dtype)
    n = x.shape[0]
    ref[(*idx, pl.ds(pl.multiple_of(block * n, n), n), slice(None))] = x


def _get(ref, *idx):
    return ref[idx] if ref.dtype == bf16 else _halves(ref[idx])


def _dot(a, b):
    return jnp.dot(a, b, preferred_element_type=f32)


def _slab_sum(x, acc=None):
    x = x if acc is None else jnp.concatenate([acc, x], axis=0)
    return jnp.sum(x.reshape(-1, 8, x.shape[1]), axis=0)


def _slab_max(x, acc=None):
    x = x if acc is None else jnp.concatenate([acc, x], axis=0)
    return jnp.max(x.reshape(-1, 8, x.shape[1]), axis=0)


def _inverse(x):
    r = pl.reciprocal(x, approx=True)
    return r * (2.0 - x * r)


def _after(x, *deps):
    low = x
    for dep in deps:
        if dep is not None:
            low = jnp.minimum(low, lax.bitcast_convert_type(dep, x.dtype))
    return x if low is x else jnp.maximum(x, low)


def _head_after(x, n, *deps):
    return jnp.concatenate([_after(x[:n], *deps), x[n:]], axis=0)


def _slab(mark):
    return mark and mark[0][_rows(mark[1], 8)]


LEFT = [((1, 0), 1, (1, 1)), ((1, 1),), ((0, 0), 1, (1, 1)), ((1, 0), -1, (0, 0)),
        ((0, 0),), ((0, 0), 1, (0, 1)), ((0, 1), -1, (1, 1))]
RIGHT = [((0, 0),), ((1, 0), -1, (0, 0)), ((0, 0), -1, (1, 1)), ((0, 0), -1, (0, 1)),
         ((0, 1), -1, (1, 1)), ((1, 1),), ((1, 0), -1, (1, 1))]


def _operand(term, block):
    if len(term) == 1:
        return block(*term[0])
    a, b = block(*term[0]).astype(f32), block(*term[2]).astype(f32)
    return a + b if term[1] > 0 else a - b


def _operands(side, block):
    grid = [[block(r, c) for c in range(2)] for r in range(2)]
    return [_operand(term, lambda r, c: grid[r][c]) for term in side]


def _inner_operands(side, e, block):
    return _operands(side, lambda r, c: _operand(side[e], lambda i, j: block(2 * i + r, 2 * j + c)))


def _project(w, i, h, j, first=0):
    ms = []
    for e in range(first, first + 7):
        a, b = _get(w, i, e), _get(h, j, e)
        ms.append(_dot(jnp.concatenate(jnp.split(a, b.shape[0] // 128), axis=1), b))
    m2, m4, m1, m6, m3, m5, m7 = ms
    y1 = jnp.concatenate([m4 + m1 + m5 + m7, m2 + m4], axis=0)
    y2 = jnp.concatenate([m5 + m3, m2 - m1 - m6 + m3], axis=0)
    return (y1, y2), ms


def _marks(ms):
    return [(m, s) for m in ms for s in range(8)]


def _interleave(main, *sides, marks=None):
    done = [0] * len(sides)
    marks = marks or [None] * DELAY
    for i, step in enumerate(main):
        marks += step()
        total = (len(marks) - DELAY) * len(main) // (i + 1)
        for k, side in enumerate(sides):
            upto = (i + 1) * len(side) // len(main)
            for e in range(done[k], upto):
                if side[e] is not None:
                    side[e](_slab(marks[e * total // len(side)]))
            done[k] = upto
    return marks[-DELAY:]


def _run(steps):
    for step in steps:
        if step is not None:
            step(None)


def _moments(x):
    mean = _slab_sum(x) * (1.0 / 16)
    d = x - jnp.tile(mean, (16, 1))
    return jnp.concatenate([mean, _slab_sum(d * d)], axis=0)


def _layernorm_steps(tiles, moments, load, dst, j):
    mean, rstd, last = [], [], []

    def stats(n):
        def run(dep):
            part = moments(n)
            mu = jnp.sum(_head_after(part[:, :8], 1, dep), axis=0)
            mu = jnp.sum(mu, axis=0, keepdims=True) * (16.0 / D)
            d = part[:, :8] - mu
            var = jnp.sum(part[:, 8:], axis=0) + 16.0 * jnp.sum(d * d, axis=0)
            var = jnp.sum(var, axis=0, keepdims=True) * (1.0 / D)
            mean.append(jnp.broadcast_to(mu, (8, 128)))
            rstd.append(jnp.broadcast_to(lax.rsqrt(var + EPS), (16, 128)))
            last[:] = [rstd[-1][:8]]
        return run

    slabs = 8 // tiles

    def step(c, i, e):
        def run(dep):
            dep = last[0] if dep is None else jnp.minimum(dep, last[0])
            mu = [jnp.tile(_after(m, dep), (2, 1)) for m in mean]

            def block(k, n):
                return (load(n, c, _rows(slabs * k + i, 16), e) - mu[n]) * rstd[n]

            ops = _operands(RIGHT, block) if tiles == 2 else _inner_operands(RIGHT, e, block)
            for k, b in enumerate(ops):
                _put(dst, (j, 7 * e + k), slabs * c + i, b)
            last[:] = [ops[2][:8]]
        return run

    return [stats(n) for n in range(tiles)] + [None] + [
        step(c, i, e) for c in range(NG) for i in range(slabs)
        for e in range(1 if tiles == 2 else 7)]


def _kernel(x_hbm, wqa_hbm, woa_hbm, wqb_hbm, wob_hbm, out_hbm,
            xio, xw, wa, wb, wj, wot, wq2, wo2, wt, xa, xb, ha, oa, ho2,
            q0, q1, k0, k1, v0, v1, ol, y0, y1, ma, m0, m1,
            kk, vt, qb0, qb1, s0, s1, oq0, oq1, x_sem, a_sem, b_sem, o_sem, *sums):
    qbuf, kbuf, vbuf, oq = (q0, q1), (k0, k1), (v0, v1), (oq0, oq1)
    kb = (ha, oa)
    ybuf, mbuf, qb, sbuf = (y0, y1), (m0, m1), (qb0, qb1), (s0, s1)

    zeros, blocks = [], []

    def separately(body):
        blocks.append(body)
        pl.when(zeros[len(blocks)] == 0)(body)

    def cols(c):
        return pl.ds(pl.multiple_of(c * 128, 128), 128)

    def x_copy(c):
        return pltpu.make_async_copy(x_hbm.at[:, cols(c)], xio.at[c], x_sem.at[c])

    def out_copy(c):
        return pltpu.make_async_copy(xio.at[c], out_hbm.at[:, cols(c)], o_sem.at[c])

    def w_copies(qkv_hbm, o_hbm, dst, g, sem):
        srcs = [qkv_hbm.at[:, cols(i * NG + g)] for i in range(3)] + [o_hbm.at[:, cols(g)]]
        return [pltpu.make_async_copy(src, dst.at[4 * g + i], sem(i)) for i, src in enumerate(srcs)]

    def local_copies(g):
        return w_copies(wqa_hbm, woa_hbm, wa, g, lambda i: a_sem.at[4 * g + i])

    def full_copies(g):
        return w_copies(wqb_hbm, wob_hbm, wb, g, lambda i: b_sem)

    def quarters(copy):
        lax.fori_loop(0, 4, lambda i, _: copy(pl.ds(pl.multiple_of(i * 512, 512), 512),
                                              pl.ds(pl.multiple_of(i * 256, 256), 256)), None)

    def transposed(src, i, blocks, rows, dep):
        w = [src[i, _rows(b, rows), :] for b in blocks]
        w[0] = _halves(_head_after(_words(w[0]), 8, dep))
        return jnp.concatenate(w, axis=0).T

    def weight_steps(i, dst, j):
        def step(k):
            def run(dep):
                t = [transposed(wa, i, (4 * k + e, 4 * k + 2 + e), 64, None if e else dep)
                     for e in range(2)]
                for e, a in enumerate(_operands(LEFT, lambda r, c: t[c][_rows(r, 64)])):
                    _put(dst, (j, e), k, a)
            return run
        return [step(k) for k in range(4)]

    def weight2_steps(i, dst, j):
        def flip(k, r, c):
            def run(dep):
                for e in (c, c + 1):
                    wt[e, _rows(r, 64), :] = _words(transposed(
                        wb, i + 4 * r, range(16 * k + e, 16 * k + 16, 4), 32, None if e > c else dep))
            return run

        def step(k, s, e):
            def run(dep):
                def block(r, c):
                    x = _halves(wt[c + zeros[e], _rows(4 * r + s, 8), :]).astype(f32)
                    return _head_after(x, 8, dep) if r % 2 == c % 2 else x

                for n, a in enumerate(_inner_operands(LEFT, e, block)):
                    _put(dst, (j, 7 * e + n), 4 * k + s, a)
            return run
        return [x for k in range(2)
                for x in [flip(k, r, c) for r in range(2) for c in (0, 2)] + [None] * 6
                + [step(k, s, e) for s in range(4) for e in range(7)]]

    def project2_steps(w, i, j, emit):
        def step(e):
            def run():
                ys, ms = _project(w, i, ho2, j, 7 * e)
                m = jnp.stack(ys)

                def held(k):
                    return sums[k][pl.ds(zeros[e], 2)]

                if e == 0:
                    sums[0][...] = m
                elif e == 1:
                    emit(1, 0, held(0) + m)
                    sums[1][...] = m
                elif e == 2:
                    sums[2][...] = held(0) - m
                    sums[3][...] = held(1) + m
                elif e == 3:
                    sums[0][...] = held(2) - m
                elif e == 4:
                    emit(1, 1, held(0) + m)
                    sums[1][...] = m
                elif e == 5:
                    emit(0, 1, held(1) + m)
                    sums[2][...] = held(3) + m
                else:
                    emit(0, 0, held(2) + m)
                return [(ms[min(s // 8 * 2 + e % 2, 6)], s % 8) for s in range(28)]
            return run
        return [step(e) for e in range(7)]

    def local_tile(j, n):
        return 4 * (j & 3) + 2 * n + (j >> 2)

    def local_qkv_steps(par):
        def put(buf, i, y):
            for h in range(4):
                buf[i, pl.ds(h, DH, stride=4), :] = y[_rows(h, DH)]

        def step(j, i):
            def run():
                ys, ms = _project(wj, i, ha, par * (NP // 2) + j)
                for r, y in zip((2 * j, 2 * j + 1), ys):
                    if i == 0:
                        put(qbuf[par], r, y)
                        continue
                    buf = kbuf[par] if i == 1 else vbuf[par]
                    put(buf, r + WIN - 1, y)
                    if r > 0:
                        put(buf, r - 1, pltpu.roll(y, 1, 1))
                return _marks(ms)
            return run
        return [step(j, i) for i in (1, 2, 0) for j in range(NP // 2)]

    def local_att_steps(g, par):
        def tile_steps(r):
            logits, probs = [], []

            def score(i):
                def run(dep):
                    q = _head_after(qbuf[par][r + zeros[i]], 8, dep, *logits[-1:])
                    for w in (i, i + 1):
                        s = _slab_sum(q * kbuf[par][r + w + zeros[r]])
                        logits.append(s + pltpu.roll(s, 4, 0))
                return run

            def softmax(dep):
                s = jnp.concatenate(logits, axis=0) * QSCALE
                if r < WIN - 1:
                    wrapped = 8 * (WIN - 1 - r)
                    first = lax.broadcasted_iota(i32, (wrapped, 128), 1) == 0
                    s = jnp.concatenate([jnp.where(first, MASKED, s[:wrapped]), s[wrapped:]], axis=0)
                s = s.reshape(WIN, 8, 128)
                p = jnp.exp2(s - jnp.max(s, axis=0))
                probs.append(p * _inverse(jnp.sum(p, axis=0)))

            def mix(i):
                def run(dep):
                    p = _head_after(probs[0], 1, dep)
                    v = vbuf[par][pl.ds(r + zeros[r], WIN), _rows(i, 16), :]
                    ol[r % 2, _rows(i, 16), :] = jnp.sum(jnp.concatenate([p, p], axis=1) * v, axis=0)
                return run

            return ([s for i in range(0, WIN, 2) for s in (score(i), None)] + [softmax, None]
                    + [mix(i) for i in range(8)])

        def operands(j, i):
            def run(dep):
                def block(e, n):
                    x = ol[n + zeros[0], pl.ds(64 * (i % 2) + i // 2 + 2 * e, 16, stride=4), :]
                    return _head_after(x, 8, dep) if e == n else x

                for e, b in enumerate(_operands(RIGHT, block)):
                    _put(oa, (par * (NP // 2) + j, e), 4 * g + i, b)
            return run

        return [s for j in range(NP // 2) for s in tile_steps(2 * j) + tile_steps(2 * j + 1)
                + [operands(j, i) for i in range(4)]]

    def input_ln_steps(j):
        return _layernorm_steps(2, lambda n: ma[local_tile(j, n)],
                                lambda n, c, rows, i: xa[local_tile(j, n), c, rows, :], ha, j)

    def proj_steps(quad):
        def step(j, c):
            def run():
                ys, ms = _project(wot, c, oa, j)
                for n in range(2):
                    y = xa[local_tile(j, n), c] + ys[n]
                    xb[local_tile(j, n), c] = y
                    ybuf[quad % 2][j % 2 * 2 + n, c] = y
                    mbuf[quad % 2][j % 2 * 2 + n, c] = _moments(y)
                return _marks(ms)
            return run
        return [step(j, c) for j in (2 * quad, 2 * quad + 1) for c in range(NG)]

    def proj_ln_steps(quad):
        return _layernorm_steps(4, lambda n: mbuf[quad % 2][n + zeros[0]],
                                lambda n, c, rows, i: ybuf[quad % 2][n + zeros[i], c, rows, :],
                                ho2, quad)

    def local_layer(rep):
        def fetch_weights(g):
            @pl.when(rep == 0)
            def _():
                @pl.when(g + 1 < NG)
                def _():
                    for cp in local_copies(g + 1):
                        cp.wait()

                @pl.when(g + 2 < NG)
                def _():
                    for cp in local_copies(g + 2):
                        cp.start()

                for cp in full_copies(g):
                    cp.start()

        def w_steps(g):
            nxt = 4 * ((g + 1) & (NG - 1))
            return (weight_steps(4 * g, wj, 0) + [None] * 4
                    + weight_steps(4 * g + 3, wot, g) + [None] * 4
                    + weight_steps(nxt + 1, wj, 1) + weight_steps(nxt + 2, wj, 2))

        if 'a' in PHASES:
          with scope('A0'):
            ln = [input_ln_steps(j) for j in range(NP)]
            even, odd, first = local_qkv_steps(0), local_qkv_steps(1), w_steps(0)
            _run(ln[0])
            marks = _interleave(even[0::4], [None] * 8 + ln[1] + [None] * 6, first[:4] + [None] * 3)
            for j in (1, 2, 3):
                marks = _interleave(even[j::4], ln[j + 1] + [None] * 6, [first[8 + j]], marks=marks)
            fetch_weights(0)
            att = local_att_steps(0, 0)
            marks = None
            for j in (0, 1, 2):
                marks = _interleave(odd[j::4], ln[j + 5] + [None] * 6, att[30 * j:30 * j + 30],
                                    marks=marks)
            _interleave(odd[3::4], att[90:], first[8:9] + [None] * 2 + first[16:], marks=marks)

        def group(g, _):
            fetch_weights(g)
            _interleave(local_qkv_steps(0) + local_qkv_steps(1),
                        local_att_steps(g - 1, 1) + local_att_steps(g, 0), w_steps(g))

        if 'b' in PHASES:
          with scope('A1'):
            lax.fori_loop(1, NG, group, None)

        @pl.when(rep == 0)
        def _():
            pltpu.make_async_copy(wb, wb, b_sem).wait()

    def full_qkv_steps(gp, i):
        def steps(quad):
            def emit(r, c, ys):
                for n in range(2):
                    g, kt = 2 * gp + r, 4 * quad + 2 * c + n
                    if i == 0:
                        xa[local_tile(2 * quad + c, n), g] = ys[n] * QSCALE
                    elif i == 1:
                        kk[g, kt] = _words(ys[n].astype(bf16).T)
                    else:
                        vt[g, kt] = _words(ys[n])
            return project2_steps(wq2, i, quad, emit)
        return [s for quad in range(NQ) for s in steps(quad)]

    def spread_steps(g):
        def step(kt, e):
            def run(dep):
                k = _after(kk[g + zeros[e % 8], kt, 56:, :], dep)
                for f in range(4 * e, 4 * e + 4):
                    h, d = divmod(f, DH)
                    x = _halves(jnp.broadcast_to(k[:, f:f + 1], (8, 128))).astype(f32)
                    kb[h // 2][g, pl.ds(h % 2 * 8 + 2 * kt, 2), _rows(d, 8), :] = x.reshape(2, 8, 128)
            return run
        return [step(kt, e) for kt in range(VPU_TILES) for e in range(32)]

    def full_qkv(gp, more):
        pad = [None] * 4
        out_w = weight2_steps(8 * gp + 3, wo2, gp)
        marks = _interleave(full_qkv_steps(gp, 0),
                            weight2_steps(8 * gp + 2, wq2, 2)
                            + (weight2_steps(8 * gp + 9, wq2, 1) if more else out_w))
        marks = _interleave(full_qkv_steps(gp, 2),
                            spread_steps(2 * gp) + spread_steps(2 * gp + 1) + 2 * pad,
                            weight2_steps(8 * gp + 8, wq2, 0) if more else [], marks=marks)
        if more:
            _interleave(full_qkv_steps(gp + 1, 1), out_w + pad, marks=marks)

    def full_att(base, count, state, first=False, last=False):
        def item(u):
            return base + u // 16, u % 4, u % 16 // 4

        def operands(blk, slot, step, dep):
            i, e = divmod(step, 7)

            def block(r, c):
                x = oq[slot % 2][4 * r + c + zeros[e], _rows(i, 16), :]
                return _head_after(x, 8, dep) if r % 2 == c % 2 else x

            ops = _inner_operands(RIGHT, e, block)
            for k, b in enumerate(ops):
                _put(ho2, (blk & 3, 7 * e + k), 2 * (blk >> 2) + i, b)
            return ops[2][:8]

        m, m_next, den, acc = state
        marks = None
        for u in range(count + (2 if last else 0)):
            scores = u < count
            if scores:
                blk, n, h = item(u)
                parts = [jnp.zeros((DH, 128), f32)] * 4
                parts[h] = xa[4 * (blk & 3) + n, blk >> 2, _rows(h, DH), :]
                q = jnp.concatenate(parts, axis=0).astype(bf16)
                for i in range(4):
                    rows = _after(parts[h][_rows(i, 8)], marks and _slab(marks[42 + 3 * i]))
                    for d in range(8):
                        qb[u % 2][0, _rows(8 * i + d, 8), :] = jnp.broadcast_to(rows[d:d + 1], (8, 128))
                top, marks = None, []
            for c in range(4):
                if scores:
                    for kt in range(4 * c, 4 * c + 4):
                        keys = 112 if kt < VPU_TILES else 128
                        s = _dot(_halves(kk[blk >> 2, kt, :keys // 2, :]), q)
                        sbuf[u % 2][128 * kt:128 * kt + keys, :] = s
                        top = _slab_max(s, top)
                    marks += [(s, i) for i in range(14)]
                up, cp = divmod(4 * (u - 1) + c - 2, 4)
                if (first and up < 0) or up >= count:
                    continue
                if cp == 0:
                    m, den, acc = m_next, None, None
                blkp, _, hp = item(up)
                for kt in range(4 * cp, 4 * cp + 4):
                    p = jnp.exp2(sbuf[up % 2][_rows(kt), :] - m)
                    den = _slab_sum(p, den)
                    o = _dot(_halves(vt[blkp >> 2, kt, _rows(hp, DH // 2), :]), p)
                    acc = o if acc is None else acc + o
                if cp == 3:
                    o = acc * _inverse(jnp.sum(den, axis=0, keepdims=True))
                    oq[(up // 16 + first) % 2][up % 16] = o
                if up % 16 < 4 and not (first and up < 16) and 4 * (up % 16) + cp < 14:
                    operands(blkp - 1, up // 16 - 1, 4 * (up % 16) + cp, _slab(marks[-7]))
            if scores:
                s = None
                for e in range(2 * VPU_TILES):
                    qd = _head_after(qb[u % 2][zeros[e]], 8, _slab(marks[7 * e]), s)
                    s = _slab_sum(kb[h // 2][(blk >> 2) + zeros[u % 8], h % 2 * 8 + e] * qd)
                    sbuf[u % 2][pl.ds(128 * (e // 2) + 112 + 8 * (e % 2), 8), :] = s
                    top = jnp.maximum(top, s)
                m_next = jnp.max(top, axis=0, keepdims=True)
        if last:
            dep = None
            for step in range(14):
                dep = operands(base + count // 16 - 1, count // 16 - 1, step, dep)
        return m, m_next, den, acc

    def full_layer(rep):
        if 'c' in PHASES:
          with scope('A2'):
            @separately
            def _():
                marks = _interleave(proj_steps(0), local_att_steps(NG - 1, 1),
                                    weight2_steps(1, wq2, 1))
                _interleave(proj_steps(1), [None] * 6 + proj_ln_steps(0), marks=marks)

            @separately
            def _():
                marks = _interleave(proj_steps(2), proj_ln_steps(1))
                marks = _interleave(proj_steps(3), [None] * 6 + proj_ln_steps(2), marks=marks)
                _interleave(full_qkv_steps(0, 1), [None] * 6 + proj_ln_steps(3) + [None] * 48,
                            weight2_steps(0, wq2, 0) + [None] * 4, marks=marks)
        if 'e' in PHASES:
          with scope('B1'):
            lax.fori_loop(0, NG // 2 - 1, lambda gp, _: full_qkv(gp, True), None)
        if 'f' in PHASES:
            separately(lambda: full_qkv(NG // 2 - 1, False))

        items = HEADS * NT
        head = ATT_UNROLL // 2
        if 'd' in PHASES:
          with scope('B2'):
            state = full_att(0, head, (None,) * 4, first=True)
            state = lax.fori_loop(
                0, items // ATT_UNROLL - 1,
                lambda j, st: full_att(head // 16 + j * (ATT_UNROLL // 16), ATT_UNROLL, st), state)
            full_att((items - ATT_UNROLL + head) // 16, ATT_UNROLL - head, state, last=True)
        else:
            full_att(1, 4, (None,) * 4, first=True, last=True)

        def proj(i, _):
            def steps(quad):
                def emit(r, c, ys):
                    bits = []
                    for n in range(2):
                        t = 4 * quad + 2 * c + n
                        y = xb[t, 2 * i + r] + ys[n]
                        xa[t, 2 * i + r] = y
                        ma[t, 2 * i + r] = _moments(y)
                        bits.append(lax.bitcast_convert_type(y.astype(bf16).astype(f32), i32))
                    pair = lax.shift_right_logical(bits[0], 16) | bits[1]
                    xw[r, pl.ds(2 * quad + c, 128, stride=NP), :] = pair.T
                return project2_steps(wo2, i, quad, emit)

            _interleave([s for quad in range(NQ) for s in steps(quad)])

            @pl.when(rep == 1)
            def _():
                for r in (1, 0):
                    @quarters
                    def _(rows, words):
                        xio[2 * i + r, rows, :] = _halves(xw[r, words, :]).astype(f32).astype(bf16)

                    out_copy(2 * i + r).start()

        with scope('B3'):
            lax.fori_loop(0, NG // 2, proj, None)

    first_w = local_copies(0)
    for cp in first_w[1:3] + [x_copy(0)]:
        cp.start()
    for i in (1, 2):
        with scope(f'ww{i}'):
            first_w[i].wait()
        x_copy(i).start()
        _run(weight_steps(i, wj, i))

    def stage_in(c, _):
        with scope('xw'):
            x_copy(c).wait()

        @pl.when(c + 3 < NG)
        def _():
            x_copy(c + 3).start()

        @pl.when(c + 2 == NG)
        def _():
            for cp in first_w[::3]:
                cp.start()

        @quarters
        def _(rows, words):
            xw[0, words, :] = _words(xio[c, rows, :])

        for j in range(NP):
            pair = xw[0, pl.ds(j, 128, stride=NP), :].T
            for n, bits in enumerate((pair << 16, pair & -65536)):
                y = lax.bitcast_convert_type(bits, f32)
                xa[2 * j + n, c] = y
                ma[2 * j + n, c] = _moments(y)

    with scope('stage'):
        lax.fori_loop(0, NG, stage_in, None)
    for cp in local_copies(1):
        cp.start()
    with scope('ww03'):
      for cp in first_w[::3]:
        cp.wait()

    def two_layers(rep, _):
        zeros[:] = [(rep + i) >> 4 for i in range(8)]
        local_layer(rep)
        full_layer(rep)

    with scope('main'):
        lax.fori_loop(0, 2, two_layers, None)
    with scope('tail'):
      for c in range(NG):
        out_copy(c).wait()


@jax.jit
def pallas_interleave_layers__sliding_local_dilated__softmax_full_mha__prompt_kernel(
    A_x: jax.Array,
    A_wqkv: jax.Array,
    A_wo: jax.Array,
    B_x: jax.Array,
    B_wqkv: jax.Array,
    B_wo: jax.Array,
):
    del B_x
    assert A_x.shape == (1, SEQ, D) and A_x.dtype == bf16
    vmem, dma = pltpu.VMEM, pltpu.SemaphoreType.DMA
    tile, words = (128, 128), (64, 128)
    scratch = [
        vmem((NG, SEQ, 128), bf16),
        vmem((2, SEQ // 2, 128), i32),
        *[vmem((4 * NG, D, 128), bf16)] * 2,
        vmem((3, 7, D // 8, 128), i32),
        vmem((NG, 7, D // 8, 128), i32),
        vmem((3, 49) + tile, bf16),
        vmem((NG // 2, 49) + tile, bf16),
        vmem((4,) + tile, i32),
        *[vmem((NT, NG) + tile, f32)] * 2,
        *[vmem((NP, 16, D // 4, 128), f32)] * 2,
        vmem((NQ, 49, D // 4, 128), bf16),
        *[vmem((WIN,) + tile, f32)] * 2,
        *[vmem((2 * WIN - 1,) + tile, f32)] * 4,
        vmem((2,) + tile, f32),
        *[vmem((4, NG) + tile, f32)] * 2,
        vmem((NT, NG, 16, 128), f32),
        *[vmem((4, NG, 16, 128), f32)] * 2,
        *[vmem((NG, NT) + words, i32)] * 2,
        *[vmem((1, DH * 8, 128), f32)] * 2,
        *[vmem((SEQ, 128), f32)] * 2,
        *[vmem((16, DH, 128), f32)] * 2,
        dma((NG,)), dma((4 * NG,)), dma(()), dma((NG,)),
        *[vmem((2,) + tile, f32)] * 4,
    ]
    hbm = pl.BlockSpec(memory_space=pl.ANY)
    out = pl.pallas_call(
        _kernel,
        out_shape=jax.ShapeDtypeStruct((SEQ, D), bf16),
        in_specs=[hbm] * 5,
        out_specs=hbm,
        scratch_shapes=scratch,
        compiler_params=pltpu.CompilerParams(
            vmem_limit_bytes=127 * 1024 * 1024,
            disable_bounds_checks=True,
            flags={"XLA_TPU_FORCE_LP_LLO_SCHEDULER": True},
        ),
        name="interleaved_layers",
    )(A_x.reshape(SEQ, D), A_wqkv, A_wo, B_wqkv, B_wo)
    return out.reshape(1, SEQ, D)
```

```python
import math

import jax
import jax.numpy as jnp
from jax import lax
import jax.experimental.pallas as pl
import jax.experimental.pallas.tpu as pltpu

SEQ, D, HEADS, DH = 2048, 1024, 32, 32
WIN = 8
NT = SEQ // 128
NP = NT // 2
NQ = NT // 4
NG = D // 128
EPS = 1e-5
LOG2E = math.log2(math.e)
QSCALE = DH ** -0.5 * LOG2E
MASKED = -1e9 * LOG2E
ATT_UNROLL = 32
VPU_TILES = 4
DELAY = 16
PHASES = 'abcdef'
SCOPES = False
import contextlib
def scope(n):
    return jax.named_scope(n) if SCOPES else contextlib.nullcontext()

bf16, f32, i32 = jnp.bfloat16, jnp.float32, jnp.int32


def _rows(i, n=128):
    return slice(i * n, (i + 1) * n)


def _words(x):
    return pltpu.bitcast(x.astype(bf16), i32)


def _halves(x):
    return pltpu.bitcast(x, bf16)


def _put(ref, idx, block, x):
    x = x.astype(bf16) if ref.dtype == bf16 else pltpu.bitcast(x.astype(bf16), ref.dtype)
    n = x.shape[0]
    ref[(*idx, pl.ds(pl.multiple_of(block * n, n), n), slice(None))] = x


def _get(ref, *idx):
    return ref[idx] if ref.dtype == bf16 else _halves(ref[idx])


def _dot(a, b):
    return jnp.dot(a, b, preferred_element_type=f32)


def _slab_sum(x, acc=None):
    x = x if acc is None else jnp.concatenate([acc, x], axis=0)
    return jnp.sum(x.reshape(-1, 8, x.shape[1]), axis=0)


def _slab_max(x, acc=None):
    x = x if acc is None else jnp.concatenate([acc, x], axis=0)
    return jnp.max(x.reshape(-1, 8, x.shape[1]), axis=0)


def _inverse(x):
    r = pl.reciprocal(x, approx=True)
    return r * (2.0 - x * r)


def _after(x, *deps):
    low = x
    for dep in deps:
        if dep is not None:
            low = jnp.minimum(low, lax.bitcast_convert_type(dep, x.dtype))
    return x if low is x else jnp.maximum(x, low)


def _head_after(x, n, *deps):
    return jnp.concatenate([_after(x[:n], *deps), x[n:]], axis=0)


def _slab(mark):
    return mark and mark[0][_rows(mark[1], 8)]


LEFT = [((1, 0), 1, (1, 1)), ((1, 1),), ((0, 0), 1, (1, 1)), ((1, 0), -1, (0, 0)),
        ((0, 0),), ((0, 0), 1, (0, 1)), ((0, 1), -1, (1, 1))]
RIGHT = [((0, 0),), ((1, 0), -1, (0, 0)), ((0, 0), -1, (1, 1)), ((0, 0), -1, (0, 1)),
         ((0, 1), -1, (1, 1)), ((1, 1),), ((1, 0), -1, (1, 1))]


def _operand(term, block):
    if len(term) == 1:
        return block(*term[0])
    a, b = block(*term[0]).astype(f32), block(*term[2]).astype(f32)
    return a + b if term[1] > 0 else a - b


def _operands(side, block):
    grid = [[block(r, c) for c in range(2)] for r in range(2)]
    return [_operand(term, lambda r, c: grid[r][c]) for term in side]


def _inner_operands(side, e, block):
    return _operands(side, lambda r, c: _operand(side[e], lambda i, j: block(2 * i + r, 2 * j + c)))


def _project(w, i, right, first=0):
    ms = []
    for e in range(first, first + 7):
        a, b = _get(w, i, e), right(e)
        ms.append(_dot(jnp.concatenate(jnp.split(a, b.shape[0] // 128), axis=1), b))
    m2, m4, m1, m6, m3, m5, m7 = ms
    y1 = jnp.concatenate([m4 + m1 + m5 + m7, m2 + m4], axis=0)
    y2 = jnp.concatenate([m5 + m3, m2 - m1 - m6 + m3], axis=0)
    return (y1, y2), ms


def _marks(ms):
    return [(m, s) for m in ms for s in range(8)]


def _interleave(main, *sides, marks=None):
    done = [0] * len(sides)
    marks = marks or [None] * DELAY
    for i, step in enumerate(main):
        marks += step()
        total = (len(marks) - DELAY) * len(main) // (i + 1)
        for k, side in enumerate(sides):
            upto = (i + 1) * len(side) // len(main)
            for e in range(done[k], upto):
                if side[e] is not None:
                    side[e](_slab(marks[e * total // len(side)]))
            done[k] = upto
    return marks[-DELAY:]


def _run(steps):
    for step in steps:
        if step is not None:
            step(None)


def _moments(x):
    mean = _slab_sum(x) * (1.0 / 16)
    d = x - jnp.tile(mean, (16, 1))
    return jnp.concatenate([mean, _slab_sum(d * d)], axis=0)


def _stats_steps(tiles, moments):
    mean, rstd = [], []

    def step(n):
        def run(dep):
            part = moments(n)
            mu = jnp.sum(_head_after(part[:, :8], 1, dep), axis=0)
            mu = jnp.sum(mu, axis=0, keepdims=True) * (16.0 / D)
            d = part[:, :8] - mu
            var = jnp.sum(part[:, 8:], axis=0) + 16.0 * jnp.sum(d * d, axis=0)
            var = jnp.sum(var, axis=0, keepdims=True) * (1.0 / D)
            mean.append(jnp.broadcast_to(mu, (8, 128)))
            rstd.append(jnp.broadcast_to(lax.rsqrt(var + EPS), (8, 128)))
        return run

    return [step(n) for n in range(tiles)] + [None], mean, rstd


def _normalize(x, mean, rstd):
    reps = (x.shape[0] // 8, 1)
    return (x - jnp.tile(mean, reps)) * jnp.tile(rstd, reps)


def _kernel(x_hbm, wqa_hbm, woa_hbm, wqb_hbm, wob_hbm, out_hbm,
            xio, xw, wa, wb, wj, wot, wq2, wo2, wt, xa, xb, ha, oa, ho2,
            q0, q1, k0, k1, v0, v1, ol, y0, y1, n0, n1, ma, m0, m1,
            kk, vt, qb0, qb1, s0, s1, oq0, oq1, x_sem, a_sem, b_sem, o_sem, *sums):
    qbuf, kbuf, vbuf, oq = (q0, q1), (k0, k1), (v0, v1), (oq0, oq1)
    kb = (ha, oa)
    ybuf, normed, mbuf, qb, sbuf = (y0, y1), (n0, n1), (m0, m1), (qb0, qb1), (s0, s1)

    zeros, blocks = [], []

    def separately(body):
        blocks.append(body)
        pl.when(zeros[len(blocks)] == 0)(body)

    def cols(c):
        return pl.ds(pl.multiple_of(c * 128, 128), 128)

    def x_copy(c):
        return pltpu.make_async_copy(x_hbm.at[:, cols(c)], xio.at[c], x_sem.at[c])

    def out_copy(c):
        return pltpu.make_async_copy(xio.at[c], out_hbm.at[:, cols(c)], o_sem.at[c])

    def w_copies(qkv_hbm, o_hbm, dst, g, sem):
        srcs = [qkv_hbm.at[:, cols(i * NG + g)] for i in range(3)] + [o_hbm.at[:, cols(g)]]
        return [pltpu.make_async_copy(src, dst.at[4 * g + i], sem(i)) for i, src in enumerate(srcs)]

    def local_copies(g):
        return w_copies(wqa_hbm, woa_hbm, wa, g, lambda i: a_sem.at[4 * g + i])

    def full_copies(g):
        return w_copies(wqb_hbm, wob_hbm, wb, g, lambda i: b_sem)

    def quarters(copy):
        lax.fori_loop(0, 4, lambda i, _: copy(pl.ds(pl.multiple_of(i * 512, 512), 512),
                                              pl.ds(pl.multiple_of(i * 256, 256), 256)), None)

    def transposed(src, i, blocks, rows, dep):
        w = [src[i, _rows(b, rows), :] for b in blocks]
        w[0] = _halves(_head_after(_words(w[0]), 8, dep))
        return jnp.concatenate(w, axis=0).T

    def weight_steps(i, dst, j):
        def step(k):
            def run(dep):
                t = [transposed(wa, i, (4 * k + e, 4 * k + 2 + e), 64, None if e else dep)
                     for e in range(2)]
                for e, a in enumerate(_operands(LEFT, lambda r, c: t[c][_rows(r, 64)])):
                    _put(dst, (j, e), k, a)
            return run
        return [step(k) for k in range(4)]

    def weight2_steps(i, dst, j):
        def flip(k, r, c):
            def run(dep):
                for e in (c, c + 1):
                    wt[4 * k + e, _rows(r, 64), :] = _words(transposed(
                        wb, i + 4 * r, range(16 * k + e, 16 * k + 16, 4), 32, None if e > c else dep))
            return run

        def step(k, s, e):
            def run(dep):
                def block(r, c):
                    x = _halves(wt[4 * k + c + zeros[e], _rows(4 * r + s, 8), :]).astype(f32)
                    return _head_after(x, 8, dep) if r % 2 == c % 2 else x

                for n, a in enumerate(_inner_operands(LEFT, e, block)):
                    _put(dst, (j, 7 * e + n), 4 * k + s, a)
            return run
        return ([flip(k, r, c) for k in range(2) for r in range(2) for c in (0, 2)] + [None] * 6
                + [step(k, s, e) for k in range(2) for s in range(4) for e in range(7)])

    def project2_steps(w, i, j, emit):
        def step(e):
            def run():
                ys, ms = _project(w, i, lambda k: ho2[j, k], 7 * e)
                m = jnp.stack(ys)

                def held(k):
                    return sums[k][pl.ds(zeros[e], 2)]

                if e == 0:
                    sums[0][...] = m
                elif e == 1:
                    emit(1, 0, held(0) + m)
                    sums[1][...] = m
                elif e == 2:
                    sums[2][...] = held(0) - m
                    sums[3][...] = held(1) + m
                elif e == 3:
                    sums[0][...] = held(2) - m
                elif e == 4:
                    emit(1, 1, held(0) + m)
                    sums[1][...] = m
                elif e == 5:
                    emit(0, 1, held(1) + m)
                    sums[2][...] = held(3) + m
                else:
                    emit(0, 0, held(2) + m)
                return [(ms[min(s // 8 * 2 + e % 2, 6)], s % 8) for s in range(28)]
            return run
        return [step(e) for e in range(7)]

    def local_tile(j, n):
        return 4 * (j & 3) + 2 * n + (j >> 2)

    def local_qkv_steps(par, first=False):
        def put(buf, i, y):
            for h in range(4):
                buf[i, pl.ds(h, DH, stride=4), :] = y[_rows(h, DH)]

        def step(j, i):
            def run():
                pair = par * (NP // 2) + j

                def right(e):
                    if not first:
                        return _get(ha, pair, e)
                    quad, slot = parked(pair, e)
                    b = ho2[quad, pl.ds(slot, 2)].reshape(D // 2, 128)
                    if e % 3 == i:
                        _put(ha, (pair, e), 0, b)
                    return b

                ys, ms = _project(wj, i, right)
                for r, y in zip((2 * j, 2 * j + 1), ys):
                    if i == 0:
                        put(qbuf[par], r, y)
                        continue
                    buf = kbuf[par] if i == 1 else vbuf[par]
                    put(buf, r + WIN - 1, y)
                    if r > 0:
                        put(buf, r - 1, pltpu.roll(y, 1, 1))
                return _marks(ms)
            return run
        return [step(j, i) for i in (1, 2, 0) for j in range(NP // 2)]

    def local_att_steps(g, par):
        def tile_steps(r):
            logits, probs = [], []

            def score(i):
                def run(dep):
                    q = _head_after(qbuf[par][r + zeros[i]], 8, dep, *logits[-1:])
                    for w in (i, i + 1):
                        s = _slab_sum(q * kbuf[par][r + w + zeros[r]])
                        logits.append(s + pltpu.roll(s, 4, 0))
                return run

            def softmax(dep):
                s = jnp.concatenate(logits, axis=0) * QSCALE
                if r < WIN - 1:
                    wrapped = 8 * (WIN - 1 - r)
                    first = lax.broadcasted_iota(i32, (wrapped, 128), 1) == 0
                    s = jnp.concatenate([jnp.where(first, MASKED, s[:wrapped]), s[wrapped:]], axis=0)
                s = s.reshape(WIN, 8, 128)
                p = jnp.exp2(s - jnp.max(s, axis=0))
                probs.append(p * _inverse(jnp.sum(p, axis=0)))

            def mix(i):
                def run(dep):
                    p = _head_after(probs[0], 1, dep)
                    v = vbuf[par][pl.ds(r + zeros[r], WIN), _rows(i, 16), :]
                    ol[r % 2, _rows(i, 16), :] = jnp.sum(jnp.concatenate([p, p], axis=1) * v, axis=0)
                return run

            return ([s for i in range(0, WIN, 2) for s in (score(i), None)] + [softmax, None]
                    + [mix(i) for i in range(8)])

        def operands(j, i):
            def run(dep):
                def block(e, n):
                    x = ol[n + zeros[0], pl.ds(64 * (i % 2) + i // 2 + 2 * e, 16, stride=4), :]
                    return _head_after(x, 8, dep) if e == n else x

                for e, b in enumerate(_operands(RIGHT, block)):
                    _put(oa, (par * (NP // 2) + j, e), 4 * g + i, b)
            return run

        return [s for j in range(NP // 2) for s in tile_steps(2 * j) + tile_steps(2 * j + 1)
                + [operands(j, i) for i in range(4)]]

    def parked(j, e):
        return j // 2, 14 * (j % 2) + 2 * e

    def input_ln_steps(j):
        stats, mean, rstd = _stats_steps(2, lambda n: ma[local_tile(j, n)])
        last = []

        def step(c, i):
            def run(dep):
                prev = last.pop() if last else rstd[1]
                dep = prev if dep is None else jnp.minimum(dep, prev)
                mu = [_after(m, dep) for m in mean]
                ops = _operands(RIGHT, lambda k, n: _normalize(
                    xa[local_tile(j, n), c, _rows(4 * k + i, 16), :], mu[n], rstd[n]))
                for e, b in enumerate(ops):
                    quad, slot = parked(j, e)
                    _put(ho2, (quad, slot + c // 4), 4 * (c % 4) + i, b)
                last.append(ops[2][:8])
            return run
        return stats + [step(c, i) for c in range(NG) for i in range(4)]

    def proj_steps(quad):
        def step(j, c):
            def run():
                ys, ms = _project(wot, c, lambda e: _get(oa, j, e))
                for n in range(2):
                    y = xa[local_tile(j, n), c] + ys[n]
                    xb[local_tile(j, n), c] = y
                    ybuf[quad % 2][j % 2 * 2 + n, c] = y
                    mbuf[quad % 2][j % 2 * 2 + n, c] = _moments(y)
                return _marks(ms)
            return run
        return [step(j, c) for j in (2 * quad, 2 * quad + 1) for c in range(NG)]

    def quad_operands(quad, block_index, e, load, dep):
        def block(r, c):
            return _head_after(load(r, c), 8, dep) if r % 2 == c % 2 else load(r, c)

        ops = _inner_operands(RIGHT, e, block)
        for k, b in enumerate(ops):
            _put(ho2, (quad, 7 * e + k), block_index, b)
        return ops[2][:8]

    def proj_ln_steps(quad):
        stats, mean, rstd = _stats_steps(4, lambda n: mbuf[quad % 2][n + zeros[0]])

        def norm(c, n):
            def run(dep):
                normed[c % 2][n] = _normalize(ybuf[quad % 2][n + zeros[0], c],
                                              _after(mean[n], dep), rstd[n])
            return run

        def step(c, i, e):
            return lambda dep: quad_operands(
                quad, 2 * c + i, e,
                lambda k, n: normed[c % 2][n + zeros[e], _rows(2 * k + i, 16), :], dep)

        return stats + [s for c in range(NG) for s in [norm(c, n) for n in range(4)]
                        + [step(c, i, e) for i in range(2) for e in range(7)]]

    def local_layer(rep):
        def fetch_weights(g):
            @pl.when(rep == 0)
            def _():
                @pl.when(g + 1 < NG)
                def _():
                    for cp in local_copies(g + 1):
                        cp.wait()

                @pl.when(g + 2 < NG)
                def _():
                    for cp in local_copies(g + 2):
                        cp.start()

                for cp in full_copies(g):
                    cp.start()

        def w_steps(g):
            nxt = 4 * ((g + 1) & (NG - 1))
            return (weight_steps(4 * g, wj, 0) + [None] * 4
                    + weight_steps(4 * g + 3, wot, g) + [None] * 4
                    + weight_steps(nxt + 1, wj, 1) + weight_steps(nxt + 2, wj, 2))

        if 'a' in PHASES:
          with scope('A0'):
            ln = [input_ln_steps(j) for j in range(NP)]
            even, odd, first = local_qkv_steps(0, True), local_qkv_steps(1, True), w_steps(0)
            _run(ln[0])
            marks = _interleave(even[0::4], [None] * 8 + ln[1] + [None] * 6, first[:4] + [None] * 3)
            marks = _interleave(even[1::4], ln[2] + ln[4][:18], marks=marks)
            marks = _interleave(even[2::4], ln[3] + ln[4][18:], marks=marks)
            _interleave(even[3::4], ln[5] + ln[6], marks=marks)
            fetch_weights(0)
            att = local_att_steps(0, 0)
            marks = _interleave(odd[:2], ln[7], att[:16])
            _interleave(odd[2:], att[16:],
                        first[8:10] + first[16:20] + first[10:12] + first[20:] + [None], marks=marks)

        def group(g, _):
            fetch_weights(g)
            _interleave(local_qkv_steps(0) + local_qkv_steps(1),
                        local_att_steps(g - 1, 1) + local_att_steps(g, 0), w_steps(g))

        if 'b' in PHASES:
          with scope('A1'):
            lax.fori_loop(1, NG, group, None)

        @pl.when(rep == 0)
        def _():
            pltpu.make_async_copy(wb, wb, b_sem).wait()

    def full_qkv_steps(gp, i, slot=None):
        def steps(quad):
            def emit(r, c, ys):
                for n in range(2):
                    g, kt = 2 * gp + r, 4 * quad + 2 * c + n
                    if i == 0:
                        xa[local_tile(2 * quad + c, n), g] = ys[n] * QSCALE
                    elif i == 1:
                        kk[g, kt] = _words(ys[n].astype(bf16).T)
                    else:
                        vt[g, kt] = _words(ys[n])
            return project2_steps(wq2, i if slot is None else slot, quad, emit)
        return [s for quad in range(NQ) for s in steps(quad)]

    def spread_steps(g):
        def step(kt, e):
            def run(dep):
                k = _after(kk[g + zeros[e % 8], kt, 56:, :], dep)
                for f in range(4 * e, 4 * e + 4):
                    h, d = divmod(f, DH)
                    x = _halves(jnp.broadcast_to(k[:, f:f + 1], (8, 128))).astype(f32)
                    kb[h // 2][g, pl.ds(h % 2 * 8 + 2 * kt, 2), _rows(d, 8), :] = x.reshape(2, 8, 128)
            return run
        return [step(kt, e) for kt in range(VPU_TILES) for e in range(32)]

    def full_qkv(gp, more):
        pad = [None] * 3
        v_w, out_w = weight2_steps(8 * gp + 2, wq2, 2), weight2_steps(8 * gp + 3, wo2, gp)
        spread = spread_steps(2 * gp) + spread_steps(2 * gp + 1) + 3 * pad
        if more:
            marks = _interleave(full_qkv_steps(gp + 1, 1), v_w)
            marks = _interleave(full_qkv_steps(gp, 0),
                                weight2_steps((8 * gp + 17) & (4 * NG - 1), wq2, 1) + out_w,
                                marks=marks)
            _interleave(full_qkv_steps(gp, 2), weight2_steps(8 * gp + 8, wq2, 0) + pad,
                        [None] * 56 + spread, marks=marks)
        else:
            marks = _interleave(full_qkv_steps(gp, 0), v_w + out_w)
            _interleave(full_qkv_steps(gp, 2), spread, marks=marks)

    def full_att(base, count, state, first=False, last=False):
        def item(u):
            return base + u // 16, u % 4, u % 16 // 4

        def operands(blk, slot, step, dep):
            i, e = divmod(step, 7)
            return quad_operands(
                blk & 3, 2 * (blk >> 2) + i, e,
                lambda r, c: oq[slot % 2][4 * r + c + zeros[e], _rows(i, 16), :], dep)

        def fetch_q(u, marks):
            blk, n, h = item(u)
            q = xa[4 * (blk & 3) + n, blk >> 2, _rows(h, DH), :]
            for i in range(4):
                rows = _after(q[_rows(i, 8)], marks and _slab(marks[28 + 3 * i]))
                for d in range(8):
                    qb[u % 2][0, _rows(8 * i + d, 8), :] = jnp.broadcast_to(rows[d:d + 1], (8, 128))
            return q

        m, m_next, den, acc, q_next = state or (None,) * 4 + (fetch_q(0, None),)
        for u in range(count + (2 if last else 0)):
            scores = u < count
            if scores:
                blk, n, h = item(u)
                parts = [jnp.zeros((DH, 128), f32)] * 4
                parts[h] = q_next
                q = jnp.concatenate(parts, axis=0).astype(bf16)
                top, marks = None, []
            for c in range(4):
                if scores:
                    for kt in range(4 * c, 4 * c + 4):
                        keys = 112 if kt < VPU_TILES else 128
                        s = _dot(_halves(kk[blk >> 2, kt, :keys // 2, :]), q)
                        sbuf[u % 2][128 * kt:128 * kt + keys, :] = s
                        top = _slab_max(s, top)
                    marks += [(s, i) for i in range(14)]
                up, cp = divmod(4 * (u - 1) + c - 2, 4)
                if (first and up < 0) or up >= count:
                    continue
                if cp == 0:
                    m, den, acc = m_next, None, None
                blkp, _, hp = item(up)
                for kt in range(4 * cp, 4 * cp + 4):
                    p = jnp.exp2(sbuf[up % 2][_rows(kt), :] - m)
                    den = _slab_sum(p, den)
                    o = _dot(_halves(vt[blkp >> 2, kt, _rows(hp, DH // 2), :]), p)
                    acc = o if acc is None else acc + o
                if cp == 3:
                    o = acc * _inverse(jnp.sum(den, axis=0, keepdims=True))
                    oq[(up // 16 + first) % 2][up % 16] = o
                if up % 16 < 4 and not (first and up < 16) and 4 * (up % 16) + cp < 14:
                    operands(blkp - 1, up // 16 - 1, 4 * (up % 16) + cp, _slab(marks[-1]))
            if scores:
                s = None
                for e in range(2 * VPU_TILES):
                    qd = _head_after(qb[u % 2][zeros[e]], 8, _slab(marks[7 * e]), s)
                    s = _slab_sum(kb[h // 2][(blk >> 2) + zeros[u % 8], h % 2 * 8 + e] * qd)
                    sbuf[u % 2][pl.ds(128 * (e // 2) + 112 + 8 * (e % 2), 8), :] = s
                    top = jnp.maximum(top, s)
                m_next = jnp.max(top, axis=0, keepdims=True)
                if not (last and u + 1 == count):
                    q_next = fetch_q(u + 1, marks)
        if last:
            dep = None
            for step in range(14):
                dep = operands(base + count // 16 - 1, count // 16 - 1, step, dep)
        return m, m_next, den, acc, q_next

    def full_layer(rep):
        if 'c' in PHASES:
          with scope('A2'):
            @separately
            def _():
                marks = _interleave(proj_steps(0), local_att_steps(NG - 1, 1))
                _interleave(proj_steps(1), [None] * 6 + proj_ln_steps(0),
                            weight2_steps(1, wq2, 2) + [None], marks=marks)

            @separately
            def _():
                marks = _interleave(proj_steps(2), proj_ln_steps(1), weight2_steps(9, wq2, 1))
                marks = _interleave(proj_steps(3), [None] * 6 + proj_ln_steps(2),
                                    weight2_steps(0, wq2, 0), marks=marks)
                _interleave(full_qkv_steps(0, 1, slot=2),
                            [None] * 6 + proj_ln_steps(3) + [None] * 56, marks=marks)
        if 'e' in PHASES:
          with scope('B1'):
            lax.fori_loop(0, NG // 2 - 1, lambda gp, _: full_qkv(gp, True), None)
        if 'f' in PHASES:
            separately(lambda: full_qkv(NG // 2 - 1, False))

        items = HEADS * NT
        head = ATT_UNROLL // 2
        if 'd' in PHASES:
          with scope('B2'):
            state = full_att(0, head, None, first=True)
            state = lax.fori_loop(
                0, items // ATT_UNROLL - 1,
                lambda j, st: full_att(head // 16 + j * (ATT_UNROLL // 16), ATT_UNROLL, st), state)
            full_att((items - ATT_UNROLL + head) // 16, ATT_UNROLL - head, state, last=True)
        else:
            full_att(1, 4, None, first=True, last=True)

        def proj(i, _):
            late = []

            def steps(quad):
                def emit(r, c, ys):
                    bits = []
                    for n in range(2):
                        t = 4 * quad + 2 * c + n
                        y = xb[t, 2 * i + r] + ys[n]
                        xa[t, 2 * i + r] = y
                        ma[t, 2 * i + r] = _moments(y)
                        bits.append(lax.bitcast_convert_type(y.astype(bf16).astype(f32), i32))
                    pair = lax.shift_right_logical(bits[0], 16) | bits[1]
                    if (quad, r, c) == (NQ - 1, 0, 0):
                        late.append(pair)
                    else:
                        xw[r, pl.ds(2 * quad + c, 128, stride=NP), :] = pair.T
                return project2_steps(wo2, i, quad, emit)

            _interleave([s for quad in range(NQ) for s in steps(quad)])

            @pl.when(rep == 1)
            def _():
                xw[0, pl.ds(NP - 2, 128, stride=NP), :] = late[0].T
                for r in (1, 0):
                    @quarters
                    def _(rows, words):
                        xio[2 * i + r, rows, :] = _halves(xw[r, words, :]).astype(f32).astype(bf16)

                    out_copy(2 * i + r).start()

        with scope('B3'):
            lax.fori_loop(0, NG // 2, proj, None)

    first_w = local_copies(0)
    for cp in first_w[1:3] + [x_copy(0)]:
        cp.start()
    for i in (1, 2):
        with scope(f'ww{i}'):
            first_w[i].wait()
        x_copy(i).start()
        _run(weight_steps(i, wj, i))

    def stage_in(c, _):
        with scope('xw'):
            x_copy(c).wait()

        @pl.when(c + 3 < NG)
        def _():
            x_copy(c + 3).start()

        @pl.when(c + 2 == NG)
        def _():
            for cp in first_w[::3]:
                cp.start()

        @quarters
        def _(rows, words):
            xw[0, words, :] = _words(xio[c, rows, :])

        for j in range(NP):
            pair = xw[0, pl.ds(j, 128, stride=NP), :].T
            for n, bits in enumerate((pair << 16, pair & -65536)):
                y = lax.bitcast_convert_type(bits, f32)
                xa[2 * j + n, c] = y
                ma[2 * j + n, c] = _moments(y)

    with scope('stage'):
        lax.fori_loop(0, NG, stage_in, None)
    for cp in local_copies(1):
        cp.start()
    with scope('ww03'):
      for cp in first_w[::3]:
        cp.wait()

    def two_layers(rep, _):
        zeros[:] = [(rep + i) >> 4 for i in range(8)]
        local_layer(rep)
        full_layer(rep)

    with scope('main'):
        lax.fori_loop(0, 2, two_layers, None)
    with scope('tail'):
      for c in range(NG):
        out_copy(c).wait()


@jax.jit
def pallas_interleave_layers__sliding_local_dilated__softmax_full_mha__prompt_kernel(
    A_x: jax.Array,
    A_wqkv: jax.Array,
    A_wo: jax.Array,
    B_x: jax.Array,
    B_wqkv: jax.Array,
    B_wo: jax.Array,
):
    del B_x
    assert A_x.shape == (1, SEQ, D) and A_x.dtype == bf16
    vmem, dma = pltpu.VMEM, pltpu.SemaphoreType.DMA
    tile, words = (128, 128), (64, 128)
    scratch = [
        vmem((NG, SEQ, 128), bf16),
        vmem((2, SEQ // 2, 128), i32),
        *[vmem((4 * NG, D, 128), bf16)] * 2,
        vmem((3, 7, D // 8, 128), i32),
        vmem((NG, 7, D // 8, 128), i32),
        vmem((3, 49) + tile, bf16),
        vmem((NG // 2, 49) + tile, bf16),
        vmem((8,) + tile, i32),
        *[vmem((NT, NG) + tile, f32)] * 2,
        *[vmem((NP, 16, D // 4, 128), f32)] * 2,
        vmem((NQ, 49, D // 4, 128), bf16),
        *[vmem((WIN,) + tile, f32)] * 2,
        *[vmem((2 * WIN - 1,) + tile, f32)] * 4,
        vmem((2,) + tile, f32),
        *[vmem((4, NG) + tile, f32)] * 2,
        *[vmem((4,) + tile, f32)] * 2,
        vmem((NT, NG, 16, 128), f32),
        *[vmem((4, NG, 16, 128), f32)] * 2,
        *[vmem((NG, NT) + words, i32)] * 2,
        *[vmem((1, DH * 8, 128), f32)] * 2,
        *[vmem((SEQ, 128), f32)] * 2,
        *[vmem((16, DH, 128), f32)] * 2,
        dma((NG,)), dma((4 * NG,)), dma(()), dma((NG,)),
        *[vmem((2,) + tile, f32)] * 4,
    ]
    hbm = pl.BlockSpec(memory_space=pl.ANY)
    out = pl.pallas_call(
        _kernel,
        out_shape=jax.ShapeDtypeStruct((SEQ, D), bf16),
        in_specs=[hbm] * 5,
        out_specs=hbm,
        scratch_shapes=scratch,
        compiler_params=pltpu.CompilerParams(
            vmem_limit_bytes=127 * 1024 * 1024,
            disable_bounds_checks=True,
            flags={"XLA_TPU_FORCE_LP_LLO_SCHEDULER": True},
        ),
        name="interleaved_layers",
    )(A_x.reshape(SEQ, D), A_wqkv, A_wo, B_wqkv, B_wo)
    return out.reshape(1, SEQ, D)
```

```python
import math

import jax
import jax.numpy as jnp
from jax import lax
import jax.experimental.pallas as pl
import jax.experimental.pallas.tpu as pltpu

SEQ, D, HEADS, DH = 2048, 1024, 32, 32
WIN = 8
NT = SEQ // 128
NP = NT // 2
NQ = NT // 4
NG = D // 128
EPS = 1e-5
LOG2E = math.log2(math.e)
QSCALE = DH ** -0.5 * LOG2E
MASKED = -1e9 * LOG2E
ATT_UNROLL = 32
VPU_TILES = 4
DELAY = 16

bf16, f32, i32 = jnp.bfloat16, jnp.float32, jnp.int32


def _rows(i, n=128):
    return slice(i * n, (i + 1) * n)


def _words(x):
    return pltpu.bitcast(x.astype(bf16), i32)


def _halves(x):
    return pltpu.bitcast(x, bf16)


def _put(ref, idx, block, x):
    x = x.astype(bf16) if ref.dtype == bf16 else _words(x)
    n = x.shape[0]
    ref[(*idx, pl.ds(pl.multiple_of(block * n, n), n), slice(None))] = x


def _get(ref, *idx):
    return ref[idx] if ref.dtype == bf16 else _halves(ref[idx])


def _dot(a, b):
    return jnp.dot(a, b, preferred_element_type=f32)


def _slab_sum(x, acc=None):
    x = x if acc is None else jnp.concatenate([acc, x], axis=0)
    return jnp.sum(x.reshape(-1, 8, x.shape[1]), axis=0)


def _slab_max(x, acc=None):
    x = x if acc is None else jnp.concatenate([acc, x], axis=0)
    return jnp.max(x.reshape(-1, 8, x.shape[1]), axis=0)


def _inverse(x):
    r = pl.reciprocal(x, approx=True)
    return r * (2.0 - x * r)


def _after(x, *deps):
    low = x
    for dep in deps:
        if dep is not None:
            low = jnp.minimum(low, lax.bitcast_convert_type(dep, x.dtype))
    return x if low is x else jnp.maximum(x, low)


def _head_after(x, n, *deps):
    return jnp.concatenate([_after(x[:n], *deps), x[n:]], axis=0)


def _slab(mark):
    return mark and mark[0][_rows(mark[1], 8)]


LEFT = [((1, 0), 1, (1, 1)), ((1, 1),), ((0, 0), 1, (1, 1)), ((1, 0), -1, (0, 0)),
        ((0, 0),), ((0, 0), 1, (0, 1)), ((0, 1), -1, (1, 1))]
RIGHT = [((0, 0),), ((1, 0), -1, (0, 0)), ((0, 0), -1, (1, 1)), ((0, 0), -1, (0, 1)),
         ((0, 1), -1, (1, 1)), ((1, 1),), ((1, 0), -1, (1, 1))]


def _operand(term, block):
    if len(term) == 1:
        return block(*term[0])
    a, b = block(*term[0]).astype(f32), block(*term[2]).astype(f32)
    return a + b if term[1] > 0 else a - b


def _operands(side, block):
    grid = [[block(r, c) for c in range(2)] for r in range(2)]
    return [_operand(term, lambda r, c: grid[r][c]) for term in side]


def _inner_operands(side, e, block):
    return _operands(side, lambda r, c: _operand(side[e], lambda i, j: block(2 * i + r, 2 * j + c)))


def _project(w, i, right, first=0):
    ms = []
    for e in range(first, first + 7):
        a, b = _get(w, i, e), right(e)
        ms.append(_dot(jnp.concatenate(jnp.split(a, b.shape[0] // 128), axis=1), b))
    m2, m4, m1, m6, m3, m5, m7 = ms
    y1 = jnp.concatenate([m4 + m1 + m5 + m7, m2 + m4], axis=0)
    y2 = jnp.concatenate([m5 + m3, m2 - m1 - m6 + m3], axis=0)
    return (y1, y2), ms


def _marks(ms):
    return [(m, s) for m in ms for s in range(8)]


def _interleave(main, *sides, marks=None):
    done = [0] * len(sides)
    marks = marks or [None] * DELAY
    for i, step in enumerate(main):
        marks += step()
        total = (len(marks) - DELAY) * len(main) // (i + 1)
        for k, side in enumerate(sides):
            upto = (i + 1) * len(side) // len(main)
            for e in range(done[k], upto):
                if side[e] is not None:
                    side[e](_slab(marks[e * total // len(side)]))
            done[k] = upto
    return marks[-DELAY:]


def _run(steps):
    for step in steps:
        if step is not None:
            step(None)


def _moments(x):
    mean = _slab_sum(x) * (1.0 / 16)
    d = x - jnp.tile(mean, (16, 1))
    return jnp.concatenate([mean, _slab_sum(d * d)], axis=0)


def _stats_steps(tiles, moments):
    mean, rstd = [], []

    def step(n):
        def run(dep):
            part = moments(n)
            mu = jnp.sum(_head_after(part[:, :8], 1, dep), axis=0)
            mu = jnp.sum(mu, axis=0, keepdims=True) * (16.0 / D)
            d = part[:, :8] - mu
            var = jnp.sum(part[:, 8:], axis=0) + 16.0 * jnp.sum(d * d, axis=0)
            var = jnp.sum(var, axis=0, keepdims=True) * (1.0 / D)
            mean.append(jnp.broadcast_to(mu, (8, 128)))
            rstd.append(jnp.broadcast_to(lax.rsqrt(var + EPS), (8, 128)))
        return run

    return [step(n) for n in range(tiles)] + [None], mean, rstd


def _normalize(x, mean, rstd):
    reps = (x.shape[0] // 8, 1)
    return (x - jnp.tile(mean, reps)) * jnp.tile(rstd, reps)


def _kernel(x_hbm, wqa_hbm, woa_hbm, wqb_hbm, wob_hbm, out_hbm,
            xio, xw, wa, wb, wj, wot, wq2, wo2, wt, xa, xb, ha, oa, ho2,
            q0, q1, k0, k1, v0, v1, ol, y0, y1, n0, n1, ma, m0, m1,
            kk, vt, qb0, qb1, s0, s1, oq0, oq1, x_sem, a_sem, b_sem, o_sem, *sums):
    qbuf, kbuf, vbuf, oq = (q0, q1), (k0, k1), (v0, v1), (oq0, oq1)
    kb = (ha, oa)
    ybuf, normed, mbuf, qb, sbuf = (y0, y1), (n0, n1), (m0, m1), (qb0, qb1), (s0, s1)

    zeros, blocks = [], []

    def separately(body):
        blocks.append(body)
        pl.when(zeros[len(blocks)] == 0)(body)

    def cols(c):
        return pl.ds(pl.multiple_of(c * 128, 128), 128)

    def x_copy(c):
        return pltpu.make_async_copy(x_hbm.at[:, cols(c)], xio.at[c], x_sem.at[c])

    def out_copy(c):
        return pltpu.make_async_copy(xio.at[c], out_hbm.at[:, cols(c)], o_sem.at[c])

    def w_copies(qkv_hbm, o_hbm, dst, g, sem):
        srcs = [qkv_hbm.at[:, cols(i * NG + g)] for i in range(3)] + [o_hbm.at[:, cols(g)]]
        return [pltpu.make_async_copy(src, dst.at[4 * g + i], sem(i)) for i, src in enumerate(srcs)]

    def local_copies(g):
        return w_copies(wqa_hbm, woa_hbm, wa, g, lambda i: a_sem.at[4 * g + i])

    def full_copies(g):
        return w_copies(wqb_hbm, wob_hbm, wb, g, lambda i: b_sem)

    def quarters(copy):
        lax.fori_loop(0, 4, lambda i, _: copy(pl.ds(pl.multiple_of(i * 512, 512), 512),
                                              pl.ds(pl.multiple_of(i * 256, 256), 256)), None)

    def transposed(src, i, blocks, rows, dep):
        w = [src[i, _rows(b, rows), :] for b in blocks]
        w[0] = _halves(_head_after(_words(w[0]), 8, dep))
        return jnp.concatenate(w, axis=0).T

    def weight_steps(i, dst, j):
        def step(k):
            def run(dep):
                t = [transposed(wa, i, (4 * k + e, 4 * k + 2 + e), 64, None if e else dep)
                     for e in range(2)]
                for e, a in enumerate(_operands(LEFT, lambda r, c: t[c][_rows(r, 64)])):
                    _put(dst, (j, e), k, a)
            return run
        return [step(k) for k in range(4)]

    def weight2_steps(i, dst, j):
        def flip(k, r, c):
            def run(dep):
                for e in (c, c + 1):
                    wt[4 * k + e, _rows(r, 64), :] = _words(transposed(
                        wb, i + 4 * r, range(16 * k + e, 16 * k + 16, 4), 32, None if e > c else dep))
            return run

        def step(k, s, e):
            def run(dep):
                def block(r, c):
                    x = _halves(wt[4 * k + c + zeros[e], _rows(4 * r + s, 8), :]).astype(f32)
                    return _head_after(x, 8, dep) if r % 2 == c % 2 else x

                for n, a in enumerate(_inner_operands(LEFT, e, block)):
                    _put(dst, (j, 7 * e + n), 4 * k + s, a)
            return run
        return ([flip(k, r, c) for k in range(2) for r in range(2) for c in (0, 2)] + [None] * 6
                + [step(k, s, e) for k in range(2) for s in range(4) for e in range(7)])

    def project2_steps(w, i, j, emit):
        def step(e):
            def run():
                ys, ms = _project(w, i, lambda k: ho2[j, k], 7 * e)
                m = jnp.stack(ys)

                def held(k):
                    return sums[k][pl.ds(zeros[e], 2)]

                if e == 0:
                    sums[0][...] = m
                elif e == 1:
                    emit(1, 0, held(0) + m)
                    sums[1][...] = m
                elif e == 2:
                    sums[2][...] = held(0) - m
                    sums[3][...] = held(1) + m
                elif e == 3:
                    sums[0][...] = held(2) - m
                elif e == 4:
                    emit(1, 1, held(0) + m)
                    sums[1][...] = m
                elif e == 5:
                    emit(0, 1, held(1) + m)
                    sums[2][...] = held(3) + m
                else:
                    emit(0, 0, held(2) + m)
                return [(ms[min(s // 8 * 2 + e % 2, 6)], s % 8) for s in range(28)]
            return run
        return [step(e) for e in range(7)]

    def local_tile(j, n):
        return 4 * (j & 3) + 2 * n + (j >> 2)

    def local_qkv_steps(par, first=False):
        def put(buf, i, y):
            for h in range(4):
                buf[i, pl.ds(h, DH, stride=4), :] = y[_rows(h, DH)]

        def step(j, i):
            def run():
                pair = par * (NP // 2) + j

                def right(e):
                    if not first:
                        return _get(ha, pair, e)
                    quad, slot = parked(pair, e)
                    b = ho2[quad, pl.ds(slot, 2)].reshape(D // 2, 128)
                    if e % 3 == i:
                        _put(ha, (pair, e), 0, b)
                    return b

                ys, ms = _project(wj, i, right)
                for r, y in zip((2 * j, 2 * j + 1), ys):
                    if i == 0:
                        put(qbuf[par], r, y)
                        continue
                    buf = kbuf[par] if i == 1 else vbuf[par]
                    put(buf, r + WIN - 1, y)
                    if r > 0:
                        put(buf, r - 1, pltpu.roll(y, 1, 1))
                return _marks(ms)
            return run
        return [step(j, i) for i in (1, 2, 0) for j in range(NP // 2)]

    def local_att_steps(g, par):
        def tile_steps(r):
            logits, probs = [], []

            def score(i):
                def run(dep):
                    q = _head_after(qbuf[par][r + zeros[i]], 8, dep, *logits[-1:])
                    for w in (i, i + 1):
                        s = _slab_sum(q * kbuf[par][r + w + zeros[r]])
                        logits.append(s + pltpu.roll(s, 4, 0))
                return run

            def softmax(dep):
                s = jnp.concatenate(logits, axis=0) * QSCALE
                if r < WIN - 1:
                    wrapped = 8 * (WIN - 1 - r)
                    first = lax.broadcasted_iota(i32, (wrapped, 128), 1) == 0
                    s = jnp.concatenate([jnp.where(first, MASKED, s[:wrapped]), s[wrapped:]], axis=0)
                s = s.reshape(WIN, 8, 128)
                p = jnp.exp2(s - jnp.max(s, axis=0))
                probs.append(p * _inverse(jnp.sum(p, axis=0)))

            def mix(i):
                def run(dep):
                    p = _head_after(probs[0], 1, dep)
                    v = vbuf[par][pl.ds(r + zeros[r], WIN), _rows(i, 16), :]
                    ol[r % 2, _rows(i, 16), :] = jnp.sum(jnp.concatenate([p, p], axis=1) * v, axis=0)
                return run

            return ([s for i in range(0, WIN, 2) for s in (score(i), None)] + [softmax, None]
                    + [mix(i) for i in range(8)])

        def operands(j, i):
            def run(dep):
                def block(e, n):
                    x = ol[n + zeros[0], pl.ds(64 * (i % 2) + i // 2 + 2 * e, 16, stride=4), :]
                    return _head_after(x, 8, dep) if e == n else x

                for e, b in enumerate(_operands(RIGHT, block)):
                    _put(oa, (par * (NP // 2) + j, e), 4 * g + i, b)
            return run

        return [s for j in range(NP // 2) for s in tile_steps(2 * j) + tile_steps(2 * j + 1)
                + [operands(j, i) for i in range(4)]]

    def parked(j, e):
        return j // 2, 14 * (j % 2) + 2 * e

    def input_ln_steps(j):
        stats, mean, rstd = _stats_steps(2, lambda n: ma[local_tile(j, n)])
        last = []

        def step(c, i):
            def run(dep):
                prev = last.pop() if last else rstd[1]
                dep = prev if dep is None else jnp.minimum(dep, prev)
                mu = [_after(m, dep) for m in mean]
                ops = _operands(RIGHT, lambda k, n: _normalize(
                    xa[local_tile(j, n), c, _rows(4 * k + i, 16), :], mu[n], rstd[n]))
                for e, b in enumerate(ops):
                    quad, slot = parked(j, e)
                    _put(ho2, (quad, slot + c // 4), 4 * (c % 4) + i, b)
                last.append(ops[2][:8])
            return run
        return stats + [step(c, i) for c in range(NG) for i in range(4)]

    def proj_steps(quad):
        def step(j, c):
            def run():
                ys, ms = _project(wot, c, lambda e: _get(oa, j, e))
                for n in range(2):
                    y = xa[local_tile(j, n), c] + ys[n]
                    xb[local_tile(j, n), c] = y
                    ybuf[quad % 2][j % 2 * 2 + n, c] = y
                    mbuf[quad % 2][j % 2 * 2 + n, c] = _moments(y)
                return _marks(ms)
            return run
        return [step(j, c) for j in (2 * quad, 2 * quad + 1) for c in range(NG)]

    def quad_operands(quad, block_index, e, load, dep):
        def block(r, c):
            return _head_after(load(r, c), 8, dep) if r % 2 == c % 2 else load(r, c)

        ops = _inner_operands(RIGHT, e, block)
        for k, b in enumerate(ops):
            _put(ho2, (quad, 7 * e + k), block_index, b)
        return ops[2][:8]

    def proj_ln_steps(quad):
        stats, mean, rstd = _stats_steps(4, lambda n: mbuf[quad % 2][n + zeros[0]])

        def norm(c, n):
            def run(dep):
                normed[c % 2][n] = _normalize(ybuf[quad % 2][n + zeros[0], c],
                                              _after(mean[n], dep), rstd[n])
            return run

        def step(c, i, e):
            return lambda dep: quad_operands(
                quad, 2 * c + i, e,
                lambda k, n: normed[c % 2][n + zeros[e], _rows(2 * k + i, 16), :], dep)

        return stats + [s for c in range(NG) for s in [norm(c, n) for n in range(4)]
                        + [step(c, i, e) for i in range(2) for e in range(7)]]

    def local_layer(rep):
        def fetch_weights(g):
            @pl.when(rep == 0)
            def _():
                @pl.when(g + 1 < NG)
                def _():
                    for cp in local_copies(g + 1):
                        cp.wait()

                @pl.when(g + 2 < NG)
                def _():
                    for cp in local_copies(g + 2):
                        cp.start()

                for cp in full_copies(g):
                    cp.start()

        def w_steps(g):
            nxt = 4 * ((g + 1) & (NG - 1))
            return (weight_steps(4 * g, wj, 0) + [None] * 4
                    + weight_steps(4 * g + 3, wot, g) + [None] * 4
                    + weight_steps(nxt + 1, wj, 1) + weight_steps(nxt + 2, wj, 2))

        ln = [input_ln_steps(j) for j in range(NP)]
        even, odd, first = local_qkv_steps(0, True), local_qkv_steps(1, True), w_steps(0)
        _run(ln[0])
        marks = _interleave(even[0::4], [None] * 8 + ln[1] + [None] * 6, first[:4] + [None] * 3)
        marks = _interleave(even[1::4], ln[2] + ln[4][:18], marks=marks)
        marks = _interleave(even[2::4], ln[3] + ln[4][18:], marks=marks)
        _interleave(even[3::4], ln[5] + ln[6], marks=marks)
        fetch_weights(0)
        att = local_att_steps(0, 0)
        marks = _interleave(odd[:2], ln[7], att[:16])
        _interleave(odd[2:], att[16:],
                    first[8:10] + first[16:20] + first[10:12] + first[20:] + [None], marks=marks)

        def group(g, _):
            fetch_weights(g)
            _interleave(local_qkv_steps(0) + local_qkv_steps(1),
                        local_att_steps(g - 1, 1) + local_att_steps(g, 0), w_steps(g))

        lax.fori_loop(1, NG, group, None)

        @pl.when(rep == 0)
        def _():
            pltpu.make_async_copy(wb, wb, b_sem).wait()

    def full_qkv_steps(gp, i, slot=None):
        def steps(quad):
            def emit(r, c, ys):
                for n in range(2):
                    g, kt = 2 * gp + r, 4 * quad + 2 * c + n
                    if i == 0:
                        xa[local_tile(2 * quad + c, n), g] = ys[n] * QSCALE
                    elif i == 1:
                        kk[g, kt] = _words(ys[n].astype(bf16).T)
                    else:
                        vt[g, kt] = _words(ys[n])
            return project2_steps(wq2, i if slot is None else slot, quad, emit)
        return [s for quad in range(NQ) for s in steps(quad)]

    def spread_steps(g):
        def step(kt, e):
            def run(dep):
                k = _after(kk[g + zeros[e % 8], kt, 56:, :], dep)
                for f in range(4 * e, 4 * e + 4):
                    h, d = divmod(f, DH)
                    x = _halves(jnp.broadcast_to(k[:, f:f + 1], (8, 128))).astype(f32)
                    x = lax.bitcast_convert_type(x, i32).reshape(2, 8, 128)
                    kb[h // 2][g, pl.ds(h % 2 * 8 + 2 * kt, 2), _rows(d, 8), :] = x
            return run
        return [step(kt, e) for kt in range(VPU_TILES) for e in range(32)]

    def full_qkv(gp, more):
        pad = [None] * 3
        v_w, out_w = weight2_steps(8 * gp + 2, wq2, 2), weight2_steps(8 * gp + 3, wo2, gp)
        spread = [spread_steps(2 * gp + r) + pad for r in range(2)]
        if more:
            marks = _interleave(full_qkv_steps(gp + 1, 1), v_w + out_w)
            marks = _interleave(full_qkv_steps(gp, 0),
                                weight2_steps((8 * gp + 17) & (4 * NG - 1), wq2, 1),
                                [None] * 28 + spread[0], marks=marks)
            _interleave(full_qkv_steps(gp, 2), weight2_steps(8 * gp + 8, wq2, 0) + pad,
                        [None] * 28 + spread[1], marks=marks)
        else:
            marks = _interleave(full_qkv_steps(gp, 0), v_w + pad, [None] * 28 + spread[0])
            _interleave(full_qkv_steps(gp, 2), out_w + pad, [None] * 28 + spread[1], marks=marks)

    def full_att(base, count, state, first=False, last=False):
        def item(u):
            return base + u // 16, u % 4, u % 16 // 4

        def operands(blk, slot, step, dep):
            i, e = divmod(step, 7)
            return quad_operands(
                blk & 3, 2 * (blk >> 2) + i, e,
                lambda r, c: oq[slot % 2][4 * r + c + zeros[e], _rows(i, 16), :], dep)

        def fetch_q(u, marks):
            blk, n, h = item(u)
            q = xa[4 * (blk & 3) + n, blk >> 2, _rows(h, DH), :]
            for i in range(4):
                rows = _after(q[_rows(i, 8)], marks and _slab(marks[28 + 3 * i]))
                for d in range(8):
                    qb[u % 2][0, _rows(8 * i + d, 8), :] = jnp.broadcast_to(rows[d:d + 1], (8, 128))
            return q

        m, m_next, den, acc, q_next = state or (None,) * 4 + (fetch_q(0, None),)
        for u in range(count + (2 if last else 0)):
            scores = u < count
            if scores:
                blk, n, h = item(u)
                parts = [jnp.zeros((DH, 128), f32)] * 4
                parts[h] = q_next
                q = jnp.concatenate(parts, axis=0).astype(bf16)
                top, marks = None, []
            for c in range(4):
                if scores:
                    for kt in range(4 * c, 4 * c + 4):
                        keys = 112 if kt < VPU_TILES else 128
                        s = _dot(_halves(kk[blk >> 2, kt, :keys // 2, :]), q)
                        sbuf[u % 2][128 * kt:128 * kt + keys, :] = s
                        top = _slab_max(s, top)
                    marks += [(s, i) for i in range(14)]
                up, cp = divmod(4 * (u - 1) + c - 2, 4)
                if (first and up < 0) or up >= count:
                    continue
                if cp == 0:
                    m, den, acc = m_next, None, None
                blkp, _, hp = item(up)
                for kt in range(4 * cp, 4 * cp + 4):
                    p = jnp.exp2(sbuf[up % 2][_rows(kt), :] - m)
                    den = _slab_sum(p, den)
                    o = _dot(_halves(vt[blkp >> 2, kt, _rows(hp, DH // 2), :]), p)
                    acc = o if acc is None else acc + o
                if cp == 3:
                    o = acc * _inverse(jnp.sum(den, axis=0, keepdims=True))
                    oq[(up // 16 + first) % 2][up % 16] = o
                if up % 16 < 4 and not (first and up < 16) and 4 * (up % 16) + cp < 14:
                    operands(blkp - 1, up // 16 - 1, 4 * (up % 16) + cp, _slab(marks[-1]))
            if scores:
                s = None
                for e in range(2 * VPU_TILES):
                    qd = _head_after(qb[u % 2][zeros[e]], 8, _slab(marks[7 * e]), s)
                    kd = kb[h // 2][(blk >> 2) + zeros[u % 8], h % 2 * 8 + e]
                    s = _slab_sum(lax.bitcast_convert_type(kd, f32) * qd)
                    sbuf[u % 2][pl.ds(128 * (e // 2) + 112 + 8 * (e % 2), 8), :] = s
                    top = jnp.maximum(top, s)
                m_next = jnp.max(top, axis=0, keepdims=True)
                if not (last and u + 1 == count):
                    q_next = fetch_q(u + 1, marks)
        if last:
            dep = None
            for step in range(14):
                dep = operands(base + count // 16 - 1, count // 16 - 1, step, dep)
        return m, m_next, den, acc, q_next

    def full_layer(rep):
        @separately
        def _():
            marks = _interleave(proj_steps(0), local_att_steps(NG - 1, 1))
            _interleave(proj_steps(1), [None] * 6 + proj_ln_steps(0),
                        weight2_steps(1, wq2, 2) + [None], marks=marks)

        @separately
        def _():
            marks = _interleave(proj_steps(2), proj_ln_steps(1), weight2_steps(9, wq2, 1))
            marks = _interleave(proj_steps(3), [None] * 6 + proj_ln_steps(2),
                                weight2_steps(0, wq2, 0), marks=marks)
            _interleave(full_qkv_steps(0, 1, slot=2),
                        [None] * 6 + proj_ln_steps(3) + [None] * 56, marks=marks)
        lax.fori_loop(0, NG // 2 - 1, lambda gp, _: full_qkv(gp, True), None)
        separately(lambda: full_qkv(NG // 2 - 1, False))

        items = HEADS * NT
        head = ATT_UNROLL // 2
        state = full_att(0, head, None, first=True)
        state = lax.fori_loop(
            0, items // ATT_UNROLL - 1,
            lambda j, st: full_att(head // 16 + j * (ATT_UNROLL // 16), ATT_UNROLL, st), state)
        full_att((items - ATT_UNROLL + head) // 16, ATT_UNROLL - head, state, last=True)

        def proj(i, _):
            late = []

            def steps(quad):
                def emit(r, c, ys):
                    bits = []
                    for n in range(2):
                        t = 4 * quad + 2 * c + n
                        y = xb[t, 2 * i + r] + ys[n]
                        xa[t, 2 * i + r] = y
                        ma[t, 2 * i + r] = _moments(y)
                        bits.append(lax.bitcast_convert_type(y.astype(bf16).astype(f32), i32))
                    pair = lax.shift_right_logical(bits[0], 16) | bits[1]
                    if (quad, r, c) == (NQ - 1, 0, 0):
                        late.append(pair)
                    else:
                        xw[r, pl.ds(2 * quad + c, 128, stride=NP), :] = pair.T
                return project2_steps(wo2, i, quad, emit)

            _interleave([s for quad in range(NQ) for s in steps(quad)])

            @pl.when(rep == 1)
            def _():
                xw[0, pl.ds(NP - 2, 128, stride=NP), :] = late[0].T
                for r in (1, 0):
                    @quarters
                    def _(rows, words):
                        xio[2 * i + r, rows, :] = _halves(xw[r, words, :]).astype(f32).astype(bf16)

                    out_copy(2 * i + r).start()

        lax.fori_loop(0, NG // 2, proj, None)

    first_w = local_copies(0)
    for cp in first_w[1:3] + [x_copy(0)]:
        cp.start()
    for i in (1, 2):
        first_w[i].wait()
        x_copy(i).start()
        _run(weight_steps(i, wj, i))

    def stage_in(c, _):
        x_copy(c).wait()

        @pl.when(c + 3 < NG)
        def _():
            x_copy(c + 3).start()

        @pl.when(c + 2 == NG)
        def _():
            for cp in first_w[::3]:
                cp.start()

        @quarters
        def _(rows, words):
            xw[0, words, :] = _words(xio[c, rows, :])

        for j in range(NP):
            pair = xw[0, pl.ds(j, 128, stride=NP), :].T
            for n, bits in enumerate((pair << 16, pair & -65536)):
                y = lax.bitcast_convert_type(bits, f32)
                xa[2 * j + n, c] = y
                ma[2 * j + n, c] = _moments(y)

    lax.fori_loop(0, NG, stage_in, None)
    for cp in local_copies(1):
        cp.start()
    for cp in first_w[::3]:
        cp.wait()

    def two_layers(rep, _):
        zeros[:] = [(rep + i) >> 4 for i in range(8)]
        local_layer(rep)
        full_layer(rep)

    lax.fori_loop(0, 2, two_layers, None)
    for c in range(NG):
        out_copy(c).wait()


@jax.jit
def pallas_interleave_layers__sliding_local_dilated__softmax_full_mha__prompt_kernel(
    A_x: jax.Array,
    A_wqkv: jax.Array,
    A_wo: jax.Array,
    B_x: jax.Array,
    B_wqkv: jax.Array,
    B_wo: jax.Array,
):
    del B_x
    assert A_x.shape == (1, SEQ, D) and A_x.dtype == bf16
    vmem, dma = pltpu.VMEM, pltpu.SemaphoreType.DMA
    tile, words = (128, 128), (64, 128)
    scratch = [
        vmem((NG, SEQ, 128), bf16),
        vmem((2, SEQ // 2, 128), i32),
        *[vmem((4 * NG, D, 128), bf16)] * 2,
        vmem((3, 7, D // 8, 128), i32),
        vmem((NG, 7, D // 8, 128), i32),
        vmem((3, 49) + tile, bf16),
        vmem((NG // 2, 49) + tile, bf16),
        vmem((8,) + tile, i32),
        *[vmem((NT, NG) + tile, f32)] * 2,
        *[vmem((NP, 16, D // 4, 128), i32)] * 2,
        vmem((NQ, 49, D // 4, 128), bf16),
        *[vmem((WIN,) + tile, f32)] * 2,
        *[vmem((2 * WIN - 1,) + tile, f32)] * 4,
        vmem((2,) + tile, f32),
        *[vmem((4, NG) + tile, f32)] * 2,
        *[vmem((4,) + tile, f32)] * 2,
        vmem((NT, NG, 16, 128), f32),
        *[vmem((4, NG, 16, 128), f32)] * 2,
        *[vmem((NG, NT) + words, i32)] * 2,
        *[vmem((1, DH * 8, 128), f32)] * 2,
        *[vmem((SEQ, 128), f32)] * 2,
        *[vmem((16, DH, 128), f32)] * 2,
        dma((NG,)), dma((4 * NG,)), dma(()), dma((NG,)),
        *[vmem((2,) + tile, f32)] * 4,
    ]
    hbm = pl.BlockSpec(memory_space=pl.ANY)
    out = pl.pallas_call(
        _kernel,
        out_shape=jax.ShapeDtypeStruct((SEQ, D), bf16),
        in_specs=[hbm] * 5,
        out_specs=hbm,
        scratch_shapes=scratch,
        compiler_params=pltpu.CompilerParams(
            vmem_limit_bytes=127 * 1024 * 1024,
            disable_bounds_checks=True,
            flags={"XLA_TPU_FORCE_LP_LLO_SCHEDULER": True},
        ),
        name="interleaved_layers",
    )(A_x.reshape(SEQ, D), A_wqkv, A_wo, B_wqkv, B_wo)
    return out.reshape(1, SEQ, D)
```

```python
import math

import jax
import jax.numpy as jnp
from jax import lax
import jax.experimental.pallas as pl
import jax.experimental.pallas.tpu as pltpu

SEQ, D, HEADS, DH = 2048, 1024, 32, 32
WIN = 8
NT = SEQ // 128
NP = NT // 2
NQ = NT // 4
NG = D // 128
EPS = 1e-5
LOG2E = math.log2(math.e)
QSCALE = DH ** -0.5 * LOG2E
MASKED = -1e9 * LOG2E
ATT_UNROLL = 32
VPU_TILES = 4
DELAY = 16

bf16, f32, i32 = jnp.bfloat16, jnp.float32, jnp.int32


def _rows(i, n=128):
    return slice(i * n, (i + 1) * n)


def _words(x):
    return pltpu.bitcast(x.astype(bf16), i32)


def _halves(x):
    return pltpu.bitcast(x, bf16)


def _put(ref, i, first, block, xs):
    x = jnp.stack([x.astype(bf16) for x in xs] if len({x.dtype for x in xs}) > 1 else xs)
    x = x.astype(bf16) if ref.dtype == bf16 else _words(x)
    n = x.shape[1]
    start = block * n if isinstance(block, int) else pl.multiple_of(block * n, n)
    ref[i, first:first + len(xs), pl.ds(start, n), :] = x


def _get(ref, *idx):
    return ref[idx] if ref.dtype == bf16 else _halves(ref[idx])


def _dot(a, b):
    return jnp.dot(a, b, preferred_element_type=f32)


def _slab_sum(x, acc=None):
    x = x if acc is None else jnp.concatenate([acc, x], axis=0)
    return jnp.sum(x.reshape(-1, 8, x.shape[1]), axis=0)


def _slab_max(x, acc=None):
    x = x if acc is None else jnp.concatenate([acc, x], axis=0)
    return jnp.max(x.reshape(-1, 8, x.shape[1]), axis=0)


def _inverse(x):
    r = pl.reciprocal(x, approx=True)
    return r * (2.0 - x * r)


def _after(x, *deps):
    low = x
    for dep in deps:
        if dep is not None:
            same = dep.dtype == x.dtype
            low = jnp.minimum(low, dep if same else lax.bitcast_convert_type(dep, x.dtype))
    return x if low is x else jnp.maximum(x, low)


def _head_after(x, n, *deps):
    return jnp.concatenate([_after(x[:n], *deps), x[n:]], axis=0)


def _slab(mark):
    return mark and mark[0][_rows(mark[1], 8)]


LEFT = [((1, 0), 1, (1, 1)), ((1, 1),), ((0, 0), 1, (1, 1)), ((1, 0), -1, (0, 0)),
        ((0, 0),), ((0, 0), 1, (0, 1)), ((0, 1), -1, (1, 1))]
RIGHT = [((0, 0),), ((1, 0), -1, (0, 0)), ((0, 0), -1, (1, 1)), ((0, 0), -1, (0, 1)),
         ((0, 1), -1, (1, 1)), ((1, 1),), ((1, 0), -1, (1, 1))]


def _operand(term, block):
    if len(term) == 1:
        return block(*term[0])
    a, b = block(*term[0]).astype(f32), block(*term[2]).astype(f32)
    return a + b if term[1] > 0 else a - b


def _operands(side, block):
    grid = [[block(r, c) for c in range(2)] for r in range(2)]
    return [_operand(term, lambda r, c: grid[r][c]) for term in side]


def _inner_operands(side, e, block, dep):
    x = _operand(side[e], block)
    x = jnp.concatenate([_after(x[:, :, :8], dep), x[:, :, 8:]], axis=2)
    return _operands(side, lambda r, c: x[r, c])


def _project(w, i, right, first=0):
    ms = []
    for e in range(first, first + 7):
        a, b = _get(w, i, e), right(e)
        ms.append(_dot(jnp.concatenate(jnp.split(a, b.shape[0] // 128), axis=1), b))
    m2, m4, m1, m6, m3, m5, m7 = ms
    y1 = jnp.concatenate([m4 + m1 + m5 + m7, m2 + m4], axis=0)
    y2 = jnp.concatenate([m5 + m3, m2 - m1 - m6 + m3], axis=0)
    return (y1, y2), ms


def _marks(ms):
    return [(m, s) for m in ms for s in range(8)]


def _interleave(main, *sides, marks=None):
    done = [0] * len(sides)
    marks = marks or [None] * DELAY
    for i, step in enumerate(main):
        marks += step()
        total = (len(marks) - DELAY) * len(main) // (i + 1)
        for k, side in enumerate(sides):
            upto = (i + 1) * len(side) // len(main)
            for e in range(done[k], upto):
                if side[e] is not None:
                    side[e](_slab(marks[e * total // len(side)]))
            done[k] = upto
    return marks[-DELAY:]


def _run(steps):
    for step in steps:
        if step is not None:
            step(None)


def _moments(x):
    mean = _slab_sum(x) * (1.0 / 16)
    d = x - jnp.tile(mean, (16, 1))
    return jnp.concatenate([mean, _slab_sum(d * d)], axis=0)


def _stats_steps(tiles, moments):
    mean, rstd = [], []

    def step(n):
        def run(dep):
            part = moments(n)
            mu = jnp.sum(_head_after(part[:, :8], 1, dep), axis=0)
            mu = jnp.sum(mu, axis=0, keepdims=True) * (16.0 / D)
            d = part[:, :8] - mu
            var = jnp.sum(part[:, 8:], axis=0) + 16.0 * jnp.sum(d * d, axis=0)
            var = jnp.sum(var, axis=0, keepdims=True) * (1.0 / D)
            mean.append(jnp.broadcast_to(mu, (8, 128)))
            rstd.append(jnp.broadcast_to(lax.rsqrt(var + EPS), (8, 128)))
        return run

    return [step(n) for n in range(tiles)] + [None], mean, rstd


def _normalize(x, mean, rstd):
    reps = (x.shape[0] // 8, 1)
    return (x - jnp.tile(mean, reps)) * jnp.tile(rstd, reps)


def _kernel(x_hbm, wqa_hbm, woa_hbm, wqb_hbm, wob_hbm, out_hbm,
            xio, xw, wa, wb, wj, wot, wq2, wo2, wt, xa, xb, ha, oa, ho2,
            q0, q1, k0, k1, v0, v1, ol, y0, y1, ma, m0, m1,
            kk, vt, qb0, qb1, s0, s1, oq0, oq1, x_sem, a_sem, b_sem, o_sem, *sums):
    qbuf, kbuf, vbuf, oq = (q0, q1), (k0, k1), (v0, v1), (oq0, oq1)
    kb = (ha, oa)
    ybuf, mbuf, qb, sbuf = (y0, y1), (m0, m1), (qb0, qb1), (s0, s1)

    zeros, blocks = [], []

    def separately(body):
        blocks.append(body)
        pl.when(zeros[len(blocks)] == 0)(body)

    def cols(c):
        return pl.ds(pl.multiple_of(c * 128, 128), 128)

    def x_copy(c):
        return pltpu.make_async_copy(x_hbm.at[:, cols(c)], xio.at[c], x_sem.at[c])

    def out_copy(c):
        return pltpu.make_async_copy(xio.at[c], out_hbm.at[:, cols(c)], o_sem.at[c])

    def w_copies(qkv_hbm, o_hbm, dst, g, sem):
        srcs = [qkv_hbm.at[:, cols(i * NG + g)] for i in range(3)] + [o_hbm.at[:, cols(g)]]
        return [pltpu.make_async_copy(src, dst.at[4 * g + i], sem(i)) for i, src in enumerate(srcs)]

    def local_copies(g):
        return w_copies(wqa_hbm, woa_hbm, wa, g, lambda i: a_sem.at[4 * g + i])

    def full_copies(g):
        return w_copies(wqb_hbm, wob_hbm, wb, g, lambda i: b_sem)

    def quarters(copy):
        lax.fori_loop(0, 4, lambda i, _: copy(pl.ds(pl.multiple_of(i * 512, 512), 512),
                                              pl.ds(pl.multiple_of(i * 256, 256), 256)), None)

    def transposed(src, i, blocks, rows, dep):
        w = [src[i, _rows(b, rows), :] for b in blocks]
        w[0] = _halves(_head_after(_words(w[0]), 8, dep))
        return jnp.concatenate(w, axis=0).T

    def weight_steps(i, dst, j):
        def step(k):
            def run(dep):
                t = [transposed(wa, i, (4 * k + e, 4 * k + 2 + e), 64, None if e else dep)
                     for e in range(2)]
                _put(dst, j, 0, k, _operands(LEFT, lambda r, c: t[c][_rows(r, 64)]))
            return run
        return [step(k) for k in range(4)]

    def weight2_steps(i, dst, j):
        def flip(k, r, c):
            def run(dep):
                for e in (c, c + 1):
                    t = transposed(wb, i + 4 * r, range(16 * k + e, 16 * k + 16, 4), 32,
                                   None if e > c else dep)
                    wt[k, _rows(r, 2), e] = _words(t).reshape(2, 32, 128)
            return run

        def step(k, s, e):
            def run(dep):
                def block(r, c):
                    x = wt[k + zeros[e], _rows(r, 2), _rows(c, 2), _rows(s, 8), :]
                    return _halves(x).astype(f32)

                _put(dst, j, 7 * e, 4 * k + s, _inner_operands(LEFT, e, block, dep))
            return run
        return ([flip(k, r, c) for k in range(2) for r in range(2) for c in (0, 2)] + [None] * 6
                + [step(k, s, e) for k in range(2) for s in range(4) for e in range(7)])

    def project2_steps(w, i, j, emit):
        def step(e):
            def run():
                ys, ms = _project(w, i, lambda k: ho2[j, k], 7 * e)
                m = jnp.stack(ys)

                def held(k):
                    return sums[k][pl.ds(zeros[e], 2)]

                if e == 0:
                    sums[0][...] = m
                elif e == 1:
                    emit(1, 0, held(0) + m)
                    sums[1][...] = m
                elif e == 2:
                    sums[2][...] = held(0) - m
                    sums[3][...] = held(1) + m
                elif e == 3:
                    sums[0][...] = held(2) - m
                elif e == 4:
                    emit(1, 1, held(0) + m)
                    sums[1][...] = m
                elif e == 5:
                    emit(0, 1, held(1) + m)
                    sums[2][...] = held(3) + m
                else:
                    emit(0, 0, held(2) + m)
                return [(ms[min(s // 8 * 2 + e % 2, 6)], s % 8) for s in range(28)]
            return run
        return [step(e) for e in range(7)]

    def local_tile(j, n):
        return 4 * (j & 3) + 2 * n + (j >> 2)

    def local_qkv_steps(par, first=False):
        def put(buf, i, y):
            for h in range(4):
                buf[i, pl.ds(h, DH, stride=4), :] = y[_rows(h, DH)]

        def step(j, i):
            def run():
                pair = par * (NP // 2) + j

                def right(e):
                    if not first:
                        return _get(ha, pair, e)
                    b = jnp.concatenate([ho2[pair // 2, 14 * (pair % 2) + 7 * k + e]
                                         for k in range(2)], axis=0)
                    if e % 3 == i:
                        ha[pair, e] = _words(b)
                    return b

                ys, ms = _project(wj, i, right)
                for r, y in zip((2 * j, 2 * j + 1), ys):
                    if i == 0:
                        put(qbuf[par], r, y)
                        continue
                    buf = kbuf[par] if i == 1 else vbuf[par]
                    put(buf, r + WIN - 1, y)
                    if r > 0:
                        put(buf, r - 1, pltpu.roll(y, 1, 1))
                return _marks(ms)
            return run
        return [step(j, i) for i in (1, 2, 0) for j in range(NP // 2)]

    def local_att_steps(g, par):
        def tile_steps(r):
            logits, probs = [], []

            def score(i):
                def run(dep):
                    q = _head_after(qbuf[par][r + zeros[i]], 8, dep, *logits[-1:])
                    for w in (i, i + 1):
                        s = _slab_sum(q * kbuf[par][r + w + zeros[r]])
                        logits.append(s + pltpu.roll(s, 4, 0))
                return run

            def softmax(dep):
                s = jnp.concatenate(logits, axis=0) * QSCALE
                if r < WIN - 1:
                    wrapped = 8 * (WIN - 1 - r)
                    first = lax.broadcasted_iota(i32, (wrapped, 128), 1) == 0
                    s = jnp.concatenate([jnp.where(first, MASKED, s[:wrapped]), s[wrapped:]], axis=0)
                s = s.reshape(WIN, 8, 128)
                p = jnp.exp2(s - jnp.max(s, axis=0))
                probs.append(p * _inverse(jnp.sum(p, axis=0)))

            def mix(i):
                def run(dep):
                    p = _head_after(probs[0], 1, dep)
                    v = vbuf[par][pl.ds(r + zeros[r], WIN), _rows(i, 16), :]
                    ol[r % 2, _rows(i, 16), :] = jnp.sum(jnp.concatenate([p, p], axis=1) * v, axis=0)
                return run

            return ([s for i in range(0, WIN, 2) for s in (score(i), None)] + [softmax, None]
                    + [mix(i) for i in range(8)])

        def operands(j, i):
            def run(dep):
                def block(e, n):
                    x = ol[n + zeros[0], pl.ds(64 * (i % 2) + i // 2 + 2 * e, 16, stride=4), :]
                    return _head_after(x, 8, dep) if e == n else x

                _put(oa, par * (NP // 2) + j, 0, 4 * g + i, _operands(RIGHT, block))
            return run

        return [s for j in range(NP // 2) for s in tile_steps(2 * j) + tile_steps(2 * j + 1)
                + [operands(j, i) for i in range(4)]]

    def input_ln_steps(j):
        stats, mean, rstd = _stats_steps(2, lambda n: ma[local_tile(j, n)])
        last = []

        def step(c, i):
            def run(dep):
                prev = last.pop() if last else rstd[1]
                dep = prev if dep is None else jnp.minimum(dep, prev)
                mu = [_after(m, dep) for m in mean]
                ops = _operands(RIGHT, lambda k, n: _normalize(
                    xa[local_tile(j, n), c, _rows(4 * k + i, 16), :], mu[n], rstd[n]))
                _put(ho2, j // 2, 14 * (j % 2) + 7 * (c // 4), 4 * (c % 4) + i, ops)
                last.append(ops[2][:8])
            return run
        return stats + [step(c, i) for c in range(NG) for i in range(4)]

    def proj_steps(quad):
        def step(j, c):
            def run():
                ys, ms = _project(wot, c, lambda e: _get(oa, j, e))
                for n in range(2):
                    y = xa[local_tile(j, n), c] + ys[n]
                    xb[local_tile(j, n), c] = y
                    ybuf[quad % 2][j % 2 * 2 + n, c] = y
                    mbuf[quad % 2][j % 2 * 2 + n, c] = _moments(y)
                return _marks(ms)
            return run
        return [step(j, c) for j in (2 * quad, 2 * quad + 1) for c in range(NG)]

    def quad_operands(src, quad, c, step, dep):
        i, e = divmod(step, 7)
        ops = _inner_operands(
            RIGHT, e, lambda k, n: src[zeros[e], _rows(k, 2), _rows(n, 2), _rows(i, 16), :], dep)
        _put(ho2, quad, 7 * e, 2 * c + i, ops)
        return ops[2][:8]

    def proj_ln_steps(quad):
        stats, mean, rstd = _stats_steps(4, lambda n: mbuf[quad % 2][n + zeros[0]])

        def norm(c, n):
            def run(dep):
                h = _normalize(ybuf[quad % 2][n + zeros[0], c], _after(mean[n], dep), rstd[n])
                oq[c % 2][0, :, n] = h.reshape(4, DH, 128)
            return run

        def step(c, k):
            return lambda dep: quad_operands(oq[c % 2], quad, c, k, dep)

        return stats + [s for c in range(NG) for s in [norm(c, n) for n in range(4)]
                        + [step(c, k) for k in range(14)]]

    def local_layer(rep):
        def fetch_weights(g):
            @pl.when(rep == 0)
            def _():
                @pl.when(g + 1 < NG)
                def _():
                    for cp in local_copies(g + 1):
                        cp.wait()

                @pl.when(g + 2 < NG)
                def _():
                    for cp in local_copies(g + 2):
                        cp.start()

                for cp in full_copies(g):
                    cp.start()

        def w_steps(g):
            nxt = 4 * ((g + 1) & (NG - 1))
            return (weight_steps(4 * g, wj, 0) + [None] * 4
                    + weight_steps(4 * g + 3, wot, g) + [None] * 4
                    + weight_steps(nxt + 1, wj, 1) + weight_steps(nxt + 2, wj, 2))

        ln = [input_ln_steps(j) for j in range(NP)]
        even, odd, first = local_qkv_steps(0, True), local_qkv_steps(1, True), w_steps(0)
        _run(ln[0])
        marks = _interleave(even[0::4], [None] * 8 + ln[1] + [None] * 6, first[:4] + [None] * 3)
        marks = _interleave(even[1::4], ln[2] + ln[4][:18], marks=marks)
        marks = _interleave(even[2::4], ln[3] + ln[4][18:], marks=marks)
        _interleave(even[3::4], ln[5] + ln[6], marks=marks)
        fetch_weights(0)
        att = local_att_steps(0, 0)
        marks = _interleave(odd[:2], ln[7], att[:16])
        _interleave(odd[2:], att[16:],
                    first[8:10] + first[16:20] + first[10:12] + first[20:] + [None], marks=marks)

        def group(g, _):
            fetch_weights(g)
            _interleave(local_qkv_steps(0) + local_qkv_steps(1),
                        local_att_steps(g - 1, 1) + local_att_steps(g, 0), w_steps(g))

        lax.fori_loop(1, NG, group, None)

        @pl.when(rep == 0)
        def _():
            pltpu.make_async_copy(wb, wb, b_sem).wait()

    def full_qkv_steps(gp, i, slot=None):
        def steps(quad):
            def emit(r, c, ys):
                for n in range(2):
                    g, kt = 2 * gp + r, 4 * quad + 2 * c + n
                    if i == 0:
                        xa[local_tile(2 * quad + c, n), g] = ys[n] * QSCALE
                    elif i == 1:
                        kk[g, kt] = _words(ys[n].astype(bf16).T)
                    else:
                        vt[g, kt] = _words(ys[n])
            return project2_steps(wq2, i if slot is None else slot, quad, emit)
        return [s for quad in range(NQ) for s in steps(quad)]

    def spread_steps(g):
        def step(kt, e):
            def run(dep):
                k = _after(kk[g + zeros[e % 8], kt, 56:, :], dep)
                x = jnp.stack([jnp.broadcast_to(k[:, f:f + 1], (8, 128))
                               for f in range(4 * e, 4 * e + 4)])
                x = lax.bitcast_convert_type(_halves(x).astype(f32), i32)
                h = e // 8
                for i in range(2):
                    kb[h // 2][g, h % 2 * 8 + 2 * kt + i, _rows(e % 8, 32), :] = (
                        x[:, _rows(i, 8)].reshape(32, 128))
            return run
        return [step(kt, e) for kt in range(VPU_TILES) for e in range(32)]

    def full_qkv(gp, more):
        pad = [None] * 3
        v_w, out_w = weight2_steps(8 * gp + 2, wq2, 2), weight2_steps(8 * gp + 3, wo2, gp)
        spread = [spread_steps(2 * gp + r) + pad for r in range(2)]
        if more:
            marks = _interleave(full_qkv_steps(gp + 1, 1), v_w + out_w)
            marks = _interleave(full_qkv_steps(gp, 0),
                                weight2_steps((8 * gp + 17) & (4 * NG - 1), wq2, 1),
                                [None] * 28 + spread[0], marks=marks)
            _interleave(full_qkv_steps(gp, 2), weight2_steps(8 * gp + 8, wq2, 0) + pad,
                        [None] * 28 + spread[1], marks=marks)
        else:
            marks = _interleave(full_qkv_steps(gp, 0), v_w + out_w)
            _interleave(full_qkv_steps(gp, 2), spread[0] + spread[1] + pad, marks=marks)

    def full_att(base, count, state, first=False, last=False):
        where = {b: ((base + b) >> 2, (base + b) & 3) for b in range(-1, count // 16 + 1)}

        def item(u):
            return *where[u // 16], u % 16 // 4, u % 4

        def operands(b, step, dep):
            g, quad = where[b]
            return quad_operands(oq[b % 2], quad, g, step, dep)

        def fetch_q(u, marks):
            g, quad, h, n = item(u)
            q = xa[4 * quad + n, g, _rows(h, DH), :]
            rows = [_after(q[_rows(i, 8)], marks and _slab(marks[14 * i])) for i in range(4)]
            qb[u % 2][0] = jnp.concatenate(
                [jnp.broadcast_to(x[d:d + 1], (8, 128)) for x in rows for d in range(8)], axis=0)
            return q

        m, m_next, den, acc, q_next = state or (None,) * 4 + (fetch_q(0, None),)
        for u in range(count + (2 if last else 0)):
            scores = u < count
            if scores:
                g, _, h, _ = item(u)
                parts = [jnp.zeros((DH, 128), f32)] * 4
                parts[h] = q_next
                q = jnp.concatenate(parts, axis=0).astype(bf16)
                top, marks = None, []
            for c in range(4):
                if scores:
                    for kt in range(4 * c, 4 * c + 4):
                        keys = 112 if kt < VPU_TILES else 128
                        s = _dot(_halves(kk[g, kt, :keys // 2, :]), q)
                        sbuf[u % 2][128 * kt:128 * kt + keys, :] = s
                        top = _slab_max(s, top)
                    marks += [(s, i) for i in range(14)]
                up, cp = divmod(4 * (u - 1) + c - 2, 4)
                if (first and up < 0) or up >= count:
                    continue
                if cp == 0:
                    m, den, acc = m_next, None, None
                gp, _, hp, np_ = item(up)
                for kt in range(4 * cp, 4 * cp + 4):
                    p = jnp.exp2(sbuf[up % 2][_rows(kt), :] - m)
                    den = _slab_sum(p, den)
                    o = _dot(_halves(vt[gp, kt, _rows(hp, DH // 2), :]), p)
                    acc = o if acc is None else acc + o
                if cp == 3:
                    o = acc * _inverse(jnp.sum(den, axis=0, keepdims=True))
                    oq[(up // 16 + first) % 2][0, hp, np_] = o
                if cp == 0 and up % 16 < 14 and not (first and up < 16):
                    operands(up // 16 - 1, up % 16, _slab(marks[-1]))
            if scores:
                s = None
                for e in range(2 * VPU_TILES):
                    qd = _head_after(qb[u % 2][zeros[e]], 8, _slab(marks[7 * e]), s)
                    kd = kb[h // 2][g + zeros[u % 8], h % 2 * 8 + e]
                    s = _slab_sum(lax.bitcast_convert_type(kd, f32) * qd)
                    sbuf[u % 2][pl.ds(128 * (e // 2) + 112 + 8 * (e % 2), 8), :] = s
                    top = jnp.maximum(top, s)
                m_next = jnp.max(top, axis=0, keepdims=True)
                if not (last and u + 1 == count):
                    q_next = fetch_q(u + 1, marks)
        if last:
            dep = None
            for step in range(14):
                dep = operands(count // 16 - 1, step, dep)
        return m, m_next, den, acc, q_next

    def full_layer(rep):
        @separately
        def _():
            marks = _interleave(proj_steps(0), local_att_steps(NG - 1, 1))
            _interleave(proj_steps(1), [None] * 6 + proj_ln_steps(0),
                        weight2_steps(1, wq2, 2) + [None], marks=marks)

        @separately
        def _():
            marks = _interleave(proj_steps(2), proj_ln_steps(1), weight2_steps(9, wq2, 1))
            marks = _interleave(proj_steps(3), [None] * 6 + proj_ln_steps(2),
                                weight2_steps(0, wq2, 0), marks=marks)
            _interleave(full_qkv_steps(0, 1, slot=2),
                        [None] * 6 + proj_ln_steps(3) + [None] * 56, marks=marks)
        lax.fori_loop(0, NG // 2 - 1, lambda gp, _: full_qkv(gp, True), None)
        separately(lambda: full_qkv(NG // 2 - 1, False))

        items = HEADS * NT
        head = ATT_UNROLL // 2
        state = full_att(0, head, None, first=True)
        state = lax.fori_loop(
            0, items // ATT_UNROLL - 1,
            lambda j, st: full_att(head // 16 + j * (ATT_UNROLL // 16), ATT_UNROLL, st), state)
        full_att((items - ATT_UNROLL + head) // 16, ATT_UNROLL - head, state, last=True)

        def proj(i, _):
            late = []

            def steps(quad):
                def emit(r, c, ys):
                    bits = []
                    for n in range(2):
                        t = 4 * quad + 2 * c + n
                        y = xb[t, 2 * i + r] + ys[n]
                        xa[t, 2 * i + r] = y
                        ma[t, 2 * i + r] = _moments(y)
                        bits.append(lax.bitcast_convert_type(y.astype(bf16).astype(f32), i32))
                    pair = lax.shift_right_logical(bits[0], 16) | bits[1]
                    if (quad, r, c) == (NQ - 1, 0, 0):
                        late.append(pair)
                    else:
                        xw[r, pl.ds(2 * quad + c, 128, stride=NP), :] = pair.T
                return project2_steps(wo2, i, quad, emit)

            _interleave([s for quad in range(NQ) for s in steps(quad)])

            @pl.when(rep == 1)
            def _():
                xw[0, pl.ds(NP - 2, 128, stride=NP), :] = late[0].T
                for r in (1, 0):
                    @quarters
                    def _(rows, words):
                        xio[2 * i + r, rows, :] = _halves(xw[r, words, :]).astype(f32).astype(bf16)

                    out_copy(2 * i + r).start()

        lax.fori_loop(0, NG // 2, proj, None)

    first_w = local_copies(0)
    for cp in first_w[1:3] + [x_copy(0)]:
        cp.start()
    for i in (1, 2):
        first_w[i].wait()
        x_copy(i).start()
        _run(weight_steps(i, wj, i))

    def stage_in(c, _):
        x_copy(c).wait()

        @pl.when(c + 3 < NG)
        def _():
            x_copy(c + 3).start()

        @pl.when(c + 2 == NG)
        def _():
            for cp in first_w[::3]:
                cp.start()

        @quarters
        def _(rows, words):
            xw[0, words, :] = _words(xio[c, rows, :])

        for j in range(NP):
            pair = xw[0, pl.ds(j, 128, stride=NP), :].T
            for n, bits in enumerate((pair << 16, pair & -65536)):
                y = lax.bitcast_convert_type(bits, f32)
                xa[2 * j + n, c] = y
                ma[2 * j + n, c] = _moments(y)

    lax.fori_loop(0, NG, stage_in, None)
    for cp in local_copies(1):
        cp.start()
    for cp in first_w[::3]:
        cp.wait()

    def two_layers(rep, _):
        zeros[:] = [(rep + i) >> 4 for i in range(8)]
        local_layer(rep)
        full_layer(rep)

    lax.fori_loop(0, 2, two_layers, None)
    for c in range(NG):
        out_copy(c).wait()


@jax.jit
def pallas_interleave_layers__sliding_local_dilated__softmax_full_mha__prompt_kernel(
    A_x: jax.Array,
    A_wqkv: jax.Array,
    A_wo: jax.Array,
    B_x: jax.Array,
    B_wqkv: jax.Array,
    B_wo: jax.Array,
):
    del B_x
    assert A_x.shape == (1, SEQ, D) and A_x.dtype == bf16
    vmem, dma = pltpu.VMEM, pltpu.SemaphoreType.DMA
    tile, words = (128, 128), (64, 128)
    scratch = [
        vmem((NG, SEQ, 128), bf16),
        vmem((2, SEQ // 2, 128), i32),
        *[vmem((4 * NG, D, 128), bf16)] * 2,
        vmem((3, 7, D // 8, 128), i32),
        vmem((NG, 7, D // 8, 128), i32),
        vmem((3, 49) + tile, bf16),
        vmem((NG // 2, 49) + tile, bf16),
        vmem((2, 4, 4, 32, 128), i32),
        *[vmem((NT, NG) + tile, f32)] * 2,
        *[vmem((NP, 16, D // 4, 128), i32)] * 2,
        vmem((NQ, 49, D // 4, 128), bf16),
        *[vmem((WIN,) + tile, f32)] * 2,
        *[vmem((2 * WIN - 1,) + tile, f32)] * 4,
        vmem((2,) + tile, f32),
        *[vmem((4, NG) + tile, f32)] * 2,
        vmem((NT, NG, 16, 128), f32),
        *[vmem((4, NG, 16, 128), f32)] * 2,
        *[vmem((NG, NT) + words, i32)] * 2,
        *[vmem((1, DH * 8, 128), f32)] * 2,
        *[vmem((SEQ, 128), f32)] * 2,
        *[vmem((1, 4, 4, DH, 128), f32)] * 2,
        dma((NG,)), dma((4 * NG,)), dma(()), dma((NG,)),
        *[vmem((2,) + tile, f32)] * 4,
    ]
    hbm = pl.BlockSpec(memory_space=pl.ANY)
    out = pl.pallas_call(
        _kernel,
        out_shape=jax.ShapeDtypeStruct((SEQ, D), bf16),
        in_specs=[hbm] * 5,
        out_specs=hbm,
        scratch_shapes=scratch,
        compiler_params=pltpu.CompilerParams(
            vmem_limit_bytes=127 * 1024 * 1024,
            disable_bounds_checks=True,
            flags={"XLA_TPU_FORCE_LP_LLO_SCHEDULER": True},
        ),
        name="interleaved_layers",
    )(A_x.reshape(SEQ, D), A_wqkv, A_wo, B_wqkv, B_wo)
    return out.reshape(1, SEQ, D)
```
